```python
import jax
import jax.numpy as jnp

def _softmax(x, axis=-1):
    return jax.nn.softmax(x, axis=axis)
def _gelu(x):
    return jax.nn.gelu(x, approximate=True)
def _silu(x):
    return jax.nn.silu(x)
def _sigmoid(x):
    return jax.nn.sigmoid(x)
def _layernorm(x, axis=-1, eps=1e-5):
    m = jnp.mean(x, axis=axis, keepdims=True)
    v = jnp.var(x, axis=axis, keepdims=True)
    return (x - m) / jnp.sqrt(v + eps)
def _scatter_add(tgt, idx, src, axis=0):
    return tgt.at[idx].add(src)
def _segment_sum(src, seg, n):
    return jax.ops.segment_sum(src, seg, n)
class _Rng:
    def __init__(self, key):
        self._k = key
    def _next(self):
        self._k, sub = jax.random.split(self._k)
        return sub
    def normal(self, shape):
        return jax.random.normal(self._next(), shape, dtype=jnp.bfloat16)
    def randint(self, lo, hi, shape):
        return jax.random.randint(self._next(), shape, lo, hi, dtype=jnp.int32)
    def uniform(self, shape, lo=0.0, hi=1.0):
        return jax.random.uniform(self._next(), shape, jnp.bfloat16, lo, hi)
    def permutation(self, n):
        return jax.random.permutation(self._next(), n)


kernel_name = 'gated_mix__linear_kernel_hedgehog__moe_arch_mod__prompt'

def setup_inputs():
    _rng = _Rng(jax.random.key(int.from_bytes(__import__("os").urandom(4), "little")))
    _w = (lambda a: (lambda t: t.astype(jnp.bfloat16) if jnp.issubdtype(t.dtype, jnp.floating) else t)(jnp.asarray(a)))
    def _A_setup():
        B, S, D, H = 1, 2048, 1024, 32
        Dh = D // H
        return {
            "x": _w((lambda *s: _rng.normal(s) * 0.05)(B, S, D)),
            "wqkv": _w((lambda *s: _rng.normal(s) * 0.05)(D, 3 * D)),
            "w_phi": _w((lambda *s: _rng.normal(s) * 0.05)(H, Dh, Dh) * (Dh ** -0.5)),
            "wo": _w((lambda *s: _rng.normal(s) * 0.05)(D, D)),
        }
    _A_in = _A_setup()

    def _B_setup():
        B, S, D, F, C = 1, 2048, 1024, 3584, 1
        return {
            "x": _w((lambda *s: _rng.normal(s) * 0.05)(B, S, D)),
            "w_r": _w((lambda *s: _rng.normal(s) * 0.05)(D)),
            "w_gate": _w((lambda *s: _rng.normal(s) * 0.05)(D, F)),
            "w_up": _w((lambda *s: _rng.normal(s) * 0.05)(D, F)),
            "w_down": _w((lambda *s: _rng.normal(s) * 0.05)(F, D)),
        }
    _B_in = _B_setup()

    return {
        "A_x": _A_in["x"],
        "A_wqkv": _A_in["wqkv"],
        "A_w_phi": _A_in["w_phi"],
        "A_wo": _A_in["wo"],
        "B_x": _B_in["x"],
        "B_w_r": _B_in["w_r"],
        "B_w_gate": _B_in["w_gate"],
        "B_w_up": _B_in["w_up"],
        "B_w_down": _B_in["w_down"],
        "gate_w": _w((lambda *s: _rng.normal(s) * 0.05)(1024)),
    }

def reference(A_x, A_wqkv, A_w_phi, A_wo, B_x, B_w_r, B_w_gate, B_w_up, B_w_down, gate_w):
    def _A_ref(x, wqkv, w_phi, wo):
        B, S, D = x.shape
        H = 32; Dh = D // H
        qkv = (lambda x, *d: x.transpose(*d))((x @ wqkv).reshape(B, S, 3, H, Dh), 2, 0, 3, 1, 4)
        q, k, v = qkv[0], qkv[1], qkv[2]
        pq = jnp.einsum("bhsd,hdf->bhsf", q, w_phi)
        pk = jnp.einsum("bhsd,hdf->bhsf", k, w_phi)
        phi_q = jnp.concatenate([_softmax(pq, axis=-1), _softmax(-pq, axis=-1)], axis=-1)
        phi_k = jnp.concatenate([_softmax(pk, axis=-1), _softmax(-pk, axis=-1)], axis=-1)
        kv = jnp.einsum("bhsf,bhsd->bhfd", phi_k, v)
        z  = jnp.einsum("bhsf->bhf", phi_k)
        num = jnp.einsum("bhqf,bhfd->bhqd", phi_q, kv)
        den = jnp.einsum("bhqf,bhf->bhq", phi_q, z)[..., None] + 1e-6
        o = num / den
        return (lambda x, *d: x.transpose(*d))(o, 0, 2, 1, 3).reshape(B, S, D) @ wo

    def _B_ref(x, w_r, w_gate, w_up, w_down):
        B, S, D = x.shape
        C = 1
        r = x @ w_r
        idx = jnp.argsort(-r, axis=-1)[:, :C]
        idx_e = jnp.repeat(idx.reshape(B, C, 1), D, axis=2)
        x_sel = jnp.take_along_axis(x, idx_e, axis=1)
        g = _silu(x_sel @ w_gate)
        u = x_sel @ w_up
        y = (g * u) @ w_down
        r_sel = _sigmoid(jnp.take_along_axis(r, idx, axis=1))
        y = y * r_sel.reshape(B, C, 1)
        b_off = (jnp.arange(B) * S).reshape(B, 1)
        flat_idx = (idx + b_off).reshape(B * C)
        zero = (x * 0.0).reshape(B * S, D)
        upd = _scatter_add(zero, flat_idx, y.reshape(B * C, D), axis=0)
        return x + upd.reshape(B, S, D)

    x = A_x
    g = _sigmoid((x * gate_w).sum(-1, keepdims=True))
    a = _A_ref(x, A_wqkv, A_w_phi, A_wo)
    b = _B_ref(x, B_w_r, B_w_gate, B_w_up, B_w_down)
    return g * a + (1 - g) * b
```

```python
import jax
import jax.numpy as jnp
import jax.experimental.pallas as pl
import jax.experimental.pallas.tpu as pltpu

_BF = jnp.bfloat16
_F32 = jnp.float32
_LOG2E = 1.4426950408889634

_S, _D, _H, _DH, _F = 2048, 1024, 32, 32, 3584
_T = 512
_NT = _S // _T
_FC = _F // _NT
_NP = _H // 2


def _dg(a, b, ca, cb):
    return jax.lax.dot_general(a, b, (((ca,), (cb,)), ((), ())), preferred_element_type=_F32)


def _pair_reduce(v, op):
    r = v[0:8]
    for j in range(1, 8):
        r = op(r, v[8 * j:8 * j + 8])
    r = op(r, pltpu.roll(r, 2, 0))
    return op(r, pltpu.roll(r, 4, 0))


def _rep8(v):
    return jnp.concatenate([v] * 8, axis=0)


def _dual_exp(p):
    ep = jnp.exp2(p - _rep8(_pair_reduce(p, jnp.maximum)))
    en = jnp.exp2(_rep8(_pair_reduce(p, jnp.minimum)) - p)
    return ep, en, _pair_reduce(ep, jnp.add), _pair_reduce(en, jnp.add)


def _col_bcast(row):
    return jnp.broadcast_to(row, (128, row.shape[1])).T


def _kernel(x_hbm, wqkv_hbm, wphi_ref, wo_hbm, wr_ref, wg_hbm, wu_hbm, wd_hbm, gw_ref,
            out_hbm,
            x_v, w_v, wo_v, wg_v, wu_v, wd_v, wt_v, kv_v, z_v, kvm_v, ot_v, xcol_v, y_v, out_v,
            sem_x, sem_w, sem_wo, sem_g, sem_u, sem_d, sem_o):
    def cp_x(i):
        return pltpu.make_async_copy(x_hbm.at[pl.ds(i * _T, _T)], x_v.at[i], sem_x.at[i])

    def cp_w(j):
        return pltpu.make_async_copy(wqkv_hbm.at[:, pl.ds(j * _D, _D)], w_v.at[j], sem_w.at[j])

    def cp_wo():
        return pltpu.make_async_copy(wo_hbm, wo_v, sem_wo.at[0])

    def cp_g(i):
        return pltpu.make_async_copy(wg_hbm.at[:, pl.ds(i * _FC, _FC)], wg_v.at[i], sem_g.at[i])

    def cp_u(i):
        return pltpu.make_async_copy(wu_hbm.at[:, pl.ds(i * _FC, _FC)], wu_v.at[i], sem_u.at[i])

    def cp_d(i):
        return pltpu.make_async_copy(wd_hbm.at[pl.ds(i * _FC, _FC)], wd_v.at[i], sem_d.at[i])

    def cp_o(i):
        return pltpu.make_async_copy(out_v.at[i], out_hbm.at[pl.ds(i * _T, _T)], sem_o.at[i])

    cp_w(1).start()
    cp_x(0).start()

    rows = jax.lax.broadcasted_iota(jnp.int32, (128, _DH), 0)
    cols = jax.lax.broadcasted_iota(jnp.int32, (128, _DH), 1)
    sel = jnp.where(((rows >> 1) & 31) == cols, 1.0, 0.0).astype(_BF)
    lfull = _dg(sel, wphi_ref[...].reshape(_H * _DH, _DH), 1, 1)
    rows = jax.lax.broadcasted_iota(jnp.int32, (128, _D), 0)
    cols = jax.lax.broadcasted_iota(jnp.int32, (128, _D), 1)
    lmat = jnp.where(((cols >> 5) & 3) == 2 * (rows >> 6) + (rows & 1), lfull, 0.0).astype(_BF)

    def fold(j):
        for g in range(8):
            c = slice(128 * g, 128 * g + 128)
            wt_v[j, c, :] = (_dg(lmat[:, c], w_v[j, :, c], 1, 1) * _LOG2E).astype(_BF)

    cp_w(1).wait()
    cp_w(2).start()
    fold(1)
    cp_x(0).wait()
    for i in range(1, _NT):
        cp_x(i).start()
    cp_w(2).wait()
    cp_w(0).start()
    cp_wo().start()
    for i in range(_NT):
        cp_g(i).start()
        cp_u(i).start()
        cp_d(i).start()
    for g in range(8):
        c = slice(128 * g, 128 * g + 128)
        wt_v[2, c, :] = w_v[2, :, c].T

    kv_v[...] = jnp.zeros_like(kv_v)
    z_v[...] = jnp.zeros_like(z_v)
    wr = wr_ref[...].astype(_F32)

    def phase1(i, carry):
        best, bidx = carry

        @pl.when(i > 0)
        def _():
            cp_x(i).wait()

        xt = x_v[i]
        pk = _dg(wt_v[1], xt, 1, 1)
        vt = _dg(wt_v[2], xt, 1, 1).astype(_BF)
        for p in range(_NP):
            r = slice(64 * p, 64 * p + 64)
            ep, en, sp, sn = _dual_exp(pk[r])
            phi = jnp.concatenate([ep * _rep8(1.0 / sp), en * _rep8(1.0 / sn)], axis=0)
            zs = phi[:, 0:128]
            for c in range(1, _T // 128):
                zs = zs + phi[:, 128 * c:128 * c + 128]
            z_v[p] += zs
            kv_v[p] += _dg(vt[r], phi.astype(_BF), 1, 1)
        rs = jnp.sum(xt.astype(_F32) * wr, axis=1, keepdims=True).astype(_BF).astype(_F32)
        for j in range(_T // 8):
            rj = rs[8 * j:8 * j + 8]
            upd = rj > best
            best = jnp.where(upd, rj, best)
            bidx = jnp.where(upd, i * _T + 8 * j, bidx)
        return best, bidx

    best, bidx = jax.lax.fori_loop(
        0, _NT, phase1,
        (jnp.full((8, 1), -jnp.inf, _F32), jnp.zeros((8, 1), jnp.int32)))

    bidx = bidx + jax.lax.broadcasted_iota(jnp.int32, (8, 1), 0)
    rmax = jnp.max(best, axis=0, keepdims=True)
    idx = jnp.min(jnp.where(best == rmax, bidx, _S - 1))
    r_sel = jax.nn.sigmoid(rmax)
    tsel = idx // _T
    rsel = idx - tsel * _T
    grp = x_v[tsel, pl.ds(pl.multiple_of((rsel >> 4) << 4, 16), 16), :].astype(_F32)
    hit = jax.lax.broadcasted_iota(jnp.int32, (16, _D), 0) == (rsel & 15)
    xcol_v[...] = _col_bcast(jnp.sum(jnp.where(hit, grp, 0.0), axis=0, keepdims=True))

    cp_w(0).wait()
    fold(0)
    rows = jax.lax.broadcasted_iota(jnp.int32, (64, 128), 0)
    cols = jax.lax.broadcasted_iota(jnp.int32, (64, 128), 1)
    same_head = (rows >> 5) == (cols & 1)
    for p in range(_NP):
        kvm_v[p] = jnp.where(same_head, kv_v[p], 0.0).astype(_BF)
        z_v[p] = jnp.broadcast_to(jnp.sum(z_v[p], axis=1, keepdims=True), (128, 128))
    y_v[...] = jnp.zeros_like(y_v)
    gw = gw_ref[...].astype(_F32)
    cp_wo().wait()

    def phase2(i, carry):
        ti = (tsel + 1 + i) % _NT
        cp_g(i).wait()
        cp_u(i).wait()
        cp_d(i).wait()
        xt = x_v[ti]
        pq = _dg(wt_v[0], xt, 1, 1)

        ag = jnp.zeros((8, _FC), _F32)
        au = jnp.zeros((8, _FC), _F32)
        for j in range(_D // 16):
            r = slice(16 * j, 16 * j + 16)
            xc = jnp.concatenate([xcol_v[r, :]] * (_FC // 128), axis=1)
            tg = wg_v[i, r, :].astype(_F32) * xc
            tu = wu_v[i, r, :].astype(_F32) * xc
            ag = ag + tg[0:8] + tg[8:16]
            au = au + tu[0:8] + tu[8:16]
        hg = jnp.sum(ag, axis=0, keepdims=True)
        hu = jnp.sum(au, axis=0, keepdims=True)
        hcol = _col_bcast(hg * jax.nn.sigmoid(hg) * hu)
        ay = y_v[...]
        for j in range(_FC // 16):
            r = slice(16 * j, 16 * j + 16)
            td = wd_v[i, r, :].astype(_F32) * jnp.concatenate([hcol[r]] * (_D // 128), axis=1)
            ay = ay + td[0:8] + td[8:16]
        y_v[...] = ay
        y = jnp.sum(ay, axis=0, keepdims=True) * r_sel

        for p in range(_NP):
            r = slice(64 * p, 64 * p + 64)
            ep, en, sp, sn = _dual_exp(pq[r])
            zp = jnp.concatenate([z_v[p, 0:64, :]] * (_T // 128), axis=1)
            zn = jnp.concatenate([z_v[p, 64:128, :]] * (_T // 128), axis=1)
            ip, iq = 1.0 / sp, 1.0 / sn
            den = _pair_reduce(ep * zp, jnp.add) * ip + _pair_reduce(en * zn, jnp.add) * iq + 1e-6
            inv = 1.0 / den
            phi = jnp.concatenate([ep * _rep8(ip * inv), en * _rep8(iq * inv)], axis=0)
            ot_v[r, :] = _dg(kvm_v[p], phi.astype(_BF), 1, 0).astype(_BF)
        a = _dg(ot_v[...], wo_v[...], 0, 0)
        g = jax.nn.sigmoid(jnp.sum(xt.astype(_F32) * gw, axis=1, keepdims=True))
        tok = jax.lax.broadcasted_iota(jnp.int32, (_T, 1), 0) + ti * _T
        b = xt.astype(_F32) + jnp.where(tok == idx, y, 0.0)
        out_v[ti] = (g * a + (1.0 - g) * b).astype(_BF)
        cp_o(ti).start()
        return carry

    jax.lax.fori_loop(0, _NT, phase2, 0)
    for i in range(_NT):
        cp_o(i).wait()


@jax.jit
def pallas_gated_mix__linear_kernel_hedgehog__moe_arch_mod__prompt_kernel(
    A_x: jax.Array,
    A_wqkv: jax.Array,
    A_w_phi: jax.Array,
    A_wo: jax.Array,
    B_x: jax.Array,
    B_w_r: jax.Array,
    B_w_gate: jax.Array,
    B_w_up: jax.Array,
    B_w_down: jax.Array,
    gate_w: jax.Array,
):
    hbm = pl.BlockSpec(memory_space=pl.ANY)
    vmem = pl.BlockSpec(memory_space=pltpu.VMEM)
    dma = pltpu.SemaphoreType.DMA
    out = pl.pallas_call(
        _kernel,
        out_shape=jax.ShapeDtypeStruct((_S, _D), _BF),
        in_specs=[hbm, hbm, vmem, hbm, vmem, hbm, hbm, hbm, vmem],
        out_specs=hbm,
        scratch_shapes=[
            pltpu.VMEM((_NT, _T, _D), _BF),
            pltpu.VMEM((3, _D, _D), _BF),
            pltpu.VMEM((_D, _D), _BF),
            pltpu.VMEM((_NT, _D, _FC), _BF),
            pltpu.VMEM((_NT, _D, _FC), _BF),
            pltpu.VMEM((_NT, _FC, _D), _BF),
            pltpu.VMEM((3, _D, _D), _BF),
            pltpu.VMEM((_NP, 64, 128), _F32),
            pltpu.VMEM((_NP, 128, 128), _F32),
            pltpu.VMEM((_NP, 64, 128), _BF),
            pltpu.VMEM((_D, _T), _BF),
            pltpu.VMEM((_D, 128), _F32),
            pltpu.VMEM((8, _D), _F32),
            pltpu.VMEM((_NT, _T, _D), _BF),
            dma((_NT,)), dma((3,)), dma((1,)),
            dma((_NT,)), dma((_NT,)), dma((_NT,)), dma((_NT,)),
        ],
        compiler_params=pltpu.CompilerParams(vmem_limit_bytes=100 * 1024 * 1024),
    )(A_x.reshape(_S, _D), A_wqkv, A_w_phi, A_wo, B_w_r.reshape(1, _D),
      B_w_gate, B_w_up, B_w_down, gate_w.reshape(1, _D))
    return out.reshape(1, _S, _D)
```

```python
import jax
import jax.numpy as jnp
import jax.experimental.pallas as pl
import jax.experimental.pallas.tpu as pltpu

_BF = jnp.bfloat16
_F32 = jnp.float32
_I32 = jnp.int32
_LOG2E = 1.4426950408889634

_S, _D, _H, _DH, _F = 2048, 1024, 32, 32, 3584
_T = 512
_HT = _T // 2
_HD = _D // 2
_NT = _S // _T
_FC = _F // _NT
_NP = _H // 2

_A_SLOT = (4, 5, 0, 3, 6, 7, 8)
_B_SLOT = (4, 0, 5, 6, 3, 7, 8)

_FIRST = ("+r +s ! W0 +a v3:16,16,16,16 v5 W1 +b v4:16,16,16,16 v2 v1 v7 W2 k2 k5 k4 +f2 k3:4,4 +f1 "
          "k1:5,5 k7:5,5 +f0 k6:6,6 +f3 g2:4,4,4,4 v6:2,2,2,2 g1 g0 g3")
_PHASE1 = ("+r k2:5,5 k5:5,5 v2:3,3,3,3 +o v5:6,6,6,6 k4 +f2 k3:8,8 +f1 v4:4,4,4,4 +s v3:2,2,2,2 g2 "
           "k1:4,4 g1 k7 +f0 k6:8,8 +f3 v1:4,4,4,4 v7 v6 g0 g3")
_PHASE2 = ("+h q4:2,2 q1:2,2 q7:2,2 q5:1,1 +f0 q3:6,6 +f1 q2:7,7 g0 +f2 q6:7,7 g1 +f3 o3:3,3,3,3 g2 "
           "o6:3,3,3,3 g3 +a ! +d o5:1,1,1,1 o4:1,1,1,1 +e1 o2:1,1,1,1 +e2 o1:2,2,2,2 +e3 o7:1,1,1,1 +e0 !")


def _dg(a, b, ca, cb):
    return jax.lax.dot_general(a, b, (((ca,), (cb,)), ((), ())), preferred_element_type=_F32)


def _bf(w):
    return pltpu.bitcast(w, _BF)


def _split(w):
    return [pltpu.unpack_elementwise(w, index=j, packed_dtype=_BF, unpacked_dtype=_F32) for j in range(2)]


def _join(even, odd):
    return pltpu.pack_elementwise([even, odd], packed_dtype=_BF)


def _a_sums(a11, a12, a21, a22):
    return (a11 + a22, a21 + a22, a11 + a12, a21 - a11, a12 - a22)


def _b_sums(b11, b12, b21, b22):
    return (b11 + b22, b12 - b22, b21 - b11, b11 + b12, b21 + b22)


def _mix(c, m):
    if c == 0:
        return m(0) + m(3) - m(4) + m(6)
    if c == 1:
        return m(2) + m(4)
    if c == 2:
        return m(1) + m(3)
    return m(0) - m(1) + m(2) + m(5)


def _sum_piece(src, dst, sums, r, c, which=range(5)):
    even, odd = zip(*[(0.0, 0.0) if b is None else _split(b[pl.ds(r, 8), c:c + 256]) for b in src])
    even, odd = sums(*even), sums(*odd)
    for k in which:
        dst[k][pl.ds(r, 8), c:c + 256] = _join(even[k], odd[k])


def _paced(w, zeros):
    if not zeros:
        return w
    groups = w.shape[0] // 8
    first = [w[8 * g:8 * g + 8, 0:128] for g in range(groups)]
    for j, z in enumerate(zeros):
        g = max((j + 1) * groups // len(zeros) - 1, 0)
        first[g] = first[g] | z
    first = jnp.concatenate(first, axis=0)
    return first if w.shape[1] == 128 else jnp.concatenate([first, w[:, 128:]], axis=1)


def _play(program, steps, pieces):
    queue = []
    for word in program.split():
        if word == "!":
            while queue:
                queue.pop(0)()
        elif word[0] == "+":
            queue.extend(pieces(word[1:]))
        else:
            name, _, counts = word.partition(":")
            name, _, tile = name.partition(".")
            step, tiles = steps[name[0]]
            tiles = [int(tile)] if tile else range(tiles)
            counts = [int(n) for n in counts.split(",")] if counts else [0] * len(tiles)
            for t, n in zip(tiles, counts):
                step(int(name[1:]), t, [queue.pop(0)() for _ in range(min(n, len(queue)))])
    assert not queue


def _recip(v):
    r = pl.reciprocal(v, approx=True)
    return r * (2.0 - v * r)


def _pair_reduce(v, op):
    r = v[0:8]
    for j in range(1, 8):
        r = op(r, v[8 * j:8 * j + 8])
    r = op(r, pltpu.roll(r, 2, 0))
    return op(r, pltpu.roll(r, 4, 0))


def _rep8(v):
    return jnp.concatenate([v] * 8, axis=0)


def _dual_exp(p):
    ep = jnp.exp2(p - _rep8(_pair_reduce(p, jnp.maximum)))
    en = jnp.exp2(_rep8(_pair_reduce(p, jnp.minimum)) - p)
    return ep, en, _recip(_pair_reduce(ep, jnp.add)), _recip(_pair_reduce(en, jnp.add))


def _col_bcast(row):
    return jnp.broadcast_to(row, (128, row.shape[1])).T


def _matvec(w_ref, col_ref, c, j0, j1, acc=None):
    for j in range(j0, j1):
        t = _bf(w_ref[8 * j:8 * j + 8, 128 * c:128 * c + 128]).astype(_F32) * col_ref[16 * j:16 * j + 16, :]
        acc = t[0:8] if acc is None else acc + t[0:8]
        acc = acc + t[8:16]
    return acc


def _kernel(x_hbm, wqkv_hbm, wphi_hbm, wo_hbm, wr_hbm, wg_hbm, wu_hbm, wd_hbm, gw_hbm,
            out_hbm,
            x_v, w_v, wg_v, wu_v, wd_v, wphi_v, wr_v, gw_v,
            lm_v, lk_v, lq_v, lv_v, lo_v, r_v, phi_v, a_v, kv_v, z_v, kvm_v, g_v, top_v, arg_v,
            f_v, xc_v, hc_v, out_v,
            sem_x, sem_w, sem_v, sem_wo, sem_s, sem_g, sem_u, sem_d, sem_o):
    x_hbm, wqkv_hbm, wo_hbm, wg_hbm, wu_hbm, wd_hbm = (
        r.bitcast(_I32) for r in (x_hbm, wqkv_hbm, wo_hbm, wg_hbm, wu_hbm, wd_hbm))

    def cp_x(i):
        return pltpu.make_async_copy(x_hbm.at[pl.ds(i * _HT, _HT)], x_v.at[i], sem_x.at[i])

    def cp_w(j):
        return pltpu.make_async_copy(wqkv_hbm.at[:, pl.ds(j * _D, _D)], w_v.at[j], sem_w.at[j])

    def cp_v(o):
        return pltpu.make_async_copy(wqkv_hbm.at[:, pl.ds(2 * _D + o * _HD, _HD)],
                                     lv_v.at[pl.ds(512 * o, 512)], sem_v.at[o])

    def cp_wo(k):
        return pltpu.make_async_copy(wo_hbm.at[pl.ds(256 * (k // 2), 256), pl.ds(_HD * (k % 2), _HD)],
                                     lo_v.at[pl.ds(256 * k, 256)], sem_wo.at[k])

    cp_small = [pltpu.make_async_copy(src, dst, sem_s.at[j]) for j, (src, dst) in enumerate(
        ((wphi_hbm, wphi_v), (wr_hbm, wr_v), (gw_hbm, gw_v)))]

    def cp_ffn(i):
        cols = pl.ds(i * _FC, _FC)
        return (pltpu.make_async_copy(wg_hbm.at[:, cols], wg_v.at[i], sem_g.at[i]),
                pltpu.make_async_copy(wu_hbm.at[:, cols], wu_v.at[i], sem_u.at[i]),
                pltpu.make_async_copy(wd_hbm.at[pl.ds(i * (_FC // 2), _FC // 2)], wd_v.at[i], sem_d.at[i]))

    def cp_o(i, t):
        return pltpu.make_async_copy(out_v.at[t], out_hbm.at[pl.ds(t * _T, _T)], sem_o.at[i])

    cp_x(0).start()
    for cp in cp_small:
        cp.start()
    cp_v(0).start()

    zero_reg = jnp.zeros((8, 128), _I32)
    kv_v[...] = jnp.zeros_like(kv_v)
    z_v[...] = jnp.zeros_like(z_v)
    f_v[...] = jnp.zeros_like(f_v)
    top_v[...] = jnp.full((8, 128), -jnp.inf, _F32)
    arg_v[...] = jnp.zeros_like(arg_v)
    g_v[_S // 128, 0:8, :] = jnp.zeros((8, 128), _F32)
    r_v[5 * _NT, 0:8, 0:128] = zero_reg
    lv_v[9 * 256:, 0:128] = zero_reg
    lo_v[9 * 256:, 0:128] = zero_reg
    out_v[_NT, 0:16, 0:128] = jnp.zeros((16, 128), _BF)
    for p_v in phi_v:
        p_v[16, 0:8, :] = zero_reg

    for cp in cp_small:
        cp.wait()
    rows = jax.lax.broadcasted_iota(_I32, (128, _DH), 0)
    cols = jax.lax.broadcasted_iota(_I32, (128, _DH), 1)
    sel = jnp.where(((rows >> 1) & 24) + (rows & 7) == cols, 1.0, 0.0).astype(_BF)
    full = _dg(sel, wphi_v[...].reshape(_H * _DH, _DH), 1, 1)
    rows = jax.lax.broadcasted_iota(_I32, (128, _D), 0)
    cols = jax.lax.broadcasted_iota(_I32, (128, _D), 1)
    keep = ((cols >> 5) & 3) == 2 * (rows >> 6) + ((rows >> 3) & 1)
    lm_v[...] = pltpu.bitcast(jnp.where(keep, full, 0.0).astype(_BF), _I32)

    def fold(j, l_v):
        for g in range(4):
            for d in range(4):
                blk = []
                for gg in (g, g + 4):
                    c = slice(128 * gg, 128 * gg + 128)
                    for dd in (d, d + 4):
                        blk.append(_dg(_bf(lm_v[:, c]), _bf(w_v[j, 64 * dd:64 * dd + 64, c]), 1, 1) * _LOG2E)
                blk += _a_sums(*blk)
                for m in range(7):
                    l = blk[_A_SLOT[m]].reshape(8, 16, 128)
                    l_v[m, 64 * g:64 * g + 64, 128 * d:128 * d + 128] = (
                        _join(l[:, 0:8], l[:, 8:16]).reshape(64, 128))

    def weight_piece(ref, sums, r, c, have=range(4), which=range(5)):
        def run():
            grp = [ref.at[256 * k:256 * k + 256] for k in range(9)]
            _sum_piece([grp[k] if k in have else None for k in range(4)], grp[4:], sums,
                       pl.multiple_of(r, 8), c, which)
            return ref[9 * 256:, 0:128]
        return run

    def x_blk(i, k):
        return x_v.at[i, 128 * (k % 2):128 * (k % 2) + 128, _HD * (k // 2):_HD * (k // 2) + _HD]

    def tok_words(i, m):
        k = _B_SLOT[m]
        return x_blk(i, k) if k < 4 else r_v.at[5 * i + k - 4]

    def phase1(i, zero, program):
        pk, pv = {}, {}

        def kprod(m, t, zeros):
            pk[m - 1, t] = _dg(_bf(_paced(lk_v[m - 1], zeros)), _bf(tok_words(i, m - 1)[64 * t:64 * t + 64, :]), 1, 1)

        def vprod(m, c, zeros):
            k = _A_SLOT[m - 1]
            pv[m - 1, c] = _dg(_bf(_paced(tok_words(i, m - 1)[...], zeros)),
                               _bf(lv_v[256 * k:256 * k + 256, 128 * c:128 * c + 128]), 1, 0)

        def kv(blk, c, zeros):
            vt = _mix(blk, lambda m: pv[m, c]).astype(_BF).T
            for h in range(2):
                p = 2 * c + h
                phi = [phi_v[blk][2 * p + t + zero] for t in range(2)]
                phi[0] = _paced(phi[0], zeros[h::2])
                kv_v[8 * (blk // 2) + p] += _dg(vt[64 * h:64 * h + 64], _bf(jnp.concatenate(phi, axis=1)), 1, 1)

        def wait(j, t, zeros):
            cp_v(j).wait() if j < 2 else cp_w(1).wait()
            if j == 0:
                cp_w(1).start()
            elif j == 1:
                cp_x(1).start()
                for k in range(4):
                    cp_wo(k).start()
            else:
                for k in range(2, _NT):
                    cp_x(k).start()
                cp_w(0).start()
                for k in range(_NT):
                    for cp in cp_ffn(k):
                        cp.start()
                fold(1, lk_v)

        def sum_piece(j):
            def run():
                _sum_piece([x_blk(i, k) for k in range(4)], [r_v.at[5 * i + k + zero] for k in range(5)],
                           _b_sums, 8 * (j // 2), 256 * (j % 2))
                return r_v[5 * _NT, 0:8, 0:128]
            return run

        def feat_piece(blk, t, p):
            def run():
                ep, en, ip, iq = _dual_exp(_mix(blk, lambda m: pk[m, t][64 * p:64 * p + 64]))
                ep, en = ep * _rep8(ip), en * _rep8(iq)
                z_v[8 * (blk // 2) + p] += jnp.concatenate([ep, en], axis=0)
                phi_v[blk][2 * p + t] = _join(ep, en)
                return phi_v[blk][16 + zero, 0:8, :]
            return run

        def score_piece(c):
            def run():
                xh = _bf(x_v[i, 16 * c:16 * c + 16, :]).astype(_F32)
                wr = wr_v[...].astype(_F32).reshape(1, _D)
                gw = gw_v[...].astype(_F32).reshape(1, _D)
                g = jax.nn.sigmoid(jnp.sum(xh * gw, axis=1, keepdims=True))
                g_v[4 * i + c // 4, 32 * (c % 4):32 * (c % 4) + 32, :] = jnp.broadcast_to(g, (32, 128))
                sc = jnp.sum(xh * wr, axis=1, keepdims=True).astype(_BF).astype(_F32)
                best, bidx = top_v[...], arg_v[0]
                for j in range(4):
                    rj = sc[8 * j:8 * j + 8]
                    upd = rj > best
                    best = jnp.where(upd, rj, best)
                    bidx = jnp.where(upd, i * _T + 32 * c + 8 * j, bidx)
                top_v[...] = best
                arg_v[0] = bidx
                return arg_v[1 + zero] | pltpu.bitcast(g_v[_S // 128 + zero, 0:8, :], _I32)
            return run

        def pieces(name):
            if name == "r":
                return [sum_piece(j) for j in range(32)]
            if name == "s":
                return [score_piece(c) for c in range(16)]
            if name in "ab":
                part = ((0, 1), [2]) if name == "a" else (range(4), (0, 1, 3, 4))
                return [weight_piece(lv_v, _a_sums, 8 * (j // 2) + zero, 256 * (j % 2), *part) for j in range(64)]
            if name == "o":
                start = jnp.minimum(88 * (i - 1), 256 - 88)
                return [weight_piece(lo_v, _b_sums, start + 8 * (j // 2), 256 * (j % 2)) for j in range(22)]
            return [feat_piece(int(name[1]), t, p) for t in ([int(name[2])] if name[2:] else range(2))
                    for p in range(8)]

        _play(program, {"k": (kprod, 2), "v": (vprod, 4), "g": (kv, 4), "W": (wait, 1)}, pieces)

    def later_tile(i):
        cp_x(i).wait()
        phase1(i, i >> 8, _PHASE1)

    cp_x(0).wait()
    cp_v(1).start()
    phase1(0, arg_v[1, 0, 0], _FIRST)
    for k in range(4):
        cp_wo(k).wait()
    pl.loop(1, _NT)(later_tile)

    best = top_v[...]
    bidx = arg_v[0] + jax.lax.broadcasted_iota(_I32, (8, 128), 0)
    rmax = jnp.max(best, axis=0, keepdims=True)
    idx = jnp.min(jnp.where(best == rmax, bidx, _S - 1))
    r_sel = jax.nn.sigmoid(rmax)
    tsel = idx // _T
    rsel = idx - tsel * _T
    grp = _bf(x_v[tsel, pl.ds(pl.multiple_of((rsel >> 4) << 3, 8), 8), :]).astype(_F32)
    hit = jax.lax.broadcasted_iota(_I32, (16, _D), 0) == (rsel & 15)
    xc_v[...] = _col_bcast(jnp.sum(jnp.where(hit, grp, 0.0), axis=0, keepdims=True))

    cp_w(0).wait()
    fold(0, lq_v)
    rows = jax.lax.broadcasted_iota(_I32, (64, 128), 0)
    cols = jax.lax.broadcasted_iota(_I32, (64, 128), 1)
    same_head = (rows >> 5) == ((cols >> 1) & 1)
    for p in range(_NP):
        kvm_v[p] = pltpu.bitcast(jnp.where(same_head, kv_v[p], 0.0).astype(_BF), _I32)
        z_v[p] = jnp.broadcast_to(jnp.sum(z_v[p], axis=1, keepdims=True), (128, 128))

    def phase2(i):
        ti = (tsel + 1 + i) % _NT
        for cp in cp_ffn(i):
            cp.wait()
        zero = i >> 8
        pq, po, ot = {}, {}, {}

        def qprod(m, t, zeros):
            pq[m - 1, t] = _dg(_bf(_paced(lq_v[m - 1], zeros)), _bf(tok_words(ti, m - 1)[64 * t:64 * t + 64, :]), 1, 1)

        def attn(blk, t, zeros):
            for p in range(8):
                a_v[blk][t][64 * p:64 * p + 64, :] = _dg(
                    _bf(kvm_v[8 * (blk // 2) + p]), _bf(_paced(phi_v[blk][2 * p + t + zero], zeros[p::8])), 1, 0)

        def oprod(m, c, zeros):
            if m not in ot:
                at = []
                for t in range(2):
                    blk = [a_v[b][t][pl.ds(pl.multiple_of(zero, 8), _HD), :] for b in (0, 2, 1, 3)]
                    at.append((*blk, *_a_sums(*blk))[_A_SLOT[m - 1]].astype(_BF).T)
                ot[m] = jnp.concatenate(at, axis=0)
            k = _B_SLOT[m - 1]
            w = lo_v[256 * k:256 * k + 256, 128 * c:128 * c + 128]
            po[m - 1, c] = _dg(ot[m], _bf(jnp.concatenate([_paced(w[0:64], zeros), w[64:]], axis=0)), 1, 0)

        def feat_piece(blk, t, p):
            def run():
                ep, en, ip, iq = _dual_exp(_mix(blk, lambda m: pq[m, t][64 * p:64 * p + 64]))
                z = z_v[8 * (blk // 2) + p]
                inv = _recip(_pair_reduce(ep * z[0:64], jnp.add) * ip
                             + _pair_reduce(en * z[64:128], jnp.add) * iq + 1e-6)
                phi_v[blk][2 * p + t] = _join(ep * _rep8(ip * inv), en * _rep8(iq * inv))
                return phi_v[blk][16 + zero, 0:8, :]
            return run

        def hidden_piece(c, half):
            def run():
                for k, w in enumerate((wg_v, wu_v)):
                    acc = f_v[2 * c + k + zero] if half else None
                    f_v[2 * c + k] = _matvec(w.at[i], xc_v, c, 32 * half, 32 * half + 32, acc)
                return pltpu.bitcast(f_v[22 + zero], _I32)
            return run

        def act_piece(c):
            def run():
                hg, hu = (jnp.sum(f_v[2 * c + k + zero], axis=0, keepdims=True) for k in range(2))
                hc_v[128 * c:128 * c + 128, :] = _col_bcast(hg * jax.nn.sigmoid(hg) * hu)
            return run

        def down_piece(c, half):
            def run():
                for cc in (c, c + 1):
                    f_v[14 + cc] = _matvec(wd_v.at[i], hc_v, cc, 28 * half, 28 * half + 28, f_v[14 + cc + zero])
                return pltpu.bitcast(f_v[22 + zero], _I32)
            return run

        def emit_piece(blk, u, c):
            def run():
                h, d = blk // 2, blk % 2
                g = g_v[4 * ti + 2 * h + u]
                tok = jax.lax.broadcasted_iota(_I32, (128, 128), 0) + (ti * _T + _HT * h + 128 * u)
                o = []
                for cc in (c, c + 1):
                    y = jnp.sum(f_v[14 + 4 * d + cc + zero], axis=0, keepdims=True) * r_sel
                    b = _bf(x_blk(ti, 2 * d + h)[64 * u:64 * u + 64, 128 * cc:128 * cc + 128]).astype(_F32)
                    b = b + jnp.where(tok == idx, y, 0.0)
                    o.append(g * _mix(blk, lambda m: po[m, cc][128 * u:128 * u + 128]) + (1.0 - g) * b)
                r0, c0 = _HT * h + 128 * u, _HD * d + 128 * c
                out_v[ti, r0:r0 + 128, c0:c0 + 256] = jnp.concatenate(o, axis=1).astype(_BF)
                return pltpu.bitcast(out_v[_NT + zero, 0:16, 0:128], _I32)
            return run

        def pieces(name):
            if name == "h":
                return [hidden_piece(c, half) for c in range(_FC // 128) for half in range(2)]
            if name == "a":
                return [act_piece(c) for c in range(_FC // 128)]
            if name == "d":
                return [down_piece(c, half) for c in (4, 6, 0, 2) for half in range(2)]
            if name[0] == "e":
                return [emit_piece(int(name[1]), u, c) for c in (0, 2) for u in range(2)]
            return [feat_piece(int(name[1]), t, p) for t in ([int(name[2])] if name[2:] else range(2))
                    for p in range(8)]

        _play(_PHASE2, {"q": (qprod, 2), "o": (oprod, 4), "g": (attn, 2)}, pieces)
        cp_o(i, ti).start()

    pl.loop(0, _NT)(phase2)
    for i in range(_NT):
        cp_o(i, i).wait()


@jax.jit
def pallas_gated_mix__linear_kernel_hedgehog__moe_arch_mod__prompt_kernel(
    A_x: jax.Array,
    A_wqkv: jax.Array,
    A_w_phi: jax.Array,
    A_wo: jax.Array,
    B_x: jax.Array,
    B_w_r: jax.Array,
    B_w_gate: jax.Array,
    B_w_up: jax.Array,
    B_w_down: jax.Array,
    gate_w: jax.Array,
):
    del B_x
    hbm = pl.BlockSpec(memory_space=pl.ANY)
    dma = pltpu.SemaphoreType.DMA
    out = pl.pallas_call(
        _kernel,
        out_shape=jax.ShapeDtypeStruct((_S, _D), _BF),
        in_specs=[hbm] * 9,
        out_specs=hbm,
        scratch_shapes=[
            pltpu.VMEM((_NT, _HT, _D), _I32),
            pltpu.VMEM((2, _HD, _D), _I32),
            pltpu.VMEM((_NT, _HD, _FC), _I32),
            pltpu.VMEM((_NT, _HD, _FC), _I32),
            pltpu.VMEM((_NT, _FC // 2, _D), _I32),
            pltpu.VMEM((_H, _DH, _DH), _BF),
            pltpu.VMEM((_D,), _BF),
            pltpu.VMEM((_D,), _BF),
            pltpu.VMEM((64, _D), _I32),
            pltpu.VMEM((7, 256, _HD), _I32),
            pltpu.VMEM((7, 256, _HD), _I32),
            pltpu.VMEM((9 * 256 + 8, _HD), _I32),
            pltpu.VMEM((9 * 256 + 8, _HD), _I32),
            pltpu.VMEM((5 * _NT + 1, 128, _HD), _I32),
            [pltpu.VMEM((17, 64, 128), _I32)] * 4,
            [[pltpu.VMEM((_HD, 128), _F32)] * 2] * 4,
            pltpu.VMEM((_NP, 64, 128), _F32),
            pltpu.VMEM((_NP, 128, 128), _F32),
            pltpu.VMEM((_NP, 32, 128), _I32),
            pltpu.VMEM((_S // 128 + 1, 128, 128), _F32),
            pltpu.VMEM((8, 128), _F32),
            pltpu.VMEM((2, 8, 128), _I32),
            pltpu.VMEM((23, 8, 128), _F32),
            pltpu.VMEM((_D, 128), _F32),
            pltpu.VMEM((_FC, 128), _F32),
            pltpu.VMEM((_NT + 1, _T, _D), _BF),
            dma((_NT,)), dma((2,)), dma((2,)), dma((4,)), dma((3,)),
            dma((_NT,)), dma((_NT,)), dma((_NT,)), dma((_NT,)),
        ],
        compiler_params=pltpu.CompilerParams(vmem_limit_bytes=100 * 1024 * 1024,
                                             disable_bounds_checks=True),
    )(A_x.reshape(_S, _D), A_wqkv, A_w_phi, A_wo, B_w_r, B_w_gate, B_w_up, B_w_down, gate_w)
    return out.reshape(1, _S, _D)
```

```python
import jax
import jax.numpy as jnp
import jax.experimental.pallas as pl
import jax.experimental.pallas.tpu as pltpu

_BF = jnp.bfloat16
_F32 = jnp.float32
_I32 = jnp.int32
_LOG2E = 1.4426950408889634

_S, _D, _H, _DH, _F = 2048, 1024, 32, 32, 3584
_T = 512
_HT = _T // 2
_HD = _D // 2
_NT = _S // _T
_FC = _F // _NT
_NP = _H // 2

_A_SLOT = (4, 5, 0, 3, 6, 7, 8)
_B_SLOT = (4, 0, 5, 6, 3, 7, 8)

_FIRST = ("+r +s ! W0 +a v3:16,16,16,16 v5 W1 +b v4:16,16,16,16 v2 v1 v7 W2 k2 k5 k4 +f2 k3:4,4 +f1 k1:5,5 "
          "k7:5,5 +f0 k6:6,6 +f3 g2:4,4,4,4 v6:2,2,2,2 g1 g0 g3")
_PHASE1 = ("k2:3,2 +r k5:5,5 +o v2:3,3,3,3 v5:7,7,7,7 k4 +f2 +f1 k3:8,8 v4.0:4 +s v4.1:4 v4.2:4 v4.3:2 "
           "v3:2,2,2,2 g2 k7 k1:4,4 +f0 g1 k6:10,12 +f3 v7 v1:5,5,3,5 v6 g0:1,0,0,1 g3:1,1,1,1")
_PHASE2 = ("+h0 +h1 q4.1:2 q4.0:2 q7.1:2 q7.0:3 q1:2,2 q5.0 +f0 q5.1:1 q3:6,6 q2.0:9 +f1 g0 q2.1:9 +f2 "
           "q6:7,7 +f3 g1 o3:3,3,3,3 g2 o6:4,3,3,3 +a ! g3 +d o5:2,2,2,5 +e1 o4:1,1,1,1 o2:1,1,2,1 +e2 "
           "o1:2,0,2,2 +e3 o7:1,1,1,1 +e0 !")


def _dg(a, b, ca, cb):
    return jax.lax.dot_general(a, b, (((ca,), (cb,)), ((), ())), preferred_element_type=_F32)


def _bf(w):
    return pltpu.bitcast(w, _BF)


def _put(ref, g, c, v):
    for j in range(v.shape[1] // 128):
        ref[pl.ds(g, v.shape[0] // 16), c + j] = v[:, 128 * j:128 * j + 128].reshape(-1, 16, 128).astype(_BF)


def _get(ref, k, g, n, tiles=range(4)):
    words = ref.bitcast(_I32)
    return jnp.concatenate([words[k, pl.ds(g, n), c].reshape(8 * n, 128) for c in tiles], axis=1)


def _a_sums(a11, a12, a21, a22):
    return (a11 + a22, a21 + a22, a11 + a12, a21 - a11, a12 - a22)


def _b_sums(b11, b12, b21, b22):
    return (b11 + b22, b12 - b22, b21 - b11, b11 + b12, b21 + b22)


def _mix(c, m):
    if c == 0:
        return m(0) + m(3) - m(4) + m(6)
    if c == 1:
        return m(2) + m(4)
    if c == 2:
        return m(1) + m(3)
    return m(0) - m(1) + m(2) + m(5)


def _sum_piece(src, dst, sums, g, c, which=range(5)):
    r = 8 * g if isinstance(g, int) else pl.multiple_of(8 * g, 8)
    out = sums(*[0.0 if b is None else _bf(b[pl.ds(r, 8), 128 * c:128 * c + 256]).astype(_F32) for b in src])
    for k in which:
        _put(dst[k], g, c, out[k])


def _paced(w, zeros):
    if not zeros:
        return w
    groups = w.shape[0] // 8
    first = [w[8 * g:8 * g + 8, 0:128] for g in range(groups)]
    for j, z in enumerate(zeros):
        g = max((j + 1) * groups // len(zeros) - 1, 0)
        first[g] = first[g] | z
    first = jnp.concatenate(first, axis=0)
    return first if w.shape[1] == 128 else jnp.concatenate([first, w[:, 128:]], axis=1)


def _play(program, steps, pieces):
    queue = []
    for word in program.split():
        if word == "!":
            while queue:
                queue.pop(0)()
        elif word[0] == "+":
            queue.extend(pieces(word[1:]))
        else:
            name, _, counts = word.partition(":")
            name, _, tile = name.partition(".")
            step, tiles = steps[name[0]]
            tiles = [int(tile)] if tile else range(tiles)
            counts = [int(n) for n in counts.split(",")] if counts else [0] * len(tiles)
            for t, n in zip(tiles, counts):
                step(int(name[1:]), t, [queue.pop(0)() for _ in range(min(n, len(queue)))])
    assert not queue


def _recip(v):
    r = pl.reciprocal(v, approx=True)
    return r * (2.0 - v * r)


def _pair_reduce(v, op):
    r = v[0:8]
    for j in range(1, 8):
        r = op(r, v[8 * j:8 * j + 8])
    r = op(r, pltpu.roll(r, 2, 0))
    return op(r, pltpu.roll(r, 4, 0))


def _rep8(v):
    return jnp.concatenate([v] * 8, axis=0)


def _dual_exp(p):
    ep = jnp.exp2(p - _rep8(_pair_reduce(p, jnp.maximum)))
    en = jnp.exp2(_rep8(_pair_reduce(p, jnp.minimum)) - p)
    return ep, en, _pair_reduce(ep, jnp.add), _pair_reduce(en, jnp.add)


def _col_bcast(row):
    return jnp.broadcast_to(row, (128, row.shape[1])).T


def _matvec(w_ref, col_ref, c, j0, j1, acc=None):
    for j in range(j0, j1):
        t = _bf(w_ref[8 * j:8 * j + 8, 128 * c:128 * c + 128]).astype(_F32) * col_ref[16 * j:16 * j + 16, :]
        acc = t[0:8] if acc is None else acc + t[0:8]
        acc = acc + t[8:16]
    return acc


def _kernel(x_hbm, wqkv_hbm, wphi_hbm, wo_hbm, wr_hbm, wg_hbm, wu_hbm, wd_hbm, gw_hbm,
            out_hbm,
            x_v, w_v, wg_v, wu_v, wd_v, wphi_v, wr_v, gw_v,
            wv_v, wo_v, lm_v, lk_v, lq_v, lv_v, lo_v, r_v, phi_v, a_v, kv_v, z_v, kvm_v, g_v, top_v, arg_v,
            f_v, xc_v, hc_v, out_v,
            sem_x, sem_w, sem_v, sem_wo, sem_s, sem_g, sem_u, sem_d, sem_o):
    x_hbm, wqkv_hbm, wo_hbm, wg_hbm, wu_hbm, wd_hbm = (
        r.bitcast(_I32) for r in (x_hbm, wqkv_hbm, wo_hbm, wg_hbm, wu_hbm, wd_hbm))

    def cp_x(i):
        return pltpu.make_async_copy(x_hbm.at[pl.ds(i * _HT, _HT)], x_v.at[i], sem_x.at[i])

    def cp_w(j):
        return pltpu.make_async_copy(wqkv_hbm.at[:, pl.ds(j * _D, _D)], w_v.at[j], sem_w.at[j])

    def cp_v(k):
        return pltpu.make_async_copy(wqkv_hbm.at[pl.ds(256 * (k % 2), 256), pl.ds(2 * _D + _HD * (k // 2), _HD)],
                                     wv_v.at[k], sem_v.at[k])

    def cp_wo(k):
        return pltpu.make_async_copy(wo_hbm.at[pl.ds(256 * (k // 2), 256), pl.ds(_HD * (k % 2), _HD)],
                                     wo_v.at[k], sem_wo.at[k])

    cp_small = [pltpu.make_async_copy(src, dst, sem_s.at[j]) for j, (src, dst) in enumerate(
        ((wphi_hbm, wphi_v), (wr_hbm, wr_v), (gw_hbm, gw_v)))]

    def cp_ffn(i):
        cols = pl.ds(i * _FC, _FC)
        return (pltpu.make_async_copy(wg_hbm.at[:, cols], wg_v.at[i], sem_g.at[i]),
                pltpu.make_async_copy(wu_hbm.at[:, cols], wu_v.at[i], sem_u.at[i]),
                pltpu.make_async_copy(wd_hbm.at[pl.ds(i * (_FC // 2), _FC // 2)], wd_v.at[i], sem_d.at[i]))

    def cp_o(t, blk):
        return pltpu.make_async_copy(
            out_v[blk].at[t], out_hbm.at[pl.ds(t * _T + _HT * (blk // 2), _HT), pl.ds(_HD * (blk % 2), _HD)],
            sem_o.at[4 * t + blk])

    for cp in cp_small:
        cp.start()
    cp_x(0).start()
    cp_v(0).start()
    cp_v(1).start()

    kv_v[...] = jnp.zeros_like(kv_v)
    z_v[...] = jnp.zeros_like(z_v)
    f_v[...] = jnp.zeros_like(f_v)
    xc_v[_D:, :] = jnp.zeros((8, 128), _F32)
    top_v[...] = jnp.full((8, 128), -jnp.inf, _F32)
    arg_v[...] = jnp.zeros_like(arg_v)
    g_v[_S // 128, 0:8, :] = jnp.zeros((8, 128), _F32)
    for ref in (r_v, lv_v, lo_v, *phi_v):
        ref[ref.shape[0] - 1, 0, 0] = jnp.zeros((16, 128), _BF)
    for ref in out_v:
        ref[_NT, 0:16, 0:128] = jnp.zeros((16, 128), _BF)

    for cp in cp_small:
        cp.wait()
    rows = jax.lax.broadcasted_iota(_I32, (128, _DH), 0)
    cols = jax.lax.broadcasted_iota(_I32, (128, _DH), 1)
    sel = jnp.where(((rows >> 1) & 31) == cols, 1.0, 0.0).astype(_BF)
    full = _dg(sel, wphi_v[...].reshape(_H * _DH, _DH), 1, 1)
    rows = jax.lax.broadcasted_iota(_I32, (128, _D), 0)
    cols = jax.lax.broadcasted_iota(_I32, (128, _D), 1)
    keep = ((cols >> 5) & 3) == 2 * (rows >> 6) + (rows & 1)
    _put(lm_v.at[0], 0, 0, jnp.where(keep, full, 0.0))

    def fold(j, l_v, queue=()):
        for g in range(4):
            for d in range(2):
                blk = []
                for gg in (g, g + 4):
                    c = slice(128 * gg, 128 * gg + 128)
                    for dd in (d, d + 2):
                        w = _paced(w_v[j, 128 * dd:128 * dd + 128, c], [queue.pop(0)() for _ in queue[:1]])
                        blk.append(_dg(_bf(_get(lm_v, 0, 0, 8, [gg])), _bf(w), 1, 1) * _LOG2E)
                blk += _a_sums(*blk)
                for m in range(7):
                    _put(l_v.at[m], 8 * g, 2 * d, blk[_A_SLOT[m]])

    def weight_piece(blocks, ref, sums, g, c, zero, have=range(4), which=range(5)):
        def run():
            _sum_piece([blocks.at[k] if k in have else None for k in range(4)], [ref.at[k] for k in range(5)],
                       sums, g, c, which)
            return _get(ref, 5 + zero, 0, 1, [0])
        return run

    def weight_words(blocks, ref, k, c):
        return blocks[k, :, 128 * c:128 * c + 128] if k < 4 else _get(ref, k - 4, 0, 32, [c])

    def x_blk(i, k):
        return x_v.at[i, 128 * (k % 2):128 * (k % 2) + 128, _HD * (k // 2):_HD * (k // 2) + _HD]

    def tok_words(i, m, g=0, n=16):
        k = _B_SLOT[m]
        return x_blk(i, k)[8 * g:8 * (g + n), :] if k < 4 else _get(r_v, 5 * i + k - 4, g, n)

    def put_phi(blk, p, t, zero, pos, neg):
        _put(phi_v[blk].at[2 * p + t], 0, 0, jnp.concatenate([pos, neg], axis=0))
        return _get(phi_v[blk], 16 + zero, 0, 1, [0])

    def get_phi(blk, p, t, zero, zeros=()):
        return _bf(_paced(_get(phi_v[blk], 2 * p + t + zero, 0, 8, [0]), zeros))

    def phase1(i, zero, program):
        pk, pv = {}, {}

        def kprod(m, t, zeros):
            pk[m - 1, t] = _dg(_bf(_paced(_get(lk_v, m - 1, 0, 32), zeros)), _bf(tok_words(i, m - 1, 8 * t, 8)), 1, 1)

        def vprod(m, c, zeros):
            pv[m - 1, c] = _dg(_bf(_paced(tok_words(i, m - 1), zeros)),
                               _bf(weight_words(wv_v, lv_v, _A_SLOT[m - 1], c)), 1, 0)

        def kv(blk, c, zeros):
            vt = _mix(blk, lambda m: pv[m, c]).astype(_BF).T
            for h in range(2):
                p = 2 * c + h
                phi = jnp.concatenate([get_phi(blk, p, 0, zero, zeros[h::2]), get_phi(blk, p, 1, zero)], axis=1)
                kv_v[8 * (blk // 2) + p] += _dg(vt[64 * h:64 * h + 64], phi, 1, 1)

        def wait(j, t, zeros):
            for cp in (cp_v(2 * j), cp_v(2 * j + 1)) if j < 2 else (cp_w(1),):
                cp.wait()
            if j == 0:
                cp_w(1).start()
            elif j == 1:
                cp_x(1).start()
                for k in range(4):
                    cp_wo(k).start()
            else:
                for k in range(2, _NT):
                    cp_x(k).start()
                cp_w(0).start()
                for k in range(_NT):
                    for cp in cp_ffn(k):
                        cp.start()
                fold(1, lk_v)

        def sum_piece(j):
            def run():
                _sum_piece([x_blk(i, k) for k in range(4)], [r_v.at[5 * i + k + zero] for k in range(5)],
                           _b_sums, j // 2, 2 * (j % 2))
                return _get(r_v, 5 * _NT, 0, 1, [0])
            return run

        def feat_piece(blk, t, p):
            def run():
                ep, en, sp, sn = _dual_exp(_mix(blk, lambda m: pk[m, t][64 * p:64 * p + 64]))
                ep, en = ep * _rep8(_recip(sp)), en * _rep8(_recip(sn))
                z_v[8 * (blk // 2) + p] += jnp.concatenate([ep, en], axis=0)
                return put_phi(blk, p, t, zero, ep, en)
            return run

        def score_piece(c):
            def run():
                xh = _bf(x_v[i, 16 * c:16 * c + 16, :]).astype(_F32)
                wr = wr_v[...].astype(_F32).reshape(1, _D)
                gw = gw_v[...].astype(_F32).reshape(1, _D)
                g = jax.nn.sigmoid(jnp.sum(xh * gw, axis=1, keepdims=True))
                g_v[4 * i + c // 4, 32 * (c % 4):32 * (c % 4) + 32, :] = jnp.broadcast_to(g, (32, 128))
                sc = jnp.sum(xh * wr, axis=1, keepdims=True).astype(_BF).astype(_F32)
                best, bidx = top_v[...], arg_v[0]
                for j in range(4):
                    rj = sc[8 * j:8 * j + 8]
                    upd = rj > best
                    best = jnp.where(upd, rj, best)
                    bidx = jnp.where(upd, i * _T + 32 * c + 8 * j, bidx)
                top_v[...] = best
                arg_v[0] = bidx
                return arg_v[1 + zero] | pltpu.bitcast(g_v[_S // 128 + zero, 0:8, :], _I32)
            return run

        def pieces(name):
            if name == "r":
                return [sum_piece(j) for j in range(32)]
            if name == "s":
                return [score_piece(c) for c in range(16)]
            if name in "ab":
                part = ((0, 1), [2]) if name == "a" else (range(4), (0, 1, 3, 4))
                return [weight_piece(wv_v, lv_v, _a_sums, j // 2, 2 * (j % 2), zero, *part) for j in range(64)]
            if name == "o":
                start = jnp.minimum(11 * (i - 1), 32 - 11)
                return [weight_piece(wo_v, lo_v, _b_sums, start + j // 2, 2 * (j % 2), 0) for j in range(22)]
            return [feat_piece(int(name[1]), t, p) for t in ([int(name[2])] if name[2:] else range(2))
                    for p in range(8)]

        _play(program, {"k": (kprod, 2), "v": (vprod, 4), "g": (kv, 4), "W": (wait, 1)}, pieces)

    def later_tile(i):
        cp_x(i).wait()
        phase1(i, i >> 8, _PHASE1)

    zero = arg_v[1, 0, 0]
    cp_x(0).wait()
    cp_v(2).start()
    cp_v(3).start()
    phase1(0, zero, _FIRST)
    for k in range(4):
        cp_wo(k).wait()
    pl.loop(1, _NT)(later_tile)

    best = top_v[...]
    bidx = arg_v[0] + jax.lax.broadcasted_iota(_I32, (8, 128), 0)
    rmax = jnp.max(best, axis=0, keepdims=True)
    idx = jnp.min(jnp.where(best == rmax, bidx, _S - 1))
    r_sel = jax.nn.sigmoid(rmax)
    tsel = idx // _T
    rsel = idx - tsel * _T
    grp = _bf(x_v[tsel, pl.ds(pl.multiple_of((rsel >> 4) << 3, 8), 8), :]).astype(_F32)
    hit = jax.lax.broadcasted_iota(_I32, (16, _D), 0) == (rsel & 15)
    x_sel = jnp.sum(jnp.where(hit, grp, 0.0), axis=0, keepdims=True)

    def state_piece(p):
        def run():
            rows = jax.lax.broadcasted_iota(_I32, (64, 128), 0)
            cols = jax.lax.broadcasted_iota(_I32, (64, 128), 1)
            _put(kvm_v.at[p], 0, 0, jnp.where((rows >> 5) == (cols & 1), kv_v[p], 0.0))
            z_v[p] = jnp.broadcast_to(jnp.sum(z_v[p], axis=1, keepdims=True), (128, 128))
            return pltpu.bitcast(z_v[_NP + zero, 0:8, :], _I32)
        return run

    def column_piece(c):
        def run():
            xc_v[128 * c:128 * c + 128, :] = _col_bcast(x_sel[:, 128 * c:128 * c + 128])
            return pltpu.bitcast(xc_v[pl.ds(pl.multiple_of(_D + zero, 8), 8), :], _I32)
        return run

    cp_w(0).wait()
    fold(0, lq_v, [state_piece(p) for p in range(_NP)] + [column_piece(c) for c in range(8)])

    def phase2(i):
        ti = (tsel + 1 + i) % _NT
        for cp in cp_ffn(i):
            cp.wait()
        zero = i >> 8
        pq, po, ot = {}, {}, {}

        def qprod(m, t, zeros):
            pq[m - 1, t] = _dg(_bf(_paced(_get(lq_v, m - 1, 0, 32), zeros)), _bf(tok_words(ti, m - 1, 8 * t, 8)), 1, 1)

        def attn(blk, t, zeros):
            for p in range(8):
                a_v[blk][t][64 * p:64 * p + 64, :] = _dg(
                    _bf(_get(kvm_v, 8 * (blk // 2) + p, 0, 4, [0])), get_phi(blk, p, t, zero, zeros[p::8]), 1, 0)

        def oprod(m, c, zeros):
            if m not in ot:
                at = []
                for t in range(2):
                    blk = [a_v[b][t][pl.ds(pl.multiple_of(zero, 8), _HD), :] for b in (0, 2, 1, 3)]
                    at.append((*blk, *_a_sums(*blk))[_A_SLOT[m - 1]].astype(_BF).T)
                ot[m] = jnp.concatenate(at, axis=0)
            w = weight_words(wo_v, lo_v, _B_SLOT[m - 1], c)
            po[m - 1, c] = _dg(ot[m], _bf(jnp.concatenate([_paced(w[0:64], zeros), w[64:]], axis=0)), 1, 0)

        def feat_piece(blk, t, p):
            def run():
                ep, en, sp, sn = _dual_exp(_mix(blk, lambda m: pq[m, t][64 * p:64 * p + 64]))
                z = z_v[8 * (blk // 2) + p]
                dp, dn = _pair_reduce(ep * z[0:64], jnp.add), _pair_reduce(en * z[64:128], jnp.add)
                inv = _recip(dp * sn + sp * (dn + 1e-6 * sn))
                return put_phi(blk, p, t, zero, ep * _rep8(sn * inv), en * _rep8(sp * inv))
            return run

        def hidden_piece(c, half):
            def run():
                for k, w in enumerate((wg_v, wu_v)):
                    acc = f_v[2 * c + k + zero] if half else None
                    f_v[2 * c + k] = _matvec(w.at[i], xc_v, c, 32 * half, 32 * half + 32, acc)
                return pltpu.bitcast(f_v[22 + zero], _I32)
            return run

        def act_piece(c):
            def run():
                hg, hu = (jnp.sum(f_v[2 * c + k + zero], axis=0, keepdims=True) for k in range(2))
                hc_v[128 * c:128 * c + 128, :] = _col_bcast(hg * jax.nn.sigmoid(hg) * hu)
            return run

        def down_piece(c, half):
            def run():
                for cc in (c, c + 1):
                    f_v[14 + cc] = _matvec(wd_v.at[i], hc_v, cc, 28 * half, 28 * half + 28, f_v[14 + cc + zero])
                return pltpu.bitcast(f_v[22 + zero], _I32)
            return run

        def emit_piece(blk, u, c):
            def run():
                h, d = blk // 2, blk % 2
                g = g_v[4 * ti + 2 * h + u]
                tok = jax.lax.broadcasted_iota(_I32, (128, 128), 0) + (ti * _T + _HT * h + 128 * u)
                o = []
                for cc in (c, c + 1):
                    y = jnp.sum(f_v[14 + 4 * d + cc + zero], axis=0, keepdims=True) * r_sel
                    b = _bf(x_blk(ti, 2 * d + h)[64 * u:64 * u + 64, 128 * cc:128 * cc + 128]).astype(_F32)
                    b = b + jnp.where(tok == idx, y, 0.0)
                    o.append(g * _mix(blk, lambda m: po[m, cc][128 * u:128 * u + 128]) + (1.0 - g) * b)
                out_v[blk][ti, 128 * u:128 * u + 128, 128 * c:128 * c + 256] = jnp.concatenate(o, axis=1).astype(_BF)
                if (u, c) == (1, 2):
                    cp_o(ti, blk).start()
                    out_v[blk][_NT, 16:32, 0:128] = jnp.zeros((16, 128), _BF)
                return pltpu.bitcast(out_v[blk][_NT + zero, 0:16, 0:128], _I32)
            return run

        def pieces(name):
            if name[0] == "h":
                return [hidden_piece(c, int(name[1])) for c in range(_FC // 128)]
            if name == "a":
                return [act_piece(c) for c in range(_FC // 128)]
            if name == "d":
                return [down_piece(c, half) for c in (4, 6, 0, 2) for half in range(2)]
            if name[0] == "e":
                return [emit_piece(int(name[1]), u, c) for c in (0, 2) for u in range(2)]
            return [feat_piece(int(name[1]), t, p) for t in ([int(name[2])] if name[2:] else range(2))
                    for p in range(8)]

        _play(_PHASE2, {"q": (qprod, 2), "o": (oprod, 4), "g": (attn, 2)}, pieces)

    pl.loop(0, _NT)(phase2)
    for t in range(_NT):
        for blk in range(4):
            cp_o(t, blk).wait()


@jax.jit
def pallas_gated_mix__linear_kernel_hedgehog__moe_arch_mod__prompt_kernel(
    A_x: jax.Array,
    A_wqkv: jax.Array,
    A_w_phi: jax.Array,
    A_wo: jax.Array,
    B_x: jax.Array,
    B_w_r: jax.Array,
    B_w_gate: jax.Array,
    B_w_up: jax.Array,
    B_w_down: jax.Array,
    gate_w: jax.Array,
):
    del B_x
    hbm = pl.BlockSpec(memory_space=pl.ANY)
    dma = pltpu.SemaphoreType.DMA
    out = pl.pallas_call(
        _kernel,
        out_shape=jax.ShapeDtypeStruct((_S, _D), _BF),
        in_specs=[hbm] * 9,
        out_specs=hbm,
        scratch_shapes=[
            pltpu.VMEM((_NT, _HT, _D), _I32),
            pltpu.VMEM((2, _HD, _D), _I32),
            pltpu.VMEM((_NT, _HD, _FC), _I32),
            pltpu.VMEM((_NT, _HD, _FC), _I32),
            pltpu.VMEM((_NT, _FC // 2, _D), _I32),
            pltpu.VMEM((_H, _DH, _DH), _BF),
            pltpu.VMEM((_D,), _BF),
            pltpu.VMEM((_D,), _BF),
            pltpu.VMEM((4, 256, _HD), _I32),
            pltpu.VMEM((4, 256, _HD), _I32),
            pltpu.VMEM((1, 8, 8, 16, 128), _BF),
            pltpu.VMEM((7, 32, 4, 16, 128), _BF),
            pltpu.VMEM((7, 32, 4, 16, 128), _BF),
            pltpu.VMEM((6, 32, 4, 16, 128), _BF),
            pltpu.VMEM((6, 32, 4, 16, 128), _BF),
            pltpu.VMEM((5 * _NT + 1, 16, 4, 16, 128), _BF),
            [pltpu.VMEM((17, 8, 1, 16, 128), _BF)] * 4,
            [[pltpu.VMEM((_HD, 128), _F32)] * 2] * 4,
            pltpu.VMEM((_NP, 64, 128), _F32),
            pltpu.VMEM((_NP + 1, 128, 128), _F32),
            pltpu.VMEM((_NP, 4, 1, 16, 128), _BF),
            pltpu.VMEM((_S // 128 + 1, 128, 128), _F32),
            pltpu.VMEM((8, 128), _F32),
            pltpu.VMEM((2, 8, 128), _I32),
            pltpu.VMEM((23, 8, 128), _F32),
            pltpu.VMEM((_D + 8, 128), _F32),
            pltpu.VMEM((_FC, 128), _F32),
            [pltpu.VMEM((_NT + 1, _HT, _HD), _BF)] * 4,
            dma((_NT,)), dma((2,)), dma((2,)), dma((4,)), dma((3,)),
            dma((_NT,)), dma((_NT,)), dma((_NT,)), dma((4 * _NT,)),
        ],
        compiler_params=pltpu.CompilerParams(vmem_limit_bytes=100 * 1024 * 1024,
                                             disable_bounds_checks=True),
    )(A_x.reshape(_S, _D), A_wqkv, A_w_phi, A_wo, B_w_r, B_w_gate, B_w_up, B_w_down, gate_w)
    return out.reshape(1, _S, _D)
```

```python
import jax
import jax.numpy as jnp
import jax.experimental.pallas as pl
import jax.experimental.pallas.tpu as pltpu

_BF = jnp.bfloat16
_F32 = jnp.float32
_I32 = jnp.int32
_LOG2E = 1.4426950408889634

_S, _D, _H, _DH, _F = 2048, 1024, 32, 32, 3584
_T = 512
_HT = _T // 2
_HD = _D // 2
_NT = _S // _T
_FC = _F // _NT
_NP = _H // 2

_A_SLOT = (4, 5, 0, 3, 6, 7, 8)
_B_SLOT = (4, 0, 5, 6, 3, 7, 8)

_FIRST = ("+r +s ! W0 +a v3:16,16,16,16 v5 W1 +b v4:16,16,16,16 v2 v1 v7 W2 k2 k5 k4 +f2 k3:4,4 +f1 k1:5,5 "
          "k7:5,5 +f0 k6:6,6 +f3 g2:4,4,4,4 v6:2,2,2,2 g1 g0 g3")
_PHASE1 = ("k2.1:2 k2.0:3 +r k5:5,5 +o v2:3,3,3,3 v5:7,7,7,7 k4 +f2 +f1 k3:8,8 +s v4.3:2 v4.0:4 v4.1:4 "
           "v4.2:4 v3:2,2,2,1 g2 k7 k1:6,4 +f0 g1.1 g1.0 g1.2 g1.3 k6:10,12 +f3 v7 v1:5,5,3,5 v6 g0:1,0,0,1 "
           "g3:1,1,2,1")
_PHASE2 = ("+h0 +h1 q4.1:2 q4.0:4 q7.1:1 q1:1,2 q7.0:3 q5.0 +f0 q5.1:2 q3:7,6 q2.0:9 g0 +f1 q2.1:9 +f2 "
           "q6:6,6 +f3 +a g1 o3:2,3,3,3 ! g2 o6:4,3,3,3 g3 +d o5:2,2,2,4 +e1 o1.0:2 o2:1,1,1,1 o4:2,2,2,2 "
           "+e2 o1.2:1 o1.1 o1.3:2 +e3 o7:0,1,3,1 +e0 !")


def _dg(a, b, ca, cb):
    return jax.lax.dot_general(a, b, (((ca,), (cb,)), ((), ())), preferred_element_type=_F32)


def _bf(w):
    return pltpu.bitcast(w, _BF)


def _put(ref, g, c, v):
    for j in range(v.shape[1] // 128):
        ref[pl.ds(g, v.shape[0] // 16), c + j] = v[:, 128 * j:128 * j + 128].reshape(-1, 16, 128).astype(_BF)


def _get(ref, k, g, n, tiles=range(4)):
    words = ref.bitcast(_I32)
    return jnp.concatenate([words[k, pl.ds(g, n), c].reshape(8 * n, 128) for c in tiles], axis=1)


def _a_sums(a11, a12, a21, a22):
    return (a11 + a22, a21 + a22, a11 + a12, a21 - a11, a12 - a22)


def _b_sums(b11, b12, b21, b22):
    return (b11 + b22, b12 - b22, b21 - b11, b11 + b12, b21 + b22)


def _mix(c, m):
    if c == 0:
        return m(0) + m(3) - m(4) + m(6)
    if c == 1:
        return m(2) + m(4)
    if c == 2:
        return m(1) + m(3)
    return m(0) - m(1) + m(2) + m(5)


def _sum_piece(src, dst, sums, g, c, which=range(5)):
    r = 8 * g if isinstance(g, int) else pl.multiple_of(8 * g, 8)
    out = sums(*[0.0 if b is None else _bf(b[pl.ds(r, 8), 128 * c:128 * c + 256]).astype(_F32) for b in src])
    for k in which:
        _put(dst[k], g, c, out[k])


def _paced(w, zeros):
    if not zeros:
        return w
    groups = w.shape[0] // 8
    first = [w[8 * g:8 * g + 8, 0:128] for g in range(groups)]
    for j, z in enumerate(zeros):
        g = max((j + 1) * groups // len(zeros) - 1, 0)
        first[g] = first[g] | z
    first = jnp.concatenate(first, axis=0)
    return first if w.shape[1] == 128 else jnp.concatenate([first, w[:, 128:]], axis=1)


def _play(program, steps, pieces):
    queue = []
    for word in program.split():
        if word == "!":
            while queue:
                queue.pop(0)()
        elif word[0] == "+":
            queue.extend(pieces(word[1:]))
        else:
            name, _, counts = word.partition(":")
            name, _, tile = name.partition(".")
            step, tiles = steps[name[0]]
            tiles = [int(tile)] if tile else range(tiles)
            counts = [int(n) for n in counts.split(",")] if counts else [0] * len(tiles)
            for t, n in zip(tiles, counts):
                step(int(name[1:]), t, [queue.pop(0)() for _ in range(min(n, len(queue)))])
    assert not queue


def _recip(v):
    r = pl.reciprocal(v, approx=True)
    return r * (2.0 - v * r)


def _pair_reduce(v, op):
    r = v[0:8]
    for j in range(1, 8):
        r = op(r, v[8 * j:8 * j + 8])
    r = op(r, pltpu.roll(r, 2, 0))
    return op(r, pltpu.roll(r, 4, 0))


def _rep8(v):
    return jnp.concatenate([v] * 8, axis=0)


def _dual_exp(p):
    ep = jnp.exp2(p - _rep8(_pair_reduce(p, jnp.maximum)))
    en = jnp.exp2(_rep8(_pair_reduce(p, jnp.minimum)) - p)
    return ep, en, _pair_reduce(ep, jnp.add), _pair_reduce(en, jnp.add)


def _col_bcast(row):
    return jnp.broadcast_to(row, (128, row.shape[1])).T


def _matvec(w_ref, col_ref, c, j0, j1, acc=None):
    for j in range(j0, j1):
        t = _bf(w_ref[8 * j:8 * j + 8, 128 * c:128 * c + 128]).astype(_F32) * col_ref[16 * j:16 * j + 16, :]
        acc = t[0:8] if acc is None else acc + t[0:8]
        acc = acc + t[8:16]
    return acc


def _kernel(x_hbm, wqkv_hbm, wphi_hbm, wo_hbm, wr_hbm, wg_hbm, wu_hbm, wd_hbm, gw_hbm,
            out_hbm,
            x_v, w_v, wg_v, wu_v, wd_v, wphi_v, wr_v, gw_v,
            wv_v, wo_v, lm_v, lk_v, lq_v, lv_v, lo_v, r_v, phi_v, a_v, kv_v, z_v, kvm_v, g_v, top_v, arg_v,
            f_v, xc_v, hc_v, out_v,
            sem_x, sem_w, sem_v, sem_wo, sem_s, sem_g, sem_u, sem_d, sem_o):
    x_hbm, wqkv_hbm, wo_hbm, wg_hbm, wu_hbm, wd_hbm = (
        r.bitcast(_I32) for r in (x_hbm, wqkv_hbm, wo_hbm, wg_hbm, wu_hbm, wd_hbm))

    def cp_x(i):
        return pltpu.make_async_copy(x_hbm.at[pl.ds(i * _HT, _HT)], x_v.at[i], sem_x.at[i])

    def cp_w(j):
        return pltpu.make_async_copy(wqkv_hbm.at[:, pl.ds(j * _D, _D)], w_v.at[j], sem_w.at[j])

    def cp_v(k):
        return pltpu.make_async_copy(wqkv_hbm.at[pl.ds(256 * (k % 2), 256), pl.ds(2 * _D + _HD * (k // 2), _HD)],
                                     wv_v.at[k], sem_v.at[k])

    def cp_wo(k):
        return pltpu.make_async_copy(wo_hbm.at[pl.ds(256 * (k // 2), 256), pl.ds(_HD * (k % 2), _HD)],
                                     wo_v.at[k], sem_wo.at[k])

    cp_small = [pltpu.make_async_copy(src, dst, sem_s.at[j]) for j, (src, dst) in enumerate(
        ((wphi_hbm, wphi_v), (wr_hbm, wr_v), (gw_hbm, gw_v)))]

    def cp_ffn(i):
        cols = pl.ds(i * _FC, _FC)
        return (pltpu.make_async_copy(wg_hbm.at[:, cols], wg_v.at[i], sem_g.at[i]),
                pltpu.make_async_copy(wu_hbm.at[:, cols], wu_v.at[i], sem_u.at[i]),
                pltpu.make_async_copy(wd_hbm.at[pl.ds(i * (_FC // 2), _FC // 2)], wd_v.at[i], sem_d.at[i]))

    def cp_o(t, blk):
        return pltpu.make_async_copy(
            out_v[blk].at[t], out_hbm.at[pl.ds(t * _T + _HT * (blk // 2), _HT), pl.ds(_HD * (blk % 2), _HD)],
            sem_o.at[4 * t + blk])

    for cp in cp_small:
        cp.start()
    cp_x(0).start()
    cp_v(0).start()
    cp_v(1).start()

    kv_v[...] = jnp.zeros_like(kv_v)
    z_v[...] = jnp.zeros_like(z_v)
    f_v[...] = jnp.zeros_like(f_v)
    xc_v[_D:, :] = jnp.zeros((8, 128), _F32)
    top_v[...] = jnp.full((8, 128), -jnp.inf, _F32)
    arg_v[...] = jnp.zeros_like(arg_v)
    g_v[_S // 128, 0:8, :] = jnp.zeros((8, 128), _F32)
    for ref in (r_v, lv_v, lo_v, *phi_v):
        ref[ref.shape[0] - 1, 0, 0] = jnp.zeros((16, 128), _BF)
    for ref in out_v:
        ref[_NT, 0:16, 0:128] = jnp.zeros((16, 128), _BF)

    for cp in cp_small:
        cp.wait()
    rows = jax.lax.broadcasted_iota(_I32, (128, _DH), 0)
    cols = jax.lax.broadcasted_iota(_I32, (128, _DH), 1)
    sel = jnp.where(((rows >> 1) & 31) == cols, 1.0, 0.0).astype(_BF)
    full = _dg(sel, wphi_v[...].reshape(_H * _DH, _DH), 1, 1)
    rows = jax.lax.broadcasted_iota(_I32, (128, _D), 0)
    cols = jax.lax.broadcasted_iota(_I32, (128, _D), 1)
    keep = ((cols >> 5) & 3) == 2 * (rows >> 6) + (rows & 1)
    _put(lm_v.at[0], 0, 0, jnp.where(keep, full, 0.0))

    def fold(j, l_v, queue=()):
        for g in range(4):
            for d in range(2):
                blk = []
                for gg in (g, g + 4):
                    c = slice(128 * gg, 128 * gg + 128)
                    for dd in (d, d + 2):
                        w = _paced(w_v[j, 128 * dd:128 * dd + 128, c], [queue.pop(0)() for _ in queue[:1]])
                        blk.append(_dg(_bf(_get(lm_v, 0, 0, 8, [gg])), _bf(w), 1, 1) * _LOG2E)
                blk += _a_sums(*blk)
                for m in range(7):
                    _put(l_v.at[m], 8 * g, 2 * d, blk[_A_SLOT[m]])

    def weight_piece(blocks, ref, sums, g, c, zero, have=range(4), which=range(5)):
        def run():
            _sum_piece([blocks.at[k] if k in have else None for k in range(4)], [ref.at[k] for k in range(5)],
                       sums, g, c, which)
            return _get(ref, 5 + zero, 0, 1, [0])
        return run

    def weight_words(blocks, ref, k, c):
        return blocks[k, :, 128 * c:128 * c + 128] if k < 4 else _get(ref, k - 4, 0, 32, [c])

    def x_blk(i, k):
        return x_v.at[i, 128 * (k % 2):128 * (k % 2) + 128, _HD * (k // 2):_HD * (k // 2) + _HD]

    def tok_words(i, m, g=0, n=16):
        k = _B_SLOT[m]
        return x_blk(i, k)[8 * g:8 * (g + n), :] if k < 4 else _get(r_v, 5 * i + k - 4, g, n)

    def put_phi(blk, p, t, zero, pos, neg):
        _put(phi_v[blk].at[2 * p + t], 0, 0, jnp.concatenate([pos, neg], axis=0))
        return _get(phi_v[blk], 16 + zero, 0, 1, [0])

    def get_phi(blk, p, t, zero, zeros=()):
        return _bf(_paced(_get(phi_v[blk], 2 * p + t + zero, 0, 8, [0]), zeros))

    def phase1(i, zero, program):
        pk, pv = {}, {}

        def kprod(m, t, zeros):
            pk[m - 1, t] = _dg(_bf(_paced(_get(lk_v, m - 1, 0, 32), zeros)), _bf(tok_words(i, m - 1, 8 * t, 8)), 1, 1)

        def vprod(m, c, zeros):
            pv[m - 1, c] = _dg(_bf(_paced(tok_words(i, m - 1), zeros)),
                               _bf(weight_words(wv_v, lv_v, _A_SLOT[m - 1], c)), 1, 0)

        def kv(blk, c, zeros):
            vt = _mix(blk, lambda m: pv[m, c]).astype(_BF).T
            for h in range(2):
                p = 2 * c + h
                phi = jnp.concatenate([get_phi(blk, p, 0, zero, zeros[h::2]), get_phi(blk, p, 1, zero)], axis=1)
                kv_v[8 * (blk // 2) + p] += _dg(vt[64 * h:64 * h + 64], phi, 1, 1)

        def wait(j, t, zeros):
            for cp in (cp_v(2 * j), cp_v(2 * j + 1)) if j < 2 else (cp_w(1),):
                cp.wait()
            if j == 0:
                cp_w(1).start()
            elif j == 1:
                cp_x(1).start()
                for k in range(4):
                    cp_wo(k).start()
            else:
                for k in range(2, _NT):
                    cp_x(k).start()
                cp_w(0).start()
                for k in range(_NT):
                    for cp in cp_ffn(k):
                        cp.start()
                fold(1, lk_v)

        def sum_piece(j):
            def run():
                _sum_piece([x_blk(i, k) for k in range(4)], [r_v.at[5 * i + k + zero] for k in range(5)],
                           _b_sums, j // 2, 2 * (j % 2))
                return _get(r_v, 5 * _NT, 0, 1, [0])
            return run

        def feat_piece(blk, t, p):
            def run():
                ep, en, sp, sn = _dual_exp(_mix(blk, lambda m: pk[m, t][64 * p:64 * p + 64]))
                ep, en = ep * _rep8(_recip(sp)), en * _rep8(_recip(sn))
                z_v[8 * (blk // 2) + p] += jnp.concatenate([ep, en], axis=0)
                return put_phi(blk, p, t, zero, ep, en)
            return run

        def score_piece(c):
            def run():
                xh = _bf(x_v[i, 16 * c:16 * c + 16, :]).astype(_F32)
                wr = wr_v[...].astype(_F32).reshape(1, _D)
                gw = gw_v[...].astype(_F32).reshape(1, _D)
                g = jax.nn.sigmoid(jnp.sum(xh * gw, axis=1, keepdims=True))
                g_v[4 * i + c // 4, 32 * (c % 4):32 * (c % 4) + 32, :] = jnp.broadcast_to(g, (32, 128))
                sc = jnp.sum(xh * wr, axis=1, keepdims=True).astype(_BF).astype(_F32)
                best, bidx = top_v[...], arg_v[0]
                for j in range(4):
                    rj = sc[8 * j:8 * j + 8]
                    upd = rj > best
                    best = jnp.where(upd, rj, best)
                    bidx = jnp.where(upd, i * _T + 32 * c + 8 * j, bidx)
                top_v[...] = best
                arg_v[0] = bidx
                return arg_v[1 + zero] | pltpu.bitcast(g_v[_S // 128 + zero, 0:8, :], _I32)
            return run

        def pieces(name):
            if name == "r":
                return [sum_piece(j) for j in range(32)]
            if name == "s":
                return [score_piece(c) for c in range(16)]
            if name in "ab":
                part = ((0, 1), [2]) if name == "a" else (range(4), (0, 1, 3, 4))
                return [weight_piece(wv_v, lv_v, _a_sums, j // 2, 2 * (j % 2), zero, *part) for j in range(64)]
            if name == "o":
                start = jnp.minimum(11 * (i - 1), 32 - 11)
                return [weight_piece(wo_v, lo_v, _b_sums, start + j // 2, 2 * (j % 2), 0) for j in range(22)]
            return [feat_piece(int(name[1]), t, p) for t in ([int(name[2])] if name[2:] else range(2))
                    for p in range(8)]

        _play(program, {"k": (kprod, 2), "v": (vprod, 4), "g": (kv, 4), "W": (wait, 1)}, pieces)

    def later_tile(i):
        cp_x(i).wait()
        phase1(i, i >> 8, _PHASE1)

    zero = arg_v[1, 0, 0]
    cp_x(0).wait()
    cp_v(2).start()
    cp_v(3).start()
    phase1(0, zero, _FIRST)
    for k in range(4):
        cp_wo(k).wait()
    pl.loop(1, _NT)(later_tile)

    cp_w(0).wait()
    best = top_v[...]
    bidx = arg_v[0] + jax.lax.broadcasted_iota(_I32, (8, 128), 0)
    rmax = jnp.max(best, axis=0, keepdims=True)
    idx = jnp.min(jnp.where(best == rmax, bidx, _S - 1))
    r_sel = jax.nn.sigmoid(rmax)
    tsel = idx // _T
    rsel = idx - tsel * _T
    grp = _bf(x_v[tsel, pl.ds(pl.multiple_of((rsel >> 4) << 3, 8), 8), :]).astype(_F32)
    hit = jax.lax.broadcasted_iota(_I32, (16, _D), 0) == (rsel & 15)
    x_sel = jnp.sum(jnp.where(hit, grp, 0.0), axis=0, keepdims=True)

    def state_piece(p):
        def run():
            rows = jax.lax.broadcasted_iota(_I32, (64, 128), 0)
            cols = jax.lax.broadcasted_iota(_I32, (64, 128), 1)
            _put(kvm_v.at[p], 0, 0, jnp.where((rows >> 5) == (cols & 1), kv_v[p], 0.0))
            z_v[p] = jnp.broadcast_to(jnp.sum(z_v[p], axis=1, keepdims=True), (128, 128))
            return pltpu.bitcast(z_v[_NP + zero, 0:8, :], _I32)
        return run

    def column_piece(c):
        def run():
            xc_v[128 * c:128 * c + 128, :] = _col_bcast(x_sel[:, 128 * c:128 * c + 128])
            return pltpu.bitcast(xc_v[pl.ds(pl.multiple_of(_D + zero, 8), 8), :], _I32)
        return run

    fold(0, lq_v, [state_piece(p) for p in range(_NP)] + [column_piece(c) for c in range(8)])

    def phase2(i):
        ti = (tsel + 1 + i) % _NT
        for cp in cp_ffn(i):
            cp.wait()
        zero = i >> 8
        pq, po, ot = {}, {}, {}

        def qprod(m, t, zeros):
            pq[m - 1, t] = _dg(_bf(_paced(_get(lq_v, m - 1, 0, 32), zeros)), _bf(tok_words(ti, m - 1, 8 * t, 8)), 1, 1)

        def attn(blk, t, zeros):
            for p in range(8):
                a_v[blk][t][64 * p:64 * p + 64, :] = _dg(
                    _bf(_get(kvm_v, 8 * (blk // 2) + p, 0, 4, [0])), get_phi(blk, p, t, zero, zeros[p::8]), 1, 0)

        def oprod(m, c, zeros):
            if m not in ot:
                at = []
                for t in range(2):
                    blk = [a_v[b][t][pl.ds(pl.multiple_of(zero, 8), _HD), :] for b in (0, 2, 1, 3)]
                    at.append((*blk, *_a_sums(*blk))[_A_SLOT[m - 1]].astype(_BF).T)
                ot[m] = jnp.concatenate(at, axis=0)
            w = weight_words(wo_v, lo_v, _B_SLOT[m - 1], c)
            po[m - 1, c] = _dg(ot[m], _bf(jnp.concatenate([_paced(w[0:64], zeros), w[64:]], axis=0)), 1, 0)

        def feat_piece(blk, t, p):
            def run():
                ep, en, sp, sn = _dual_exp(_mix(blk, lambda m: pq[m, t][64 * p:64 * p + 64]))
                z = z_v[8 * (blk // 2) + p]
                dp, dn = _pair_reduce(ep * z[0:64], jnp.add), _pair_reduce(en * z[64:128], jnp.add)
                inv = _recip(dp * sn + sp * (dn + 1e-6 * sn))
                return put_phi(blk, p, t, zero, ep * _rep8(sn * inv), en * _rep8(sp * inv))
            return run

        def hidden_piece(c, half):
            def run():
                for k, w in enumerate((wg_v, wu_v)):
                    acc = f_v[2 * c + k + zero] if half else None
                    f_v[2 * c + k] = _matvec(w.at[i], xc_v, c, 32 * half, 32 * half + 32, acc)
                return pltpu.bitcast(f_v[22 + zero], _I32)
            return run

        def act_piece(c):
            def run():
                hg, hu = (jnp.sum(f_v[2 * c + k + zero], axis=0, keepdims=True) for k in range(2))
                hc_v[128 * c:128 * c + 128, :] = _col_bcast(hg * jax.nn.sigmoid(hg) * hu)
            return run

        def down_piece(c, half):
            def run():
                for cc in (c, c + 1):
                    f_v[14 + cc] = _matvec(wd_v.at[i], hc_v, cc, 28 * half, 28 * half + 28, f_v[14 + cc + zero])
                return pltpu.bitcast(f_v[22 + zero], _I32)
            return run

        def emit_piece(blk, u, c):
            def run():
                h, d = blk // 2, blk % 2
                g = g_v[4 * ti + 2 * h + u]
                tok = jax.lax.broadcasted_iota(_I32, (128, 128), 0) + (ti * _T + _HT * h + 128 * u)
                o = []
                for cc in (c, c + 1):
                    y = jnp.sum(f_v[14 + 4 * d + cc + zero], axis=0, keepdims=True) * r_sel
                    b = _bf(x_blk(ti, 2 * d + h)[64 * u:64 * u + 64, 128 * cc:128 * cc + 128]).astype(_F32)
                    b = b + jnp.where(tok == idx, y, 0.0)
                    o.append(g * _mix(blk, lambda m: po[m, cc][128 * u:128 * u + 128]) + (1.0 - g) * b)
                out_v[blk][ti, 128 * u:128 * u + 128, 128 * c:128 * c + 256] = jnp.concatenate(o, axis=1).astype(_BF)
                if (u, c) == (1, 2):
                    cp_o(ti, blk).start()
                    out_v[blk][_NT, 16:32, 0:128] = jnp.zeros((16, 128), _BF)
                return pltpu.bitcast(out_v[blk][_NT + zero, 0:16, 0:128], _I32)
            return run

        def pieces(name):
            if name[0] == "h":
                return [hidden_piece(c, int(name[1])) for c in range(_FC // 128)]
            if name == "a":
                return [act_piece(c) for c in range(_FC // 128)]
            if name == "d":
                return [down_piece(c, half) for c in (4, 6, 0, 2) for half in range(2)]
            if name[0] == "e":
                return [emit_piece(int(name[1]), u, c) for c in (0, 2) for u in range(2)]
            return [feat_piece(int(name[1]), t, p) for t in ([int(name[2])] if name[2:] else range(2))
                    for p in range(8)]

        _play(_PHASE2, {"q": (qprod, 2), "o": (oprod, 4), "g": (attn, 2)}, pieces)

    pl.loop(0, _NT)(phase2)
    for t in range(_NT):
        for blk in range(4):
            cp_o(t, blk).wait()


@jax.jit
def pallas_gated_mix__linear_kernel_hedgehog__moe_arch_mod__prompt_kernel(
    A_x: jax.Array,
    A_wqkv: jax.Array,
    A_w_phi: jax.Array,
    A_wo: jax.Array,
    B_x: jax.Array,
    B_w_r: jax.Array,
    B_w_gate: jax.Array,
    B_w_up: jax.Array,
    B_w_down: jax.Array,
    gate_w: jax.Array,
):
    del B_x
    hbm = pl.BlockSpec(memory_space=pl.ANY)
    dma = pltpu.SemaphoreType.DMA
    out = pl.pallas_call(
        _kernel,
        out_shape=jax.ShapeDtypeStruct((_S, _D), _BF),
        in_specs=[hbm] * 9,
        out_specs=hbm,
        scratch_shapes=[
            pltpu.VMEM((_NT, _HT, _D), _I32),
            pltpu.VMEM((2, _HD, _D), _I32),
            pltpu.VMEM((_NT, _HD, _FC), _I32),
            pltpu.VMEM((_NT, _HD, _FC), _I32),
            pltpu.VMEM((_NT, _FC // 2, _D), _I32),
            pltpu.VMEM((_H, _DH, _DH), _BF),
            pltpu.VMEM((_D,), _BF),
            pltpu.VMEM((_D,), _BF),
            pltpu.VMEM((4, 256, _HD), _I32),
            pltpu.VMEM((4, 256, _HD), _I32),
            pltpu.VMEM((1, 8, 8, 16, 128), _BF),
            pltpu.VMEM((7, 32, 4, 16, 128), _BF),
            pltpu.VMEM((7, 32, 4, 16, 128), _BF),
            pltpu.VMEM((6, 32, 4, 16, 128), _BF),
            pltpu.VMEM((6, 32, 4, 16, 128), _BF),
            pltpu.VMEM((5 * _NT + 1, 16, 4, 16, 128), _BF),
            [pltpu.VMEM((17, 8, 1, 16, 128), _BF)] * 4,
            [[pltpu.VMEM((_HD, 128), _F32)] * 2] * 4,
            pltpu.VMEM((_NP, 64, 128), _F32),
            pltpu.VMEM((_NP + 1, 128, 128), _F32),
            pltpu.VMEM((_NP, 4, 1, 16, 128), _BF),
            pltpu.VMEM((_S // 128 + 1, 128, 128), _F32),
            pltpu.VMEM((8, 128), _F32),
            pltpu.VMEM((2, 8, 128), _I32),
            pltpu.VMEM((23, 8, 128), _F32),
            pltpu.VMEM((_D + 8, 128), _F32),
            pltpu.VMEM((_FC, 128), _F32),
            [pltpu.VMEM((_NT + 1, _HT, _HD), _BF)] * 4,
            dma((_NT,)), dma((2,)), dma((2,)), dma((4,)), dma((3,)),
            dma((_NT,)), dma((_NT,)), dma((_NT,)), dma((4 * _NT,)),
        ],
        compiler_params=pltpu.CompilerParams(vmem_limit_bytes=100 * 1024 * 1024,
                                             disable_bounds_checks=True),
    )(A_x.reshape(_S, _D), A_wqkv, A_w_phi, A_wo, B_w_r, B_w_gate, B_w_up, B_w_down, gate_w)
    return out.reshape(1, _S, _D)
```

```python
import jax
import jax.numpy as jnp
import jax.experimental.pallas as pl
import jax.experimental.pallas.tpu as pltpu

_BF = jnp.bfloat16
_F32 = jnp.float32
_I32 = jnp.int32
_LOG2E = 1.4426950408889634

_S, _D, _H, _DH, _F = 2048, 1024, 32, 32, 3584
_T = 512
_HT = _T // 2
_HD = _D // 2
_NT = _S // _T
_FC = _F // _NT
_NP = _H // 2

_A_SLOT = (4, 5, 0, 3, 6, 7, 8)
_B_SLOT = (4, 0, 5, 6, 3, 7, 8)

_LEFT = ((0, 1, 3), (2, 1, 3), (0,), (3,), (0, 1, 1), (2, -1, 0), (1, -1, 3))
_RIGHT = ((0, 1, 3), (0,), (1, -1, 3), (2, -1, 0), (3,), (0, 1, 1), (2, 1, 3))
_ORDER = (1, 4, 3, 2, 0, 6, 5)

_FIRST = ("+r3 +r5 +s ! W0 +a3 ! +a5 +r4 v3:4,4,4,3,3,3,3 +r2 +r1 v5:3,3,2,2,2,2,2 W1 +a4 ! +a2 "
          "v4:3,3,2,2,2,2,2 +a1 v2:3,3,2,2,2,2,2 +a7 +r7 v1:4,4,4,3,3,3,3 +a6 +r6 v7:4,4,4,3,3,3,3 W2 k2 "
          "k5 k4 +f2 k3:4,4 +f1 k1:5,5 k7:5,5 +f0 k6:6,6 +f3 g2:4,4,4,4 v6:2,1,1,1,1,1,1 g1 g0 g3")
_PHASE1 = ("+r2 +r4 +r3 +r5 k2:8,8 +r1 +r6 +r7 k5.1:7 v2:2,2,2,2,2,1,1 k5.0:7 +o v5:5,5,5,5,5,5,4 +f2 k4.0 "
           "+f1 k4.1 k3:8,8 +s v4:2,2,2,2,2,2,2 v3:1,1,1,1,1,1,1 k7 g2 k1:6,2 +f0 g1 v7:0,1,0,0,0,0,0 "
           "k6:10,12 +f3 v1:3,3,3,3,2,3,2 v6:2,2,2,2,2,2,2 g0:1,0,0,1 g3:1,1,2,1")
_PHASE2 = ("+h0 +h1 q4.1:2 q4.0:4 q7.1:1 q1:1,2 q7.0:3 q5.0 +f0 q5.1:2 q3:7,6 q2.0:9 g0 +f1 q2.1:9 +f2 "
           "q6:6,6 +f3 +a g1 o3:2,3,3,3 ! g2 o6:4,3,3,3 g3 +d o5:2,2,2,4 +e1 o1.0:2 o2:1,1,1,1 o4:2,2,2,2 "
           "+e2 o1.2:1 o1.1 o1.3:2 +e3 o7:0,1,3,1 +e0 !")


def _dg(a, b, ca, cb):
    return jax.lax.dot_general(a, b, (((ca,), (cb,)), ((), ())), preferred_element_type=_F32)


def _bf(w):
    return pltpu.bitcast(w, _BF)


def _put(ref, g, c, v):
    for j in range(v.shape[1] // 128):
        ref[pl.ds(g, v.shape[0] // 16), c + j] = v[:, 128 * j:128 * j + 128].reshape(-1, 16, 128).astype(_BF)


def _get(ref, k, g, n, tiles=range(4)):
    words = ref.bitcast(_I32)
    return jnp.concatenate([words[k, pl.ds(g, n), c].reshape(8 * n, 128) for c in tiles], axis=1)


def _a_sums(a11, a12, a21, a22):
    return (a11 + a22, a21 + a22, a11 + a12, a21 - a11, a12 - a22)


def _b_sums(b11, b12, b21, b22):
    return (b11 + b22, b12 - b22, b21 - b11, b11 + b12, b21 + b22)


def _operand(rule, block):
    if len(rule) == 1:
        return block(rule[0])
    return block(rule[0]) + block(rule[2]) if rule[1] > 0 else block(rule[0]) - block(rule[2])


def _put_operands(side, m, block, ref, base, g):
    sub = [_operand(side[m], lambda k: block(k, j)) for j in range(4)]
    for n in range(7):
        _put(ref.at[base + n], g, 0, _operand(side[n], lambda j: sub[j]))
    return sub


def _mix(c, m):
    if c == 0:
        return m(0) + m(3) - m(4) + m(6)
    if c == 1:
        return m(2) + m(4)
    if c == 2:
        return m(1) + m(3)
    return m(0) - m(1) + m(2) + m(5)


def _sum_piece(src, dst, sums, g, c, which=range(5)):
    r = 8 * g if isinstance(g, int) else pl.multiple_of(8 * g, 8)
    out = sums(*[0.0 if b is None else _bf(b[pl.ds(r, 8), 128 * c:128 * c + 256]).astype(_F32) for b in src])
    for k in which:
        _put(dst[k], g, c, out[k])


def _paced(w, zeros):
    if not zeros:
        return w
    groups = w.shape[0] // 8
    first = [w[8 * g:8 * g + 8, 0:128] for g in range(groups)]
    for j, z in enumerate(zeros):
        g = max((j + 1) * groups // len(zeros) - 1, 0)
        first[g] = first[g] | z
    first = jnp.concatenate(first, axis=0)
    return first if w.shape[1] == 128 else jnp.concatenate([first, w[:, 128:]], axis=1)


def _play(program, steps, pieces):
    queue = []
    for word in program.split():
        if word == "!":
            while queue:
                queue.pop(0)()
        elif word[0] == "+":
            queue.extend(pieces(word[1:]))
        else:
            name, _, counts = word.partition(":")
            name, _, tile = name.partition(".")
            step, tiles = steps[name[0]]
            tiles = [int(tile)] if tile else range(tiles)
            counts = [int(n) for n in counts.split(",")] if counts else [0] * len(tiles)
            for t, n in zip(tiles, counts):
                step(int(name[1:]), t, [queue.pop(0)() for _ in range(min(n, len(queue)))])
    assert not queue


def _recip(v):
    r = pl.reciprocal(v, approx=True)
    return r * (2.0 - v * r)


def _pair_reduce(v, op):
    r = v[0:8]
    for j in range(1, 8):
        r = op(r, v[8 * j:8 * j + 8])
    r = op(r, pltpu.roll(r, 2, 0))
    return op(r, pltpu.roll(r, 4, 0))


def _rep8(v):
    return jnp.concatenate([v] * 8, axis=0)


def _dual_exp(p):
    ep = jnp.exp2(p - _rep8(_pair_reduce(p, jnp.maximum)))
    en = jnp.exp2(_rep8(_pair_reduce(p, jnp.minimum)) - p)
    return ep, en, _pair_reduce(ep, jnp.add), _pair_reduce(en, jnp.add)


def _col_bcast(row):
    return jnp.broadcast_to(row, (128, row.shape[1])).T


def _matvec(w_ref, col_ref, c, j0, j1, acc=None):
    for j in range(j0, j1):
        t = _bf(w_ref[8 * j:8 * j + 8, 128 * c:128 * c + 128]).astype(_F32) * col_ref[16 * j:16 * j + 16, :]
        acc = t[0:8] if acc is None else acc + t[0:8]
        acc = acc + t[8:16]
    return acc


def _kernel(x_hbm, wqkv_hbm, wphi_hbm, wo_hbm, wr_hbm, wg_hbm, wu_hbm, wd_hbm, gw_hbm,
            out_hbm,
            x_v, w_v, wg_v, wu_v, wd_v, wphi_v, wr_v, gw_v,
            wv_v, wo_v, lm_v, lk_v, lq_v, lv_v, lo_v, r_v, r2_v, phi_v, a_v, kv_v, z_v, kvm_v, g_v, top_v, arg_v,
            f_v, xc_v, hc_v, out_v,
            sem_x, sem_w, sem_v, sem_wo, sem_s, sem_g, sem_u, sem_d, sem_o):
    x_hbm, wqkv_hbm, wo_hbm, wg_hbm, wu_hbm, wd_hbm = (
        r.bitcast(_I32) for r in (x_hbm, wqkv_hbm, wo_hbm, wg_hbm, wu_hbm, wd_hbm))

    def cp_x(i):
        return pltpu.make_async_copy(x_hbm.at[pl.ds(i * _HT, _HT)], x_v.at[i], sem_x.at[i])

    def cp_w(j):
        return pltpu.make_async_copy(wqkv_hbm.at[:, pl.ds(j * _D, _D)], w_v.at[j], sem_w.at[j])

    def cp_v(k):
        return pltpu.make_async_copy(wqkv_hbm.at[pl.ds(256 * (k % 2), 256), pl.ds(2 * _D + _HD * (k // 2), _HD)],
                                     wv_v.at[k], sem_v.at[k])

    def cp_wo(k):
        return pltpu.make_async_copy(wo_hbm.at[pl.ds(256 * (k // 2), 256), pl.ds(_HD * (k % 2), _HD)],
                                     wo_v.at[k], sem_wo.at[k])

    cp_small = [pltpu.make_async_copy(src, dst, sem_s.at[j]) for j, (src, dst) in enumerate(
        ((wphi_hbm, wphi_v), (wr_hbm, wr_v), (gw_hbm, gw_v)))]

    def cp_ffn(i):
        cols = pl.ds(i * _FC, _FC)
        return (pltpu.make_async_copy(wg_hbm.at[:, cols], wg_v.at[i], sem_g.at[i]),
                pltpu.make_async_copy(wu_hbm.at[:, cols], wu_v.at[i], sem_u.at[i]),
                pltpu.make_async_copy(wd_hbm.at[pl.ds(i * (_FC // 2), _FC // 2)], wd_v.at[i], sem_d.at[i]))

    def cp_o(t, blk):
        return pltpu.make_async_copy(
            out_v[blk].at[t], out_hbm.at[pl.ds(t * _T + _HT * (blk // 2), _HT), pl.ds(_HD * (blk % 2), _HD)],
            sem_o.at[4 * t + blk])

    for cp in cp_small:
        cp.start()
    cp_x(0).start()
    cp_v(0).start()
    cp_v(1).start()

    kv_v[...] = jnp.zeros_like(kv_v)
    z_v[...] = jnp.zeros_like(z_v)
    f_v[...] = jnp.zeros_like(f_v)
    xc_v[_D:, :] = jnp.zeros((8, 128), _F32)
    top_v[...] = jnp.full((8, 128), -jnp.inf, _F32)
    arg_v[...] = jnp.zeros_like(arg_v)
    g_v[_S // 128, 0:8, :] = jnp.zeros((8, 128), _F32)
    for ref in (*r2_v, *lv_v, lo_v, *phi_v):
        ref[ref.shape[0] - 1, 0, 0] = jnp.zeros((16, 128), _BF)
    for ref in out_v:
        ref[_NT, 0:16, 0:128] = jnp.zeros((16, 128), _BF)

    for cp in cp_small:
        cp.wait()
    rows = jax.lax.broadcasted_iota(_I32, (128, _DH), 0)
    cols = jax.lax.broadcasted_iota(_I32, (128, _DH), 1)
    sel = jnp.where(((rows >> 1) & 31) == cols, 1.0, 0.0).astype(_BF)
    full = _dg(sel, wphi_v[...].reshape(_H * _DH, _DH), 1, 1)
    rows = jax.lax.broadcasted_iota(_I32, (128, _D), 0)
    cols = jax.lax.broadcasted_iota(_I32, (128, _D), 1)
    keep = ((cols >> 5) & 3) == 2 * (rows >> 6) + (rows & 1)
    _put(lm_v.at[0], 0, 0, jnp.where(keep, full, 0.0))

    def fold(j, l_v, queue=()):
        for g in range(4):
            for d in range(2):
                blk = []
                for gg in (g, g + 4):
                    c = slice(128 * gg, 128 * gg + 128)
                    for dd in (d, d + 2):
                        w = _paced(w_v[j, 128 * dd:128 * dd + 128, c], [queue.pop(0)() for _ in queue[:1]])
                        blk.append(_dg(_bf(_get(lm_v, 0, 0, 8, [gg])), _bf(w), 1, 1) * _LOG2E)
                blk += _a_sums(*blk)
                for m in range(7):
                    _put(l_v.at[m], 8 * g, 2 * d, blk[_A_SLOT[m]])

    def weight_piece(blocks, ref, sums, g, c, zero, have=range(4), which=range(5)):
        def run():
            _sum_piece([blocks.at[k] if k in have else None for k in range(4)], [ref.at[k] for k in range(5)],
                       sums, g, c, which)
            return _get(ref, 5 + zero, 0, 1, [0])
        return run

    def weight_words(blocks, ref, k, c):
        return blocks[k, :, 128 * c:128 * c + 128] if k < 4 else _get(ref, k - 4, 0, 32, [c])

    def x_blk(i, k):
        return x_v.at[i, 128 * (k % 2):128 * (k % 2) + 128, _HD * (k // 2):_HD * (k // 2) + _HD]

    def tok_words(i, m, g=0, n=16):
        k = _B_SLOT[m]
        return x_blk(i, k)[8 * g:8 * (g + n), :] if k < 4 else _get(r_v[k - 4], i, g, n)

    def put_phi(blk, p, t, zero, pos, neg):
        _put(phi_v[blk].at[2 * p + t], 0, 0, jnp.concatenate([pos, neg], axis=0))
        return _get(phi_v[blk], 16 + zero, 0, 1, [0])

    def get_phi(blk, p, t, zero, zeros=()):
        return _bf(_paced(_get(phi_v[blk], 2 * p + t + zero, 0, 8, [0]), zeros))

    def phase1(i, zero, program):
        pk, pv = {}, {}

        def kprod(m, t, zeros):
            pk[m - 1, t] = _dg(_bf(_paced(_get(lk_v, m - 1, 0, 32), zeros)), _bf(tok_words(i, m - 1, 8 * t, 8)), 1, 1)

        part = {}

        def vprod(m, s, zeros):
            n = _ORDER[s]
            part[m, n] = _dg(_bf(_paced(_get(r2_v[m - 1], 7 * i + n, 0, 8, range(2)), zeros)),
                             _bf(_get(lv_v[m - 1], n, 0, 16, range(2))), 1, 0)
            if s == 6:
                for o in range(2):
                    val = jnp.concatenate([_mix(2 * o + t, lambda n: part[m, n]) for t in range(2)], axis=0)
                    pv[m - 1, 2 * o], pv[m - 1, 2 * o + 1] = val[:, :128], val[:, 128:]

        def kv(blk, c, zeros):
            vt = _mix(blk, lambda m: pv[m, c]).astype(_BF).T
            for h in range(2):
                p = 2 * c + h
                phi = jnp.concatenate([get_phi(blk, p, 0, zero, zeros[h::2]), get_phi(blk, p, 1, zero)], axis=1)
                kv_v[8 * (blk // 2) + p] += _dg(vt[64 * h:64 * h + 64], phi, 1, 1)

        def wait(j, t, zeros):
            for cp in (cp_v(2 * j), cp_v(2 * j + 1)) if j < 2 else (cp_w(1),):
                cp.wait()
            if j == 0:
                cp_w(1).start()
            elif j == 1:
                cp_x(1).start()
                for k in range(4):
                    cp_wo(k).start()
            else:
                for k in range(2, _NT):
                    cp_x(k).start()
                cp_w(0).start()
                for k in range(_NT):
                    for cp in cp_ffn(k):
                        cp.start()
                fold(1, lk_v)

        def token_piece(m, g):
            def run():
                def block(k, j):
                    r = 64 * (j % 2) + 8 * g
                    return _bf(x_blk(i, k)[r:r + 8, 256 * (j // 2):256 * (j // 2) + 256]).astype(_F32)
                sub = _put_operands(_RIGHT, m, block, r2_v[m], 7 * (i + zero), g)
                if _B_SLOT[m] > 3:
                    for j in range(4):
                        _put(r_v[_B_SLOT[m] - 4].at[i + zero], 8 * (j % 2) + g, 2 * (j // 2), sub[j])
                return _get(r2_v[m], 7 * _NT, 0, 1, [0])
            return run

        def value_piece(m, g):
            def run():
                def block(k, j):
                    r = 128 * (j % 2) + 8 * g
                    return _bf(wv_v[k, r:r + 8, 256 * (j // 2):256 * (j // 2) + 256]).astype(_F32)
                _put_operands(_LEFT, m, block, lv_v[m], 0, g)
                return _get(lv_v[m], 7 + zero, 0, 1, [0])
            return run

        def feat_piece(blk, t, p):
            def run():
                ep, en, sp, sn = _dual_exp(_mix(blk, lambda m: pk[m, t][64 * p:64 * p + 64]))
                ep, en = ep * _rep8(_recip(sp)), en * _rep8(_recip(sn))
                z_v[8 * (blk // 2) + p] += jnp.concatenate([ep, en], axis=0)
                return put_phi(blk, p, t, zero, ep, en)
            return run

        def score_piece(c):
            def run():
                xh = _bf(x_v[i, 16 * c:16 * c + 16, :]).astype(_F32)
                wr = wr_v[...].astype(_F32).reshape(1, _D)
                gw = gw_v[...].astype(_F32).reshape(1, _D)
                g = jax.nn.sigmoid(jnp.sum(xh * gw, axis=1, keepdims=True))
                g_v[4 * i + c // 4, 32 * (c % 4):32 * (c % 4) + 32, :] = jnp.broadcast_to(g, (32, 128))
                sc = jnp.sum(xh * wr, axis=1, keepdims=True).astype(_BF).astype(_F32)
                best, bidx = top_v[...], arg_v[0]
                for j in range(4):
                    rj = sc[8 * j:8 * j + 8]
                    upd = rj > best
                    best = jnp.where(upd, rj, best)
                    bidx = jnp.where(upd, i * _T + 32 * c + 8 * j, bidx)
                top_v[...] = best
                arg_v[0] = bidx
                return arg_v[1 + zero] | pltpu.bitcast(g_v[_S // 128 + zero, 0:8, :], _I32)
            return run

        def pieces(name):
            if name[0] == "r":
                return [token_piece(int(name[1]) - 1, g) for g in range(8)]
            if name == "s":
                return [score_piece(c) for c in range(16)]
            if name[0] == "a":
                return [value_piece(int(name[1]) - 1, g) for g in range(16)]
            if name == "o":
                start = jnp.minimum(11 * (i - 1), 32 - 11)
                return [weight_piece(wo_v, lo_v, _b_sums, start + j // 2, 2 * (j % 2), 0) for j in range(22)]
            return [feat_piece(int(name[1]), t, p) for t in ([int(name[2])] if name[2:] else range(2))
                    for p in range(8)]

        _play(program, {"k": (kprod, 2), "v": (vprod, 7), "g": (kv, 4), "W": (wait, 1)}, pieces)

    def later_tile(i):
        cp_x(i).wait()
        phase1(i, i >> 8, _PHASE1)

    zero = arg_v[1, 0, 0]
    cp_x(0).wait()
    cp_v(2).start()
    cp_v(3).start()
    phase1(0, zero, _FIRST)
    for k in range(4):
        cp_wo(k).wait()
    pl.loop(1, _NT)(later_tile)

    cp_w(0).wait()
    best = top_v[...]
    bidx = arg_v[0] + jax.lax.broadcasted_iota(_I32, (8, 128), 0)
    rmax = jnp.max(best, axis=0, keepdims=True)
    idx = jnp.min(jnp.where(best == rmax, bidx, _S - 1))
    r_sel = jax.nn.sigmoid(rmax)
    tsel = idx // _T
    rsel = idx - tsel * _T
    grp = _bf(x_v[tsel, pl.ds(pl.multiple_of((rsel >> 4) << 3, 8), 8), :]).astype(_F32)
    hit = jax.lax.broadcasted_iota(_I32, (16, _D), 0) == (rsel & 15)
    x_sel = jnp.sum(jnp.where(hit, grp, 0.0), axis=0, keepdims=True)

    def state_piece(p):
        def run():
            rows = jax.lax.broadcasted_iota(_I32, (64, 128), 0)
            cols = jax.lax.broadcasted_iota(_I32, (64, 128), 1)
            _put(kvm_v.at[p], 0, 0, jnp.where((rows >> 5) == (cols & 1), kv_v[p], 0.0))
            z_v[p] = jnp.broadcast_to(jnp.sum(z_v[p], axis=1, keepdims=True), (128, 128))
            return pltpu.bitcast(z_v[_NP + zero, 0:8, :], _I32)
        return run

    def column_piece(c):
        def run():
            xc_v[128 * c:128 * c + 128, :] = _col_bcast(x_sel[:, 128 * c:128 * c + 128])
            return pltpu.bitcast(xc_v[pl.ds(pl.multiple_of(_D + zero, 8), 8), :], _I32)
        return run

    fold(0, lq_v, [state_piece(p) for p in range(_NP)] + [column_piece(c) for c in range(8)])

    def phase2(i):
        ti = (tsel + 1 + i) % _NT
        for cp in cp_ffn(i):
            cp.wait()
        zero = i >> 8
        pq, po, ot = {}, {}, {}

        def qprod(m, t, zeros):
            pq[m - 1, t] = _dg(_bf(_paced(_get(lq_v, m - 1, 0, 32), zeros)), _bf(tok_words(ti, m - 1, 8 * t, 8)), 1, 1)

        def attn(blk, t, zeros):
            for p in range(8):
                a_v[blk][t][64 * p:64 * p + 64, :] = _dg(
                    _bf(_get(kvm_v, 8 * (blk // 2) + p, 0, 4, [0])), get_phi(blk, p, t, zero, zeros[p::8]), 1, 0)

        def oprod(m, c, zeros):
            if m not in ot:
                at = []
                for t in range(2):
                    blk = [a_v[b][t][pl.ds(pl.multiple_of(zero, 8), _HD), :] for b in (0, 2, 1, 3)]
                    at.append((*blk, *_a_sums(*blk))[_A_SLOT[m - 1]].astype(_BF).T)
                ot[m] = jnp.concatenate(at, axis=0)
            w = weight_words(wo_v, lo_v, _B_SLOT[m - 1], c)
            po[m - 1, c] = _dg(ot[m], _bf(jnp.concatenate([_paced(w[0:64], zeros), w[64:]], axis=0)), 1, 0)

        def feat_piece(blk, t, p):
            def run():
                ep, en, sp, sn = _dual_exp(_mix(blk, lambda m: pq[m, t][64 * p:64 * p + 64]))
                z = z_v[8 * (blk // 2) + p]
                dp, dn = _pair_reduce(ep * z[0:64], jnp.add), _pair_reduce(en * z[64:128], jnp.add)
                inv = _recip(dp * sn + sp * (dn + 1e-6 * sn))
                return put_phi(blk, p, t, zero, ep * _rep8(sn * inv), en * _rep8(sp * inv))
            return run

        def hidden_piece(c, half):
            def run():
                for k, w in enumerate((wg_v, wu_v)):
                    acc = f_v[2 * c + k + zero] if half else None
                    f_v[2 * c + k] = _matvec(w.at[i], xc_v, c, 32 * half, 32 * half + 32, acc)
                return pltpu.bitcast(f_v[22 + zero], _I32)
            return run

        def act_piece(c):
            def run():
                hg, hu = (jnp.sum(f_v[2 * c + k + zero], axis=0, keepdims=True) for k in range(2))
                hc_v[128 * c:128 * c + 128, :] = _col_bcast(hg * jax.nn.sigmoid(hg) * hu)
            return run

        def down_piece(c, half):
            def run():
                for cc in (c, c + 1):
                    f_v[14 + cc] = _matvec(wd_v.at[i], hc_v, cc, 28 * half, 28 * half + 28, f_v[14 + cc + zero])
                return pltpu.bitcast(f_v[22 + zero], _I32)
            return run

        def emit_piece(blk, u, c):
            def run():
                h, d = blk // 2, blk % 2
                g = g_v[4 * ti + 2 * h + u]
                tok = jax.lax.broadcasted_iota(_I32, (128, 128), 0) + (ti * _T + _HT * h + 128 * u)
                o = []
                for cc in (c, c + 1):
                    y = jnp.sum(f_v[14 + 4 * d + cc + zero], axis=0, keepdims=True) * r_sel
                    b = _bf(x_blk(ti, 2 * d + h)[64 * u:64 * u + 64, 128 * cc:128 * cc + 128]).astype(_F32)
                    b = b + jnp.where(tok == idx, y, 0.0)
                    o.append(g * _mix(blk, lambda m: po[m, cc][128 * u:128 * u + 128]) + (1.0 - g) * b)
                out_v[blk][ti, 128 * u:128 * u + 128, 128 * c:128 * c + 256] = jnp.concatenate(o, axis=1).astype(_BF)
                if (u, c) == (1, 2):
                    cp_o(ti, blk).start()
                    out_v[blk][_NT, 16:32, 0:128] = jnp.zeros((16, 128), _BF)
                return pltpu.bitcast(out_v[blk][_NT + zero, 0:16, 0:128], _I32)
            return run

        def pieces(name):
            if name[0] == "h":
                return [hidden_piece(c, int(name[1])) for c in range(_FC // 128)]
            if name == "a":
                return [act_piece(c) for c in range(_FC // 128)]
            if name == "d":
                return [down_piece(c, half) for c in (4, 6, 0, 2) for half in range(2)]
            if name[0] == "e":
                return [emit_piece(int(name[1]), u, c) for c in (0, 2) for u in range(2)]
            return [feat_piece(int(name[1]), t, p) for t in ([int(name[2])] if name[2:] else range(2))
                    for p in range(8)]

        _play(_PHASE2, {"q": (qprod, 2), "o": (oprod, 4), "g": (attn, 2)}, pieces)

    pl.loop(0, _NT)(phase2)
    for t in range(_NT):
        for blk in range(4):
            cp_o(t, blk).wait()


@jax.jit
def pallas_gated_mix__linear_kernel_hedgehog__moe_arch_mod__prompt_kernel(
    A_x: jax.Array,
    A_wqkv: jax.Array,
    A_w_phi: jax.Array,
    A_wo: jax.Array,
    B_x: jax.Array,
    B_w_r: jax.Array,
    B_w_gate: jax.Array,
    B_w_up: jax.Array,
    B_w_down: jax.Array,
    gate_w: jax.Array,
):
    del B_x
    hbm = pl.BlockSpec(memory_space=pl.ANY)
    dma = pltpu.SemaphoreType.DMA
    out = pl.pallas_call(
        _kernel,
        out_shape=jax.ShapeDtypeStruct((_S, _D), _BF),
        in_specs=[hbm] * 9,
        out_specs=hbm,
        scratch_shapes=[
            pltpu.VMEM((_NT, _HT, _D), _I32),
            pltpu.VMEM((2, _HD, _D), _I32),
            pltpu.VMEM((_NT, _HD, _FC), _I32),
            pltpu.VMEM((_NT, _HD, _FC), _I32),
            pltpu.VMEM((_NT, _FC // 2, _D), _I32),
            pltpu.VMEM((_H, _DH, _DH), _BF),
            pltpu.VMEM((_D,), _BF),
            pltpu.VMEM((_D,), _BF),
            pltpu.VMEM((4, 256, _HD), _I32),
            pltpu.VMEM((4, 256, _HD), _I32),
            pltpu.VMEM((1, 8, 8, 16, 128), _BF),
            pltpu.VMEM((7, 32, 4, 16, 128), _BF),
            pltpu.VMEM((7, 32, 4, 16, 128), _BF),
            [pltpu.VMEM((8, 16, 2, 16, 128), _BF)] * 7,
            pltpu.VMEM((6, 32, 4, 16, 128), _BF),
            [pltpu.VMEM((_NT, 16, 4, 16, 128), _BF)] * 5,
            [pltpu.VMEM((7 * _NT + 1, 8, 2, 16, 128), _BF)] * 7,
            [pltpu.VMEM((17, 8, 1, 16, 128), _BF)] * 4,
            [[pltpu.VMEM((_HD, 128), _F32)] * 2] * 4,
            pltpu.VMEM((_NP, 64, 128), _F32),
            pltpu.VMEM((_NP + 1, 128, 128), _F32),
            pltpu.VMEM((_NP, 4, 1, 16, 128), _BF),
            pltpu.VMEM((_S // 128 + 1, 128, 128), _F32),
            pltpu.VMEM((8, 128), _F32),
            pltpu.VMEM((2, 8, 128), _I32),
            pltpu.VMEM((23, 8, 128), _F32),
            pltpu.VMEM((_D + 8, 128), _F32),
            pltpu.VMEM((_FC, 128), _F32),
            [pltpu.VMEM((_NT + 1, _HT, _HD), _BF)] * 4,
            dma((_NT,)), dma((2,)), dma((2,)), dma((4,)), dma((3,)),
            dma((_NT,)), dma((_NT,)), dma((_NT,)), dma((4 * _NT,)),
        ],
        compiler_params=pltpu.CompilerParams(vmem_limit_bytes=120 * 1024 * 1024,
                                             disable_bounds_checks=True),
    )(A_x.reshape(_S, _D), A_wqkv, A_w_phi, A_wo, B_w_r, B_w_gate, B_w_up, B_w_down, gate_w)
    return out.reshape(1, _S, _D)
```

```python
import jax
import jax.numpy as jnp
import jax.experimental.pallas as pl
import jax.experimental.pallas.tpu as pltpu

_BF = jnp.bfloat16
_F32 = jnp.float32
_I32 = jnp.int32
_LOG2E = 1.4426950408889634

_S, _D, _H, _DH, _F = 2048, 1024, 32, 32, 3584
_T = 512
_HT = _T // 2
_HD = _D // 2
_NT = _S // _T
_FC = _F // _NT
_NP = _H // 2

_A_SLOT = (4, 5, 0, 3, 6, 7, 8)
_B_SLOT = (4, 0, 5, 6, 3, 7, 8)

_LEFT = ((0, 1, 3), (2, 1, 3), (0,), (3,), (0, 1, 1), (2, -1, 0), (1, -1, 3))
_RIGHT = ((0, 1, 3), (0,), (1, -1, 3), (2, -1, 0), (3,), (0, 1, 1), (2, 1, 3))
_ORDER = (1, 4, 3, 2, 0, 6, 5)

_FIRST = ("+r3 +r5 +r4 +r2 +s ! W0 +a3 ! v3.0:2 +a5 v3.1:4 +r1 v3.2:4 v3.3:3 v3.4:3 v3.5:2 v3.6:1 "
          "v5:2,2,1,1,1,1,1 W1 +a4 ! +a2 +a1 v4:3,5,2,2,2,3,2 v2:3,3,2,2,2,2,2 +a7 +r7 v1:4,4,4,3,3,3,3 "
          "+r6 +a6 v7:4,4,4,3,1,3,3 W2 k2:1,0 k5 k4 +f2 k3:6,6 k1:5,5 +f1 k7:7,8 +f0 k6:7,6 "
          "v6:2,1,1,1,1,1,1 +f3 g0 g1.0 g2:5,5,5,5 g1.2 g1.1 g1.3 g3")
_PHASE1 = ("+r2 +r3 +r4 +r6 +r5 +r7 +r1 k5.1:7 +o k2:8,8 v2:2,2,2,2,2,1,1 k5.0:7 +f2 v5:5,5,5,5,5,5,4 +f1 "
           "k4 k3.0:8 +s k3.1:8 v4:2,2,2,2,2,2,2 v3:1,1,1,1,1,1,1 k7 g2 k1:6,2 +f0 g1.0 g1.1 g1.3 g1.2 "
           "v7:3,4,3,3,3,3,3 v1:3,1,3,3,2,3,2 k6:12,14 +f3 v6:2,0,2,2,2,2,2 g0:1,0,2,1 g3:1,0,2,1")
_PHASE2 = ("+h0 +h1 q4.1:2 q4.0:4 q7.1:1 q1:1,2 q7.0:3 q5.0 +f0 q5.1:2 q3:7,6 q2.0:9 g0 +f1 q2.1:9 +f2 "
           "q6:6,6 +f3 +a g1 o3:2,3,3,3 ! g2 o6:4,3,3,3 g3 +d o5:2,2,2,4 +e1 o1.0:2 o2:1,1,1,1 o4:2,2,2,2 "
           "+e2 o1.2:1 o1.1 o1.3:2 +e3 o7:0,1,3,1 +e0 !")


def _dg(a, b, ca, cb):
    return jax.lax.dot_general(a, b, (((ca,), (cb,)), ((), ())), preferred_element_type=_F32)


def _bf(w):
    return pltpu.bitcast(w, _BF)


def _put(ref, g, c, v):
    for j in range(v.shape[1] // 128):
        ref[pl.ds(g, v.shape[0] // 16), c + j] = v[:, 128 * j:128 * j + 128].reshape(-1, 16, 128).astype(_BF)


def _get(ref, k, g, n, tiles=range(4)):
    words = ref.bitcast(_I32)
    return jnp.concatenate([words[k, pl.ds(g, n), c].reshape(8 * n, 128) for c in tiles], axis=1)


def _a_sums(a11, a12, a21, a22):
    return (a11 + a22, a21 + a22, a11 + a12, a21 - a11, a12 - a22)


def _b_sums(b11, b12, b21, b22):
    return (b11 + b22, b12 - b22, b21 - b11, b11 + b12, b21 + b22)


def _operand(rule, block):
    if len(rule) == 1:
        return block(rule[0])
    return block(rule[0]) + block(rule[2]) if rule[1] > 0 else block(rule[0]) - block(rule[2])


def _put_operands(side, m, block, ref, base, g):
    sub = [_operand(side[m], lambda k: block(k, j)) for j in range(4)]
    for n in range(7):
        _put(ref.at[base + n], g, 0, _operand(side[n], lambda j: sub[j]))
    return sub


def _mix(c, m):
    if c == 0:
        return m(0) + m(3) - m(4) + m(6)
    if c == 1:
        return m(2) + m(4)
    if c == 2:
        return m(1) + m(3)
    return m(0) - m(1) + m(2) + m(5)


def _sum_piece(src, dst, sums, g, c, which=range(5)):
    r = 8 * g if isinstance(g, int) else pl.multiple_of(8 * g, 8)
    out = sums(*[0.0 if b is None else _bf(b[pl.ds(r, 8), 128 * c:128 * c + 256]).astype(_F32) for b in src])
    for k in which:
        _put(dst[k], g, c, out[k])


def _paced(w, zeros):
    if not zeros:
        return w
    groups = w.shape[0] // 8
    first = [w[8 * g:8 * g + 8, 0:128] for g in range(groups)]
    for j, z in enumerate(zeros):
        g = max((j + 1) * groups // len(zeros) - 1, 0)
        first[g] = first[g] | z
    first = jnp.concatenate(first, axis=0)
    return first if w.shape[1] == 128 else jnp.concatenate([first, w[:, 128:]], axis=1)


def _play(program, steps, pieces):
    queue = []
    for word in program.split():
        if word == "!":
            while queue:
                queue.pop(0)()
        elif word[0] == "+":
            queue.extend(pieces(word[1:]))
        else:
            name, _, counts = word.partition(":")
            name, _, tile = name.partition(".")
            step, tiles = steps[name[0]]
            tiles = [int(tile)] if tile else range(tiles)
            counts = [int(n) for n in counts.split(",")] if counts else [0] * len(tiles)
            for t, n in zip(tiles, counts):
                step(int(name[1:]), t, [queue.pop(0)() for _ in range(min(n, len(queue)))])
    assert not queue


def _recip(v):
    r = pl.reciprocal(v, approx=True)
    return r * (2.0 - v * r)


def _pair_reduce(v, op):
    r = v[0:8]
    for j in range(1, 8):
        r = op(r, v[8 * j:8 * j + 8])
    r = op(r, pltpu.roll(r, 2, 0))
    return op(r, pltpu.roll(r, 4, 0))


def _rep8(v):
    return jnp.concatenate([v] * 8, axis=0)


def _dual_exp(p):
    ep = jnp.exp2(p - _rep8(_pair_reduce(p, jnp.maximum)))
    en = jnp.exp2(_rep8(_pair_reduce(p, jnp.minimum)) - p)
    return ep, en, _pair_reduce(ep, jnp.add), _pair_reduce(en, jnp.add)


def _col_bcast(row):
    return jnp.broadcast_to(row, (128, row.shape[1])).T


def _matvec(w_ref, col_ref, c, j0, j1, acc=None):
    for j in range(j0, j1):
        t = _bf(w_ref[8 * j:8 * j + 8, 128 * c:128 * c + 128]).astype(_F32) * col_ref[16 * j:16 * j + 16, :]
        acc = t[0:8] if acc is None else acc + t[0:8]
        acc = acc + t[8:16]
    return acc


def _kernel(x_hbm, wqkv_hbm, wphi_hbm, wo_hbm, wr_hbm, wg_hbm, wu_hbm, wd_hbm, gw_hbm,
            out_hbm,
            x_v, w_v, wg_v, wu_v, wd_v, wphi_v, wr_v, gw_v,
            wv_v, wo_v, lm_v, lk_v, lq_v, lv_v, lo_v, r_v, r2_v, phi_v, a_v, kv_v, z_v, kvm_v, g_v, top_v, arg_v,
            f_v, xc_v, hc_v, out_v,
            sem_x, sem_w, sem_v, sem_wo, sem_s, sem_g, sem_u, sem_d, sem_o):
    x_hbm, wqkv_hbm, wo_hbm, wg_hbm, wu_hbm, wd_hbm = (
        r.bitcast(_I32) for r in (x_hbm, wqkv_hbm, wo_hbm, wg_hbm, wu_hbm, wd_hbm))

    def cp_x(i):
        return pltpu.make_async_copy(x_hbm.at[pl.ds(i * _HT, _HT)], x_v.at[i], sem_x.at[i])

    def cp_w(j):
        return pltpu.make_async_copy(wqkv_hbm.at[:, pl.ds(j * _D, _D)], w_v.at[j], sem_w.at[j])

    def cp_v(k):
        return pltpu.make_async_copy(wqkv_hbm.at[pl.ds(256 * (k % 2), 256), pl.ds(2 * _D + _HD * (k // 2), _HD)],
                                     wv_v.at[k], sem_v.at[k])

    def cp_wo(k):
        return pltpu.make_async_copy(wo_hbm.at[pl.ds(256 * (k // 2), 256), pl.ds(_HD * (k % 2), _HD)],
                                     wo_v.at[k], sem_wo.at[k])

    cp_small = [pltpu.make_async_copy(src, dst, sem_s.at[j]) for j, (src, dst) in enumerate(
        ((wphi_hbm, wphi_v), (wr_hbm, wr_v), (gw_hbm, gw_v)))]

    def cp_ffn(i):
        cols = pl.ds(i * _FC, _FC)
        return (pltpu.make_async_copy(wg_hbm.at[:, cols], wg_v.at[i], sem_g.at[i]),
                pltpu.make_async_copy(wu_hbm.at[:, cols], wu_v.at[i], sem_u.at[i]),
                pltpu.make_async_copy(wd_hbm.at[pl.ds(i * (_FC // 2), _FC // 2)], wd_v.at[i], sem_d.at[i]))

    def cp_o(t, blk):
        return pltpu.make_async_copy(
            out_v[blk].at[t], out_hbm.at[pl.ds(t * _T + _HT * (blk // 2), _HT), pl.ds(_HD * (blk % 2), _HD)],
            sem_o.at[4 * t + blk])

    for cp in cp_small:
        cp.start()
    cp_x(0).start()
    cp_v(0).start()
    cp_v(1).start()

    kv_v[...] = jnp.zeros_like(kv_v)
    z_v[...] = jnp.zeros_like(z_v)
    f_v[...] = jnp.zeros_like(f_v)
    xc_v[_D:, :] = jnp.zeros((8, 128), _F32)
    top_v[...] = jnp.full((8, 128), -jnp.inf, _F32)
    arg_v[...] = jnp.zeros_like(arg_v)
    g_v[_S // 128, 0:8, :] = jnp.zeros((8, 128), _F32)
    for ref in (*r2_v, *lv_v, lo_v, *phi_v):
        ref[ref.shape[0] - 1, 0, 0] = jnp.zeros((16, 128), _BF)
    for ref in out_v:
        ref[_NT, 0:16, 0:128] = jnp.zeros((16, 128), _BF)

    for cp in cp_small:
        cp.wait()
    rows = jax.lax.broadcasted_iota(_I32, (128, _DH), 0)
    cols = jax.lax.broadcasted_iota(_I32, (128, _DH), 1)
    sel = jnp.where(((rows >> 1) & 31) == cols, 1.0, 0.0).astype(_BF)
    full = _dg(sel, wphi_v[...].reshape(_H * _DH, _DH), 1, 1)
    rows = jax.lax.broadcasted_iota(_I32, (128, _D), 0)
    cols = jax.lax.broadcasted_iota(_I32, (128, _D), 1)
    keep = ((cols >> 5) & 3) == 2 * (rows >> 6) + (rows & 1)
    _put(lm_v.at[0], 0, 0, jnp.where(keep, full, 0.0))

    def fold(j, l_v, queue=()):
        for g in range(4):
            for d in range(2):
                blk = []
                for gg in (g, g + 4):
                    c = slice(128 * gg, 128 * gg + 128)
                    for dd in (d, d + 2):
                        w = _paced(w_v[j, 128 * dd:128 * dd + 128, c], [queue.pop(0)() for _ in queue[:1]])
                        blk.append(_dg(_bf(_get(lm_v, 0, 0, 8, [gg])), _bf(w), 1, 1) * _LOG2E)
                blk += _a_sums(*blk)
                for m in range(7):
                    _put(l_v.at[m], 8 * g, 2 * d, blk[_A_SLOT[m]])

    def weight_piece(blocks, ref, sums, g, c, zero, have=range(4), which=range(5)):
        def run():
            _sum_piece([blocks.at[k] if k in have else None for k in range(4)], [ref.at[k] for k in range(5)],
                       sums, g, c, which)
            return _get(ref, 5 + zero, 0, 1, [0])
        return run

    def weight_words(blocks, ref, k, c):
        return blocks[k, :, 128 * c:128 * c + 128] if k < 4 else _get(ref, k - 4, 0, 32, [c])

    def x_blk(i, k):
        return x_v.at[i, 128 * (k % 2):128 * (k % 2) + 128, _HD * (k // 2):_HD * (k // 2) + _HD]

    def tok_words(i, m, g=0, n=16):
        k = _B_SLOT[m]
        return x_blk(i, k)[8 * g:8 * (g + n), :] if k < 4 else _get(r_v[k - 4], i, g, n)

    def put_phi(blk, p, t, zero, pos, neg):
        _put(phi_v[blk].at[2 * p + t], 0, 0, jnp.concatenate([pos, neg], axis=0))
        return _get(phi_v[blk], 16 + zero, 0, 1, [0])

    def get_phi(blk, p, t, zero, zeros=()):
        return _bf(_paced(_get(phi_v[blk], 2 * p + t + zero, 0, 8, [0]), zeros))

    def phase1(i, zero, program):
        pk, pv = {}, {}

        def kprod(m, t, zeros):
            pk[m - 1, t] = _dg(_bf(_paced(_get(lk_v, m - 1, 0, 32), zeros)), _bf(tok_words(i, m - 1, 8 * t, 8)), 1, 1)

        part = {}

        def vprod(m, s, zeros):
            n = _ORDER[s]
            part[m, n] = _dg(_bf(_paced(_get(r2_v[m - 1], 7 * i + n, 0, 8, range(2)), zeros)),
                             _bf(_get(lv_v[m - 1], n, 0, 16, range(2))), 1, 0)
            if s == 6:
                for o in range(2):
                    val = jnp.concatenate([_mix(2 * o + t, lambda n: part[m, n]) for t in range(2)], axis=0)
                    pv[m - 1, 2 * o], pv[m - 1, 2 * o + 1] = val[:, :128], val[:, 128:]

        def kv(blk, c, zeros):
            vt = _mix(blk, lambda m: pv[m, c]).astype(_BF).T
            for h in range(2):
                p = 2 * c + h
                phi = jnp.concatenate([get_phi(blk, p, 0, zero, zeros[h::2]), get_phi(blk, p, 1, zero)], axis=1)
                kv_v[8 * (blk // 2) + p] += _dg(vt[64 * h:64 * h + 64], phi, 1, 1)

        def wait(j, t, zeros):
            for cp in (cp_v(2 * j), cp_v(2 * j + 1)) if j < 2 else (cp_w(1),):
                cp.wait()
            if j == 0:
                cp_w(1).start()
            elif j == 1:
                cp_x(1).start()
                for k in range(4):
                    cp_wo(k).start()
            else:
                for k in range(2, _NT):
                    cp_x(k).start()
                cp_w(0).start()
                for k in range(_NT):
                    for cp in cp_ffn(k):
                        cp.start()
                fold(1, lk_v)

        def token_piece(m, g):
            def run():
                def block(k, j):
                    r = 64 * (j % 2) + 8 * g
                    return _bf(x_blk(i, k)[r:r + 8, 256 * (j // 2):256 * (j // 2) + 256]).astype(_F32)
                sub = _put_operands(_RIGHT, m, block, r2_v[m], 7 * (i + zero), g)
                if _B_SLOT[m] > 3:
                    for j in range(4):
                        _put(r_v[_B_SLOT[m] - 4].at[i + zero], 8 * (j % 2) + g, 2 * (j // 2), sub[j])
                return _get(r2_v[m], 7 * _NT, 0, 1, [0])
            return run

        def value_piece(m, g):
            def run():
                def block(k, j):
                    r = 128 * (j % 2) + 8 * g
                    return _bf(wv_v[k, r:r + 8, 256 * (j // 2):256 * (j // 2) + 256]).astype(_F32)
                _put_operands(_LEFT, m, block, lv_v[m], 0, g)
                return _get(lv_v[m], 7 + zero, 0, 1, [0])
            return run

        def feat_piece(blk, t, p):
            def run():
                ep, en, sp, sn = _dual_exp(_mix(blk, lambda m: pk[m, t][64 * p:64 * p + 64]))
                ep, en = ep * _rep8(_recip(sp)), en * _rep8(_recip(sn))
                z_v[8 * (blk // 2) + p] += jnp.concatenate([ep, en], axis=0)
                return put_phi(blk, p, t, zero, ep, en)
            return run

        def score_piece(c):
            def run():
                xh = _bf(x_v[i, 16 * c:16 * c + 16, :]).astype(_F32)
                wr = wr_v[...].astype(_F32).reshape(1, _D)
                gw = gw_v[...].astype(_F32).reshape(1, _D)
                g = jax.nn.sigmoid(jnp.sum(xh * gw, axis=1, keepdims=True))
                g_v[4 * i + c // 4, 32 * (c % 4):32 * (c % 4) + 32, :] = jnp.broadcast_to(g, (32, 128))
                sc = jnp.sum(xh * wr, axis=1, keepdims=True).astype(_BF).astype(_F32)
                best, bidx = top_v[...], arg_v[0]
                for j in range(4):
                    rj = sc[8 * j:8 * j + 8]
                    upd = rj > best
                    best = jnp.where(upd, rj, best)
                    bidx = jnp.where(upd, i * _T + 32 * c + 8 * j, bidx)
                top_v[...] = best
                arg_v[0] = bidx
                return arg_v[1 + zero] | pltpu.bitcast(g_v[_S // 128 + zero, 0:8, :], _I32)
            return run

        def pieces(name):
            if name[0] == "r":
                return [token_piece(int(name[1]) - 1, g) for g in range(8)]
            if name == "s":
                return [score_piece(c) for c in range(16)]
            if name[0] == "a":
                return [value_piece(int(name[1]) - 1, g) for g in range(16)]
            if name == "o":
                start = jnp.minimum(11 * (i - 1), 32 - 11)
                return [weight_piece(wo_v, lo_v, _b_sums, start + j // 2, 2 * (j % 2), 0) for j in range(22)]
            return [feat_piece(int(name[1]), t, p) for t in ([int(name[2])] if name[2:] else range(2))
                    for p in range(8)]

        _play(program, {"k": (kprod, 2), "v": (vprod, 7), "g": (kv, 4), "W": (wait, 1)}, pieces)

    def later_tile(i):
        cp_x(i).wait()
        phase1(i, i >> 8, _PHASE1)

    zero = arg_v[1, 0, 0]
    cp_x(0).wait()
    cp_v(2).start()
    cp_v(3).start()
    phase1(0, zero, _FIRST)
    for k in range(4):
        cp_wo(k).wait()
    pl.loop(1, _NT)(later_tile)

    cp_w(0).wait()
    best = top_v[...]
    bidx = arg_v[0] + jax.lax.broadcasted_iota(_I32, (8, 128), 0)
    rmax = jnp.max(best, axis=0, keepdims=True)
    idx = jnp.min(jnp.where(best == rmax, bidx, _S - 1))
    r_sel = jax.nn.sigmoid(rmax)
    tsel = idx // _T
    rsel = idx - tsel * _T
    grp = _bf(x_v[tsel, pl.ds(pl.multiple_of((rsel >> 4) << 3, 8), 8), :]).astype(_F32)
    hit = jax.lax.broadcasted_iota(_I32, (16, _D), 0) == (rsel & 15)
    x_sel = jnp.sum(jnp.where(hit, grp, 0.0), axis=0, keepdims=True)

    def state_piece(p):
        def run():
            rows = jax.lax.broadcasted_iota(_I32, (64, 128), 0)
            cols = jax.lax.broadcasted_iota(_I32, (64, 128), 1)
            _put(kvm_v.at[p], 0, 0, jnp.where((rows >> 5) == (cols & 1), kv_v[p], 0.0))
            z_v[p] = jnp.broadcast_to(jnp.sum(z_v[p], axis=1, keepdims=True), (128, 128))
            return pltpu.bitcast(z_v[_NP + zero, 0:8, :], _I32)
        return run

    def column_piece(c):
        def run():
            xc_v[128 * c:128 * c + 128, :] = _col_bcast(x_sel[:, 128 * c:128 * c + 128])
            return pltpu.bitcast(xc_v[pl.ds(pl.multiple_of(_D + zero, 8), 8), :], _I32)
        return run

    fold(0, lq_v, [state_piece(p) for p in range(_NP)] + [column_piece(c) for c in range(8)])

    def phase2(i):
        ti = (tsel + 1 + i) % _NT
        for cp in cp_ffn(i):
            cp.wait()
        zero = i >> 8
        pq, po, ot = {}, {}, {}

        def qprod(m, t, zeros):
            pq[m - 1, t] = _dg(_bf(_paced(_get(lq_v, m - 1, 0, 32), zeros)), _bf(tok_words(ti, m - 1, 8 * t, 8)), 1, 1)

        def attn(blk, t, zeros):
            for p in range(8):
                a_v[blk][t][64 * p:64 * p + 64, :] = _dg(
                    _bf(_get(kvm_v, 8 * (blk // 2) + p, 0, 4, [0])), get_phi(blk, p, t, zero, zeros[p::8]), 1, 0)

        def oprod(m, c, zeros):
            if m not in ot:
                at = []
                for t in range(2):
                    rows = pl.ds(pl.multiple_of(zero, 8), _HD)
                    at.append(_operand(_LEFT[m - 1], lambda k: a_v[(0, 2, 1, 3)[k]][t][rows, :]).astype(_BF).T)
                ot[m] = jnp.concatenate(at, axis=0)
            w = weight_words(wo_v, lo_v, _B_SLOT[m - 1], c)
            po[m - 1, c] = _dg(ot[m], _bf(jnp.concatenate([_paced(w[0:64], zeros), w[64:]], axis=0)), 1, 0)

        def feat_piece(blk, t, p):
            def run():
                ep, en, sp, sn = _dual_exp(_mix(blk, lambda m: pq[m, t][64 * p:64 * p + 64]))
                z = z_v[8 * (blk // 2) + p]
                dp, dn = _pair_reduce(ep * z[0:64], jnp.add), _pair_reduce(en * z[64:128], jnp.add)
                inv = _recip(dp * sn + sp * (dn + 1e-6 * sn))
                return put_phi(blk, p, t, zero, ep * _rep8(sn * inv), en * _rep8(sp * inv))
            return run

        def hidden_piece(c, half):
            def run():
                for k, w in enumerate((wg_v, wu_v)):
                    acc = f_v[2 * c + k + zero] if half else None
                    f_v[2 * c + k] = _matvec(w.at[i], xc_v, c, 32 * half, 32 * half + 32, acc)
                return pltpu.bitcast(f_v[22 + zero], _I32)
            return run

        def act_piece(c):
            def run():
                hg, hu = (jnp.sum(f_v[2 * c + k + zero], axis=0, keepdims=True) for k in range(2))
                hc_v[128 * c:128 * c + 128, :] = _col_bcast(hg * jax.nn.sigmoid(hg) * hu)
            return run

        def down_piece(c, half):
            def run():
                for cc in (c, c + 1):
                    f_v[14 + cc] = _matvec(wd_v.at[i], hc_v, cc, 28 * half, 28 * half + 28, f_v[14 + cc + zero])
                return pltpu.bitcast(f_v[22 + zero], _I32)
            return run

        def emit_piece(blk, u, c):
            def run():
                h, d = blk // 2, blk % 2
                g = g_v[4 * ti + 2 * h + u]
                tok = jax.lax.broadcasted_iota(_I32, (128, 128), 0) + (ti * _T + _HT * h + 128 * u)
                o = []
                for cc in (c, c + 1):
                    y = jnp.sum(f_v[14 + 4 * d + cc + zero], axis=0, keepdims=True) * r_sel
                    b = _bf(x_blk(ti, 2 * d + h)[64 * u:64 * u + 64, 128 * cc:128 * cc + 128]).astype(_F32)
                    b = b + jnp.where(tok == idx, y, 0.0)
                    o.append(g * _mix(blk, lambda m: po[m, cc][128 * u:128 * u + 128]) + (1.0 - g) * b)
                out_v[blk][ti, 128 * u:128 * u + 128, 128 * c:128 * c + 256] = jnp.concatenate(o, axis=1).astype(_BF)
                if (u, c) == (1, 2):
                    cp_o(ti, blk).start()
                    out_v[blk][_NT, 16:32, 0:128] = jnp.zeros((16, 128), _BF)
                return pltpu.bitcast(out_v[blk][_NT + zero, 0:16, 0:128], _I32)
            return run

        def pieces(name):
            if name[0] == "h":
                return [hidden_piece(c, int(name[1])) for c in range(_FC // 128)]
            if name == "a":
                return [act_piece(c) for c in range(_FC // 128)]
            if name == "d":
                return [down_piece(c, half) for c in (4, 6, 0, 2) for half in range(2)]
            if name[0] == "e":
                return [emit_piece(int(name[1]), u, c) for c in (0, 2) for u in range(2)]
            return [feat_piece(int(name[1]), t, p) for t in ([int(name[2])] if name[2:] else range(2))
                    for p in range(8)]

        _play(_PHASE2, {"q": (qprod, 2), "o": (oprod, 4), "g": (attn, 2)}, pieces)

    pl.loop(0, _NT)(phase2)
    for t in range(_NT):
        for blk in range(4):
            cp_o(t, blk).wait()


@jax.jit
def pallas_gated_mix__linear_kernel_hedgehog__moe_arch_mod__prompt_kernel(
    A_x: jax.Array,
    A_wqkv: jax.Array,
    A_w_phi: jax.Array,
    A_wo: jax.Array,
    B_x: jax.Array,
    B_w_r: jax.Array,
    B_w_gate: jax.Array,
    B_w_up: jax.Array,
    B_w_down: jax.Array,
    gate_w: jax.Array,
):
    del B_x
    hbm = pl.BlockSpec(memory_space=pl.ANY)
    dma = pltpu.SemaphoreType.DMA
    out = pl.pallas_call(
        _kernel,
        out_shape=jax.ShapeDtypeStruct((_S, _D), _BF),
        in_specs=[hbm] * 9,
        out_specs=hbm,
        scratch_shapes=[
            pltpu.VMEM((_NT, _HT, _D), _I32),
            pltpu.VMEM((2, _HD, _D), _I32),
            pltpu.VMEM((_NT, _HD, _FC), _I32),
            pltpu.VMEM((_NT, _HD, _FC), _I32),
            pltpu.VMEM((_NT, _FC // 2, _D), _I32),
            pltpu.VMEM((_H, _DH, _DH), _BF),
            pltpu.VMEM((_D,), _BF),
            pltpu.VMEM((_D,), _BF),
            pltpu.VMEM((4, 256, _HD), _I32),
            pltpu.VMEM((4, 256, _HD), _I32),
            pltpu.VMEM((1, 8, 8, 16, 128), _BF),
            pltpu.VMEM((7, 32, 4, 16, 128), _BF),
            pltpu.VMEM((7, 32, 4, 16, 128), _BF),
            [pltpu.VMEM((8, 16, 2, 16, 128), _BF)] * 7,
            pltpu.VMEM((6, 32, 4, 16, 128), _BF),
            [pltpu.VMEM((_NT, 16, 4, 16, 128), _BF)] * 5,
            [pltpu.VMEM((7 * _NT + 1, 8, 2, 16, 128), _BF)] * 7,
            [pltpu.VMEM((17, 8, 1, 16, 128), _BF)] * 4,
            [[pltpu.VMEM((_HD, 128), _F32)] * 2] * 4,
            pltpu.VMEM((_NP, 64, 128), _F32),
            pltpu.VMEM((_NP + 1, 128, 128), _F32),
            pltpu.VMEM((_NP, 4, 1, 16, 128), _BF),
            pltpu.VMEM((_S // 128 + 1, 128, 128), _F32),
            pltpu.VMEM((8, 128), _F32),
            pltpu.VMEM((2, 8, 128), _I32),
            pltpu.VMEM((23, 8, 128), _F32),
            pltpu.VMEM((_D + 8, 128), _F32),
            pltpu.VMEM((_FC, 128), _F32),
            [pltpu.VMEM((_NT + 1, _HT, _HD), _BF)] * 4,
            dma((_NT,)), dma((2,)), dma((2,)), dma((4,)), dma((3,)),
            dma((_NT,)), dma((_NT,)), dma((_NT,)), dma((4 * _NT,)),
        ],
        compiler_params=pltpu.CompilerParams(vmem_limit_bytes=120 * 1024 * 1024,
                                             disable_bounds_checks=True),
    )(A_x.reshape(_S, _D), A_wqkv, A_w_phi, A_wo, B_w_r, B_w_gate, B_w_up, B_w_down, gate_w)
    return out.reshape(1, _S, _D)
```

```python
import jax
import jax.numpy as jnp
import jax.experimental.pallas as pl
import jax.experimental.pallas.tpu as pltpu

_BF = jnp.bfloat16
_F32 = jnp.float32
_I32 = jnp.int32
_LOG2E = 1.4426950408889634

_S, _D, _H, _DH, _F = 2048, 1024, 32, 32, 3584
_T = 512
_HT = _T // 2
_HD = _D // 2
_NT = _S // _T
_FC = _F // _NT
_NP = _H // 2

_LEFT = ((0, 1, 3), (2, 1, 3), (0,), (3,), (0, 1, 1), (2, -1, 0), (1, -1, 3))
_RIGHT = ((0, 1, 3), (0,), (1, -1, 3), (2, -1, 0), (3,), (0, 1, 1), (2, 1, 3))
_A_SLOT = (4, 5, 0, 3, 6, 7, 8)
_B_SLOT = (4, 0, 5, 6, 3, 7, 8)
_ORDER = (1, 4, 3, 2, 0, 6, 5)

_FIRST = ("+r3 +r5 +r4 +r2 +s ! W0 +a3 ! v3.0:2 +a5 v3.1:4 +r1 v3.2:4 v3.3:3 v3.4:3 v3.5:2 v3.6:1 "
          "v5:2,2,1,1,1,1,1 W1 +a4 ! +a2 +a1 v4:3,5,2,2,2,3,2 v2:3,3,2,2,2,2,2 +a7 +r7 v1:4,4,4,3,3,3,3 "
          "+r6 +a6 v7:4,4,4,3,1,3,3 W2 k2:1,0 k5 k4 +f2 k3:6,6 k1:5,5 +f1 k7:7,8 +f0 k6:7,6 "
          "v6:2,1,1,1,1,1,1 +f3 g0 g1.0 g2:5,5,5,5 g1.2 g1.1 g1.3 g3")
_PHASE1 = ("+r2 +r3 +r4 +r6 +r5 +r7 +r1 k5.1:7 +o k2:8,8 v2:2,2,2,2,2,1,1 k5.0:7 +f2 v5:5,5,5,5,5,5,4 +f1 "
           "k4 k3.0:8 +s k3.1:8 v4:2,2,2,2,2,2,2 v3:1,1,1,1,1,1,1 k7 g2 k1:6,2 +f0 g1.0 g1.1 g1.3 g1.2 "
           "v7:3,4,3,3,3,3,3 v1:3,1,3,3,2,3,2 k6:12,14 +f3 v6:2,0,2,2,2,2,2 g0:1,0,2,1 g3:1,0,2,1")
_PHASE2 = ("+h0 +h1 q4.1:2 q4.0:4 q7.1:1 q1:1,2 q7.0:3 q5.0 +f0 q5.1:2 q3:7,6 q2.0:9 g0 +f1 q2.1:9 +f2 "
           "q6:6,6 +f3 +a g1 o3:2,3,3,3 ! g2 o6:4,3,3,3 g3 +d o5:2,2,2,4 +e1 o1.0:2 o2:1,1,1,1 o4:2,2,2,2 "
           "+e2 o1.2:1 o1.1 o1.3:2 +e3 o7:0,1,3,1 +e0 !")


def _dg(a, b, ca, cb):
    return jax.lax.dot_general(a, b, (((ca,), (cb,)), ((), ())), preferred_element_type=_F32)


def _bf(w):
    return pltpu.bitcast(w, _BF)


def _put(ref, g, c, v):
    for j in range(v.shape[1] // 128):
        ref[pl.ds(g, v.shape[0] // 16), c + j] = v[:, 128 * j:128 * j + 128].reshape(-1, 16, 128).astype(_BF)


def _get(ref, k, g, n, tiles=range(4)):
    words = ref.bitcast(_I32)
    return jnp.concatenate([words[k, pl.ds(g, n), c].reshape(8 * n, 128) for c in tiles], axis=1)


def _a_sums(a11, a12, a21, a22):
    return (a11 + a22, a21 + a22, a11 + a12, a21 - a11, a12 - a22)


def _b_sums(b11, b12, b21, b22):
    return (b11 + b22, b12 - b22, b21 - b11, b11 + b12, b21 + b22)


def _operand(rule, block):
    if len(rule) == 1:
        return block(rule[0])
    return block(rule[0]) + block(rule[2]) if rule[1] > 0 else block(rule[0]) - block(rule[2])


def _put_operands(side, m, block, ref, base, g):
    sub = [_operand(side[m], lambda k: block(k, j)) for j in range(4)]
    for n in range(7):
        _put(ref.at[base + n], g, 0, _operand(side[n], lambda j: sub[j]))
    return sub


def _mix(c, m):
    if c == 0:
        return m(0) + m(3) - m(4) + m(6)
    if c == 1:
        return m(2) + m(4)
    if c == 2:
        return m(1) + m(3)
    return m(0) - m(1) + m(2) + m(5)


def _paced(w, zeros):
    if not zeros:
        return w
    groups = w.shape[0] // 8
    first = [w[8 * g:8 * g + 8, 0:128] for g in range(groups)]
    for j, z in enumerate(zeros):
        g = max((j + 1) * groups // len(zeros) - 1, 0)
        first[g] = first[g] | z
    first = jnp.concatenate(first, axis=0)
    return first if w.shape[1] == 128 else jnp.concatenate([first, w[:, 128:]], axis=1)


def _play(program, steps, pieces):
    queue = []
    for word in program.split():
        if word == "!":
            while queue:
                queue.pop(0)()
        elif word[0] == "+":
            queue.extend(pieces(word[1:]))
        else:
            name, _, counts = word.partition(":")
            name, _, tile = name.partition(".")
            step, tiles = steps[name[0]]
            tiles = [int(tile)] if tile else range(tiles)
            counts = [int(n) for n in counts.split(",")] if counts else [0] * len(tiles)
            for t, n in zip(tiles, counts):
                step(int(name[1:]), t, [queue.pop(0)() for _ in range(min(n, len(queue)))])
    assert not queue


def _recip(v):
    r = pl.reciprocal(v, approx=True)
    return r * (2.0 - v * r)


def _pair_reduce(v, op):
    r = v[0:8]
    for j in range(1, 8):
        r = op(r, v[8 * j:8 * j + 8])
    r = op(r, pltpu.roll(r, 2, 0))
    return op(r, pltpu.roll(r, 4, 0))


def _rep8(v):
    return jnp.concatenate([v] * 8, axis=0)


def _dual_exp(p):
    ep = jnp.exp2(p - _rep8(_pair_reduce(p, jnp.maximum)))
    en = jnp.exp2(_rep8(_pair_reduce(p, jnp.minimum)) - p)
    return ep, en, _pair_reduce(ep, jnp.add), _pair_reduce(en, jnp.add)


def _col_bcast(row):
    return jnp.broadcast_to(row, (128, row.shape[1])).T


def _matvec(w_ref, col_ref, c, j0, j1, acc=None):
    for j in range(j0, j1):
        t = _bf(w_ref[8 * j:8 * j + 8, 128 * c:128 * c + 128]).astype(_F32) * col_ref[16 * j:16 * j + 16, :]
        acc = t[0:8] if acc is None else acc + t[0:8]
        acc = acc + t[8:16]
    return acc


def _kernel(x_hbm, wqkv_hbm, wphi_hbm, wo_hbm, wr_hbm, wg_hbm, wu_hbm, wd_hbm, gw_hbm,
            out_hbm,
            x_v, w_v, wg_v, wu_v, wd_v, wphi_v, wr_v, gw_v,
            wv_v, wo_v, lm_v, lk_v, lq_v, lv_v, lo_v, r_v, r2_v, phi_v, a_v,
            kv_v, z_v, kvm_v, g_v, top_v, arg_v, f_v, xc_v, hc_v, out_v,
            sem_x, sem_w, sem_v, sem_wo, sem_s, sem_g, sem_u, sem_d, sem_o):
    x_hbm, wqkv_hbm, wo_hbm, wg_hbm, wu_hbm, wd_hbm = (
        r.bitcast(_I32) for r in (x_hbm, wqkv_hbm, wo_hbm, wg_hbm, wu_hbm, wd_hbm))

    def cp_x(i):
        return pltpu.make_async_copy(x_hbm.at[pl.ds(i * _HT, _HT)], x_v.at[i], sem_x.at[i])

    def cp_w(j):
        return pltpu.make_async_copy(wqkv_hbm.at[:, pl.ds(j * _D, _D)], w_v.at[j], sem_w.at[j])

    def cp_v(k):
        return pltpu.make_async_copy(wqkv_hbm.at[pl.ds(256 * (k % 2), 256), pl.ds(2 * _D + _HD * (k // 2), _HD)],
                                     wv_v.at[k], sem_v.at[k])

    def cp_wo(k):
        return pltpu.make_async_copy(wo_hbm.at[pl.ds(256 * (k // 2), 256), pl.ds(_HD * (k % 2), _HD)],
                                     wo_v.at[k], sem_wo.at[k])

    cp_small = [pltpu.make_async_copy(src, dst, sem_s.at[j]) for j, (src, dst) in enumerate(
        ((wphi_hbm, wphi_v), (wr_hbm, wr_v), (gw_hbm, gw_v)))]

    def cp_ffn(i):
        cols = pl.ds(i * _FC, _FC)
        return (pltpu.make_async_copy(wg_hbm.at[:, cols], wg_v.at[i], sem_g.at[i]),
                pltpu.make_async_copy(wu_hbm.at[:, cols], wu_v.at[i], sem_u.at[i]),
                pltpu.make_async_copy(wd_hbm.at[pl.ds(i * (_FC // 2), _FC // 2)], wd_v.at[i], sem_d.at[i]))

    def cp_o(t, blk):
        return pltpu.make_async_copy(
            out_v[blk].at[t], out_hbm.at[pl.ds(t * _T + _HT * (blk // 2), _HT), pl.ds(_HD * (blk % 2), _HD)],
            sem_o.at[4 * t + blk])

    for cp in cp_small:
        cp.start()
    cp_x(0).start()
    cp_v(0).start()
    cp_v(1).start()

    kv_v[...] = jnp.zeros_like(kv_v)
    z_v[...] = jnp.zeros_like(z_v)
    f_v[...] = jnp.zeros_like(f_v)
    xc_v[_D:, :] = jnp.zeros((8, 128), _F32)
    top_v[...] = jnp.full((8, 128), -jnp.inf, _F32)
    arg_v[...] = jnp.zeros_like(arg_v)
    g_v[_S // 128, 0:8, :] = jnp.zeros((8, 128), _F32)
    for ref in (*r2_v, *lv_v, lo_v, *phi_v):
        ref[ref.shape[0] - 1, 0, 0] = jnp.zeros((16, 128), _BF)
    for ref in out_v:
        ref[_NT, 0:16, 0:128] = jnp.zeros((16, 128), _BF)

    for cp in cp_small:
        cp.wait()
    rows = jax.lax.broadcasted_iota(_I32, (128, _DH), 0)
    cols = jax.lax.broadcasted_iota(_I32, (128, _DH), 1)
    sel = jnp.where(((rows >> 1) & 31) == cols, 1.0, 0.0).astype(_BF)
    full = _dg(sel, wphi_v[...].reshape(_H * _DH, _DH), 1, 1)
    rows = jax.lax.broadcasted_iota(_I32, (128, _D), 0)
    cols = jax.lax.broadcasted_iota(_I32, (128, _D), 1)
    keep = ((cols >> 5) & 3) == 2 * (rows >> 6) + (rows & 1)
    _put(lm_v.at[0], 0, 0, jnp.where(keep, full, 0.0))

    def fold(j, l_v, queue=()):
        for g in range(4):
            for d in range(2):
                blk = []
                for gg in (g, g + 4):
                    c = slice(128 * gg, 128 * gg + 128)
                    for dd in (d, d + 2):
                        w = _paced(w_v[j, 128 * dd:128 * dd + 128, c], [queue.pop(0)() for _ in queue[:1]])
                        blk.append(_dg(_bf(_get(lm_v, 0, 0, 8, [gg])), _bf(w), 1, 1) * _LOG2E)
                blk += _a_sums(*blk)
                for m in range(7):
                    _put(l_v.at[m], 8 * g, 2 * d, blk[_A_SLOT[m]])

    def out_piece(g, c):
        def run():
            r = pl.ds(pl.multiple_of(8 * g, 8), 8)
            sums = _b_sums(*[_bf(wo_v.at[k][r, 128 * c:128 * c + 256]).astype(_F32) for k in range(4)])
            for k in range(5):
                _put(lo_v.at[k], g, c, sums[k])
            return _get(lo_v, 5, 0, 1, [0])
        return run

    def x_blk(i, k):
        return x_v.at[i, 128 * (k % 2):128 * (k % 2) + 128, _HD * (k // 2):_HD * (k // 2) + _HD]

    def tok_words(i, m, g=0, n=16):
        k = _B_SLOT[m]
        return x_blk(i, k)[8 * g:8 * (g + n), :] if k < 4 else _get(r_v[k - 4], i, g, n)

    def put_phi(blk, p, t, zero, pos, neg):
        _put(phi_v[blk].at[2 * p + t], 0, 0, jnp.concatenate([pos, neg], axis=0))
        return _get(phi_v[blk], 16 + zero, 0, 1, [0])

    def get_phi(blk, p, t, zero, zeros=()):
        return _bf(_paced(_get(phi_v[blk], 2 * p + t + zero, 0, 8, [0]), zeros))

    def phase1(i, zero, program):
        pk, pv, part = {}, {}, {}

        def kprod(m, t, zeros):
            pk[m - 1, t] = _dg(_bf(_paced(_get(lk_v, m - 1, 0, 32), zeros)),
                               _bf(tok_words(i, m - 1, 8 * t, 8)), 1, 1)

        def vprod(m, s, zeros):
            n = _ORDER[s]
            part[m, n] = _dg(_bf(_paced(_get(r2_v[m - 1], 7 * i + n, 0, 8, range(2)), zeros)),
                             _bf(_get(lv_v[m - 1], n, 0, 16, range(2))), 1, 0)
            if s == 6:
                for o in range(2):
                    val = jnp.concatenate([_mix(2 * o + t, lambda n: part[m, n]) for t in range(2)], axis=0)
                    pv[m - 1, 2 * o], pv[m - 1, 2 * o + 1] = val[:, :128], val[:, 128:]

        def kv(blk, c, zeros):
            vt = _mix(blk, lambda m: pv[m, c]).astype(_BF).T
            for h in range(2):
                p = 2 * c + h
                phi = jnp.concatenate([get_phi(blk, p, 0, zero, zeros[h::2]), get_phi(blk, p, 1, zero)], axis=1)
                kv_v[8 * (blk // 2) + p] += _dg(vt[64 * h:64 * h + 64], phi, 1, 1)

        def wait(j, t, zeros):
            for cp in (cp_v(2 * j), cp_v(2 * j + 1)) if j < 2 else (cp_w(1),):
                cp.wait()
            if j == 0:
                cp_w(1).start()
            elif j == 1:
                cp_x(1).start()
                for k in range(4):
                    cp_wo(k).start()
            else:
                for k in range(2, _NT):
                    cp_x(k).start()
                cp_w(0).start()
                for k in range(_NT):
                    for cp in cp_ffn(k):
                        cp.start()
                fold(1, lk_v)

        def token_piece(m, g):
            def run():
                def block(k, j):
                    r = 64 * (j % 2) + 8 * g
                    return _bf(x_blk(i, k)[r:r + 8, 256 * (j // 2):256 * (j // 2) + 256]).astype(_F32)
                sub = _put_operands(_RIGHT, m, block, r2_v[m], 7 * (i + zero), g)
                if _B_SLOT[m] > 3:
                    for j in range(4):
                        _put(r_v[_B_SLOT[m] - 4].at[i + zero], 8 * (j % 2) + g, 2 * (j // 2), sub[j])
                return _get(r2_v[m], 7 * _NT, 0, 1, [0])
            return run

        def value_piece(m, g):
            def run():
                def block(k, j):
                    r = 128 * (j % 2) + 8 * g
                    return _bf(wv_v[k, r:r + 8, 256 * (j // 2):256 * (j // 2) + 256]).astype(_F32)
                _put_operands(_LEFT, m, block, lv_v[m], 0, g)
                return _get(lv_v[m], 7 + zero, 0, 1, [0])
            return run

        def feat_piece(blk, t, p):
            def run():
                ep, en, sp, sn = _dual_exp(_mix(blk, lambda m: pk[m, t][64 * p:64 * p + 64]))
                ep, en = ep * _rep8(_recip(sp)), en * _rep8(_recip(sn))
                z_v[8 * (blk // 2) + p] += jnp.concatenate([ep, en], axis=0)
                return put_phi(blk, p, t, zero, ep, en)
            return run

        def score_piece(c):
            def run():
                xh = _bf(x_v[i, 16 * c:16 * c + 16, :]).astype(_F32)
                wr = wr_v[...].astype(_F32).reshape(1, _D)
                gw = gw_v[...].astype(_F32).reshape(1, _D)
                g = jax.nn.sigmoid(jnp.sum(xh * gw, axis=1, keepdims=True))
                g_v[4 * i + c // 4, 32 * (c % 4):32 * (c % 4) + 32, :] = jnp.broadcast_to(g, (32, 128))
                sc = jnp.sum(xh * wr, axis=1, keepdims=True).astype(_BF).astype(_F32)
                best, bidx = top_v[...], arg_v[0]
                for j in range(4):
                    rj = sc[8 * j:8 * j + 8]
                    upd = rj > best
                    best = jnp.where(upd, rj, best)
                    bidx = jnp.where(upd, i * _T + 32 * c + 8 * j, bidx)
                top_v[...] = best
                arg_v[0] = bidx
                return arg_v[1 + zero] | pltpu.bitcast(g_v[_S // 128 + zero, 0:8, :], _I32)
            return run

        def pieces(name):
            if name[0] == "r":
                return [token_piece(int(name[1]) - 1, g) for g in range(8)]
            if name == "s":
                return [score_piece(c) for c in range(16)]
            if name[0] == "a":
                return [value_piece(int(name[1]) - 1, g) for g in range(16)]
            if name == "o":
                start = jnp.minimum(11 * (i - 1), 32 - 11)
                return [out_piece(start + j // 2, 2 * (j % 2)) for j in range(22)]
            return [feat_piece(int(name[1]), t, p) for t in ([int(name[2])] if name[2:] else range(2))
                    for p in range(8)]

        _play(program, {"k": (kprod, 2), "v": (vprod, 7), "g": (kv, 4), "W": (wait, 1)}, pieces)

    def later_tile(i):
        cp_x(i).wait()
        phase1(i, i >> 8, _PHASE1)

    zero = arg_v[1, 0, 0]
    cp_x(0).wait()
    cp_v(2).start()
    cp_v(3).start()
    phase1(0, zero, _FIRST)
    for k in range(4):
        cp_wo(k).wait()
    pl.loop(1, _NT)(later_tile)

    cp_w(0).wait()
    best = top_v[...]
    bidx = arg_v[0] + jax.lax.broadcasted_iota(_I32, (8, 128), 0)
    rmax = jnp.max(best, axis=0, keepdims=True)
    idx = jnp.min(jnp.where(best == rmax, bidx, _S - 1))
    r_sel = jax.nn.sigmoid(rmax)
    tsel = idx // _T
    rsel = idx - tsel * _T
    grp = _bf(x_v[tsel, pl.ds(pl.multiple_of((rsel >> 4) << 3, 8), 8), :]).astype(_F32)
    hit = jax.lax.broadcasted_iota(_I32, (16, _D), 0) == (rsel & 15)
    x_sel = jnp.sum(jnp.where(hit, grp, 0.0), axis=0, keepdims=True)

    def state_piece(p):
        def run():
            rows = jax.lax.broadcasted_iota(_I32, (64, 128), 0)
            cols = jax.lax.broadcasted_iota(_I32, (64, 128), 1)
            _put(kvm_v.at[p], 0, 0, jnp.where((rows >> 5) == (cols & 1), kv_v[p], 0.0))
            z_v[p] = jnp.broadcast_to(jnp.sum(z_v[p], axis=1, keepdims=True), (128, 128))
            return pltpu.bitcast(z_v[_NP + zero, 0:8, :], _I32)
        return run

    def column_piece(c):
        def run():
            xc_v[128 * c:128 * c + 128, :] = _col_bcast(x_sel[:, 128 * c:128 * c + 128])
            return pltpu.bitcast(xc_v[pl.ds(pl.multiple_of(_D + zero, 8), 8), :], _I32)
        return run

    fold(0, lq_v, [state_piece(p) for p in range(_NP)] + [column_piece(c) for c in range(8)])

    def phase2(i):
        ti = (tsel + 1 + i) % _NT
        for cp in cp_ffn(i):
            cp.wait()
        zero = i >> 8
        pq, po, ot = {}, {}, {}

        def qprod(m, t, zeros):
            pq[m - 1, t] = _dg(_bf(_paced(_get(lq_v, m - 1, 0, 32), zeros)),
                               _bf(tok_words(ti, m - 1, 8 * t, 8)), 1, 1)

        def attn(blk, t, zeros):
            for p in range(8):
                a_v[blk][t][64 * p:64 * p + 64, :] = _dg(
                    _bf(_get(kvm_v, 8 * (blk // 2) + p, 0, 4, [0])), get_phi(blk, p, t, zero, zeros[p::8]), 1, 0)

        def oprod(m, c, zeros):
            if m not in ot:
                at = []
                for t in range(2):
                    rows = pl.ds(pl.multiple_of(zero, 8), _HD)
                    at.append(_operand(_LEFT[m - 1], lambda k: a_v[(0, 2, 1, 3)[k]][t][rows, :]).astype(_BF).T)
                ot[m] = jnp.concatenate(at, axis=0)
            k = _B_SLOT[m - 1]
            w = wo_v[k, :, 128 * c:128 * c + 128] if k < 4 else _get(lo_v, k - 4, 0, 32, [c])
            po[m - 1, c] = _dg(ot[m], _bf(jnp.concatenate([_paced(w[0:64], zeros), w[64:]], axis=0)), 1, 0)

        def feat_piece(blk, t, p):
            def run():
                ep, en, sp, sn = _dual_exp(_mix(blk, lambda m: pq[m, t][64 * p:64 * p + 64]))
                z = z_v[8 * (blk // 2) + p]
                dp, dn = _pair_reduce(ep * z[0:64], jnp.add), _pair_reduce(en * z[64:128], jnp.add)
                inv = _recip(dp * sn + sp * (dn + 1e-6 * sn))
                return put_phi(blk, p, t, zero, ep * _rep8(sn * inv), en * _rep8(sp * inv))
            return run

        def hidden_piece(c, half):
            def run():
                for k, w in enumerate((wg_v, wu_v)):
                    acc = f_v[2 * c + k + zero] if half else None
                    f_v[2 * c + k] = _matvec(w.at[i], xc_v, c, 32 * half, 32 * half + 32, acc)
                return pltpu.bitcast(f_v[22 + zero], _I32)
            return run

        def act_piece(c):
            def run():
                hg, hu = (jnp.sum(f_v[2 * c + k + zero], axis=0, keepdims=True) for k in range(2))
                hc_v[128 * c:128 * c + 128, :] = _col_bcast(hg * jax.nn.sigmoid(hg) * hu)
            return run

        def down_piece(c, half):
            def run():
                for cc in (c, c + 1):
                    f_v[14 + cc] = _matvec(wd_v.at[i], hc_v, cc, 28 * half, 28 * half + 28, f_v[14 + cc + zero])
                return pltpu.bitcast(f_v[22 + zero], _I32)
            return run

        def emit_piece(blk, u, c):
            def run():
                h, d = blk // 2, blk % 2
                g = g_v[4 * ti + 2 * h + u]
                tok = jax.lax.broadcasted_iota(_I32, (128, 128), 0) + (ti * _T + _HT * h + 128 * u)
                o = []
                for cc in (c, c + 1):
                    y = jnp.sum(f_v[14 + 4 * d + cc + zero], axis=0, keepdims=True) * r_sel
                    b = _bf(x_blk(ti, 2 * d + h)[64 * u:64 * u + 64, 128 * cc:128 * cc + 128]).astype(_F32)
                    b = b + jnp.where(tok == idx, y, 0.0)
                    o.append(g * _mix(blk, lambda m: po[m, cc][128 * u:128 * u + 128]) + (1.0 - g) * b)
                out_v[blk][ti, 128 * u:128 * u + 128, 128 * c:128 * c + 256] = (
                    jnp.concatenate(o, axis=1).astype(_BF))
                if (u, c) == (1, 2):
                    cp_o(ti, blk).start()
                    out_v[blk][_NT, 16:32, 0:128] = jnp.zeros((16, 128), _BF)
                return pltpu.bitcast(out_v[blk][_NT + zero, 0:16, 0:128], _I32)
            return run

        def pieces(name):
            if name[0] == "h":
                return [hidden_piece(c, int(name[1])) for c in range(_FC // 128)]
            if name == "a":
                return [act_piece(c) for c in range(_FC // 128)]
            if name == "d":
                return [down_piece(c, half) for c in (4, 6, 0, 2) for half in range(2)]
            if name[0] == "e":
                return [emit_piece(int(name[1]), u, c) for c in (0, 2) for u in range(2)]
            return [feat_piece(int(name[1]), t, p) for t in ([int(name[2])] if name[2:] else range(2))
                    for p in range(8)]

        _play(_PHASE2, {"q": (qprod, 2), "o": (oprod, 4), "g": (attn, 2)}, pieces)

    pl.loop(0, _NT)(phase2)
    for t in range(_NT):
        for blk in range(4):
            cp_o(t, blk).wait()


@jax.jit
def pallas_gated_mix__linear_kernel_hedgehog__moe_arch_mod__prompt_kernel(
    A_x: jax.Array,
    A_wqkv: jax.Array,
    A_w_phi: jax.Array,
    A_wo: jax.Array,
    B_x: jax.Array,
    B_w_r: jax.Array,
    B_w_gate: jax.Array,
    B_w_up: jax.Array,
    B_w_down: jax.Array,
    gate_w: jax.Array,
):
    del B_x
    hbm = pl.BlockSpec(memory_space=pl.ANY)
    dma = pltpu.SemaphoreType.DMA
    out = pl.pallas_call(
        _kernel,
        out_shape=jax.ShapeDtypeStruct((_S, _D), _BF),
        in_specs=[hbm] * 9,
        out_specs=hbm,
        scratch_shapes=[
            pltpu.VMEM((_NT, _HT, _D), _I32),
            pltpu.VMEM((2, _HD, _D), _I32),
            pltpu.VMEM((_NT, _HD, _FC), _I32),
            pltpu.VMEM((_NT, _HD, _FC), _I32),
            pltpu.VMEM((_NT, _FC // 2, _D), _I32),
            pltpu.VMEM((_H, _DH, _DH), _BF),
            pltpu.VMEM((_D,), _BF),
            pltpu.VMEM((_D,), _BF),
            pltpu.VMEM((4, 256, _HD), _I32),
            pltpu.VMEM((4, 256, _HD), _I32),
            pltpu.VMEM((1, 8, 8, 16, 128), _BF),
            pltpu.VMEM((7, 32, 4, 16, 128), _BF),
            pltpu.VMEM((7, 32, 4, 16, 128), _BF),
            [pltpu.VMEM((8, 16, 2, 16, 128), _BF)] * 7,
            pltpu.VMEM((6, 32, 4, 16, 128), _BF),
            [pltpu.VMEM((_NT, 16, 4, 16, 128), _BF)] * 5,
            [pltpu.VMEM((7 * _NT + 1, 8, 2, 16, 128), _BF)] * 7,
            [pltpu.VMEM((17, 8, 1, 16, 128), _BF)] * 4,
            [[pltpu.VMEM((_HD, 128), _F32)] * 2] * 4,
            pltpu.VMEM((_NP, 64, 128), _F32),
            pltpu.VMEM((_NP + 1, 128, 128), _F32),
            pltpu.VMEM((_NP, 4, 1, 16, 128), _BF),
            pltpu.VMEM((_S // 128 + 1, 128, 128), _F32),
            pltpu.VMEM((8, 128), _F32),
            pltpu.VMEM((2, 8, 128), _I32),
            pltpu.VMEM((23, 8, 128), _F32),
            pltpu.VMEM((_D + 8, 128), _F32),
            pltpu.VMEM((_FC, 128), _F32),
            [pltpu.VMEM((_NT + 1, _HT, _HD), _BF)] * 4,
            dma((_NT,)), dma((2,)), dma((4,)), dma((4,)), dma((3,)),
            dma((_NT,)), dma((_NT,)), dma((_NT,)), dma((4 * _NT,)),
        ],
        compiler_params=pltpu.CompilerParams(vmem_limit_bytes=100 * 1024 * 1024),
    )(A_x.reshape(_S, _D), A_wqkv, A_w_phi, A_wo, B_w_r, B_w_gate, B_w_up, B_w_down, gate_w)
    return out.reshape(1, _S, _D)
```

```python
import jax
import jax.numpy as jnp
import jax.experimental.pallas as pl
import jax.experimental.pallas.tpu as pltpu

_BF = jnp.bfloat16
_F32 = jnp.float32
_I32 = jnp.int32
_LOG2E = 1.4426950408889634

_S, _D, _H, _DH, _F = 2048, 1024, 32, 32, 3584
_T = 512
_HT = _T // 2
_HD = _D // 2
_NT = _S // _T
_FC = _F // _NT
_NP = _H // 2

_LEFT = ((0, 1, 3), (2, 1, 3), (0,), (3,), (0, 1, 1), (2, -1, 0), (1, -1, 3))
_RIGHT = ((0, 1, 3), (0,), (1, -1, 3), (2, -1, 0), (3,), (0, 1, 1), (2, 1, 3))
_A_SLOT = (4, 5, 0, 3, 6, 7, 8)
_B_SLOT = (4, 0, 5, 6, 3, 7, 8)
_ORDER = (1, 4, 3, 2, 0, 6, 5)

_FIRST = ("+r2 +r3 +r5 +r4 +r1 +r7 +r6 +s ! W0 +a3 +a5 ! v3 v5 W1 +m +a4 ! +a2 +a1 v4:3,5,2,2,2,3,2 +a7 "
          "v2:4,4,3,3,3,3,3 v1:3,3,2,2,2,2,2 +a6 v7:5,5,4,4,4,3,4 W2 k2 k5 k4 +f2 k3:3,3 k1:5,5 +f1 k7:5,8 "
          "+f0 k6:7,6 v6:2,1,0,1,1,2,1 +f3 g0 g1.2 g1.0 g2:5,5,5,6 g1.3 g1.1 g3:0,0,1,0")
_PHASE1 = ("+r2 +r3 +r4 +r6 +r5 +r7 +r1 k5.1:7 +o k2:8,8 v2:2,2,2,2,2,1,1 k5.0:7 +f2 v5:5,5,5,5,5,5,4 +f1 "
           "k4 k3.0:8 +s k3.1:8 v4:2,2,2,2,2,2,2 v3:1,1,1,1,1,1,1 k7 g2 k1:6,2 +f0 g1.0 g1.1 g1.3 g1.2 "
           "v7:3,4,3,3,3,3,3 v1:3,1,3,3,2,3,2 k6:12,14 +f3 v6:2,0,2,2,2,2,2 g0:1,0,2,1 g3:1,0,2,1")
_PHASE2 = ("+h0 +h1 q4.1:2 q4.0:4 q7.1:1 q1:1,2 q7.0:3 q5.0 +f0 q5.1:2 q3:7,6 q2.0:9 g0 +f1 q2.1:9 +f2 "
           "q6:6,6 +f3 +a g1 o3:2,3,3,3 ! g2 o6:4,3,3,3 g3 +d o5:2,2,2,4 +e1 o1.0:2 o2:1,1,1,1 o4:2,2,2,2 "
           "+e2 o1.2:1 o1.1 o1.3:2 +e3 o7:0,1,3,1 +e0 !")


def _dg(a, b, ca, cb):
    return jax.lax.dot_general(a, b, (((ca,), (cb,)), ((), ())), preferred_element_type=_F32)


def _bf(w):
    return pltpu.bitcast(w, _BF)


def _put(ref, g, c, v):
    for j in range(v.shape[1] // 128):
        ref[pl.ds(g, v.shape[0] // 16), c + j] = v[:, 128 * j:128 * j + 128].reshape(-1, 16, 128).astype(_BF)


def _get(ref, k, g, n, tiles=range(4)):
    words = ref.bitcast(_I32)
    return jnp.concatenate([words[k, pl.ds(g, n), c].reshape(8 * n, 128) for c in tiles], axis=1)


def _a_sums(a11, a12, a21, a22):
    return (a11 + a22, a21 + a22, a11 + a12, a21 - a11, a12 - a22)


def _b_sums(b11, b12, b21, b22):
    return (b11 + b22, b12 - b22, b21 - b11, b11 + b12, b21 + b22)


def _operand(rule, block):
    if len(rule) == 1:
        return block(rule[0])
    return block(rule[0]) + block(rule[2]) if rule[1] > 0 else block(rule[0]) - block(rule[2])


def _put_operands(side, m, block, ref, base, g):
    sub = [_operand(side[m], lambda k: block(k, j)) for j in range(4)]
    for n in range(7):
        _put(ref.at[base + n], g, 0, _operand(side[n], lambda j: sub[j]))
    return sub


def _mix(c, m):
    if c == 0:
        return m(0) + m(3) - m(4) + m(6)
    if c == 1:
        return m(2) + m(4)
    if c == 2:
        return m(1) + m(3)
    return m(0) - m(1) + m(2) + m(5)


def _paced(w, zeros):
    if not zeros:
        return w
    groups = w.shape[0] // 8
    first = [w[8 * g:8 * g + 8, 0:128] for g in range(groups)]
    for j, z in enumerate(zeros):
        g = max((j + 1) * groups // len(zeros) - 1, 0)
        first[g] = first[g] | z
    first = jnp.concatenate(first, axis=0)
    return first if w.shape[1] == 128 else jnp.concatenate([first, w[:, 128:]], axis=1)


def _play(program, steps, pieces):
    queue = []
    for word in program.split():
        if word == "!":
            while queue:
                queue.pop(0)()
        elif word[0] == "+":
            queue.extend(pieces(word[1:]))
        else:
            name, _, counts = word.partition(":")
            name, _, tile = name.partition(".")
            step, tiles = steps[name[0]]
            tiles = [int(tile)] if tile else range(tiles)
            counts = [int(n) for n in counts.split(",")] if counts else [0] * len(tiles)
            for t, n in zip(tiles, counts):
                step(int(name[1:]), t, [queue.pop(0)() for _ in range(min(n, len(queue)))])
    assert not queue


def _recip(v):
    r = pl.reciprocal(v, approx=True)
    return r * (2.0 - v * r)


def _pair_reduce(v, op):
    r = v[0:8]
    for j in range(1, 8):
        r = op(r, v[8 * j:8 * j + 8])
    r = op(r, pltpu.roll(r, 2, 0))
    return op(r, pltpu.roll(r, 4, 0))


def _rep8(v):
    return jnp.concatenate([v] * 8, axis=0)


def _dual_exp(p):
    ep = jnp.exp2(p - _rep8(_pair_reduce(p, jnp.maximum)))
    en = jnp.exp2(_rep8(_pair_reduce(p, jnp.minimum)) - p)
    return ep, en, _pair_reduce(ep, jnp.add), _pair_reduce(en, jnp.add)


def _col_bcast(row):
    return jnp.broadcast_to(row, (128, row.shape[1])).T


def _matvec(w_ref, col_ref, c, j0, j1, acc=None):
    for j in range(j0, j1):
        t = _bf(w_ref[8 * j:8 * j + 8, 128 * c:128 * c + 128]).astype(_F32) * col_ref[16 * j:16 * j + 16, :]
        acc = t[0:8] if acc is None else acc + t[0:8]
        acc = acc + t[8:16]
    return acc


def _kernel(x_hbm, wqkv_hbm, wphi_hbm, wo_hbm, wr_hbm, wg_hbm, wu_hbm, wd_hbm, gw_hbm,
            out_hbm,
            x_v, w_v, wg_v, wu_v, wd_v, wphi_v, wr_v, gw_v,
            wv_v, wo_v, lm_v, lk_v, lq_v, lv_v, lo_v, r_v, r2_v, phi_v, a_v,
            kv_v, z_v, kvm_v, g_v, top_v, arg_v, f_v, xc_v, hc_v, out_v,
            sem_x, sem_w, sem_v, sem_wo, sem_s, sem_g, sem_u, sem_d, sem_o):
    x_hbm, wqkv_hbm, wo_hbm, wg_hbm, wu_hbm, wd_hbm = (
        r.bitcast(_I32) for r in (x_hbm, wqkv_hbm, wo_hbm, wg_hbm, wu_hbm, wd_hbm))

    def cp_x(i):
        return pltpu.make_async_copy(x_hbm.at[pl.ds(i * _HT, _HT)], x_v.at[i], sem_x.at[i])

    def cp_w(j):
        return pltpu.make_async_copy(wqkv_hbm.at[:, pl.ds(j * _D, _D)], w_v.at[j], sem_w.at[j])

    def cp_v(k):
        return pltpu.make_async_copy(wqkv_hbm.at[pl.ds(256 * (k % 2), 256), pl.ds(2 * _D + _HD * (k // 2), _HD)],
                                     wv_v.at[k], sem_v.at[k])

    def cp_wo(k):
        return pltpu.make_async_copy(wo_hbm.at[pl.ds(256 * (k // 2), 256), pl.ds(_HD * (k % 2), _HD)],
                                     wo_v.at[k], sem_wo.at[k])

    cp_phi, cp_wr, cp_gw = (pltpu.make_async_copy(src, dst, sem_s.at[j]) for j, (src, dst) in enumerate(
        ((wphi_hbm, wphi_v), (wr_hbm, wr_v), (gw_hbm, gw_v))))

    def cp_ffn(i):
        cols = pl.ds(i * _FC, _FC)
        return (pltpu.make_async_copy(wg_hbm.at[:, cols], wg_v.at[i], sem_g.at[i]),
                pltpu.make_async_copy(wu_hbm.at[:, cols], wu_v.at[i], sem_u.at[i]),
                pltpu.make_async_copy(wd_hbm.at[pl.ds(i * (_FC // 2), _FC // 2)], wd_v.at[i], sem_d.at[i]))

    def cp_o(t, blk):
        return pltpu.make_async_copy(
            out_v[blk].at[t], out_hbm.at[pl.ds(t * _T + _HT * (blk // 2), _HT), pl.ds(_HD * (blk % 2), _HD)],
            sem_o.at[4 * t + blk])

    cp_wr.start()
    cp_gw.start()
    cp_x(0).start()
    cp_v(0).start()
    cp_v(1).start()

    kv_v[...] = jnp.zeros_like(kv_v)
    z_v[...] = jnp.zeros_like(z_v)
    f_v[...] = jnp.zeros_like(f_v)
    xc_v[_D:, :] = jnp.zeros((8, 128), _F32)
    top_v[...] = jnp.full((8, 128), -jnp.inf, _F32)
    arg_v[...] = jnp.zeros_like(arg_v)
    g_v[_S // 128, 0:8, :] = jnp.zeros((8, 128), _F32)
    for ref in (*r2_v, *lv_v, lo_v, lm_v, *phi_v):
        ref[ref.shape[0] - 1, 0, 0] = jnp.zeros((16, 128), _BF)
    for ref in out_v:
        ref[_NT, 0:16, 0:128] = jnp.zeros((16, 128), _BF)

    def feature_matrix():
        rows = jax.lax.broadcasted_iota(_I32, (64, _DH), 0)
        cols = jax.lax.broadcasted_iota(_I32, (64, _DH), 1)
        sel = jnp.where(rows >> 1 == cols, 1.0, 0.0).astype(_BF)
        half = _dg(sel, wphi_v[...].reshape(_H * _DH, _DH), 1, 1)
        rows = jax.lax.broadcasted_iota(_I32, (128, _D), 0)
        cols = jax.lax.broadcasted_iota(_I32, (128, _D), 1)
        keep = ((cols >> 5) & 3) == 2 * (rows >> 6) + (rows & 1)
        _put(lm_v.at[0], 0, 0, jnp.where(keep, jnp.concatenate([half, half], axis=0), 0.0))
        return _get(lm_v, 1 + zero, 0, 1, [0])

    def fold(j, l_v, queue=()):
        for g in range(4):
            for d in range(2):
                blk = []
                for gg in (g, g + 4):
                    c = slice(128 * gg, 128 * gg + 128)
                    for dd in (d, d + 2):
                        w = _paced(w_v[j, 128 * dd:128 * dd + 128, c], [queue.pop(0)() for _ in queue[:1]])
                        blk.append(_dg(_bf(_get(lm_v, 0, 0, 8, [gg])), _bf(w), 1, 1) * _LOG2E)
                blk += _a_sums(*blk)
                for m in range(7):
                    _put(l_v.at[m], 8 * g, 2 * d, blk[_A_SLOT[m]])

    def out_piece(g, c):
        def run():
            r = pl.ds(pl.multiple_of(8 * g, 8), 8)
            sums = _b_sums(*[_bf(wo_v.at[k][r, 128 * c:128 * c + 256]).astype(_F32) for k in range(4)])
            for k in range(5):
                _put(lo_v.at[k], g, c, sums[k])
            return _get(lo_v, 5, 0, 1, [0])
        return run

    def x_blk(i, k):
        return x_v.at[i, 128 * (k % 2):128 * (k % 2) + 128, _HD * (k // 2):_HD * (k // 2) + _HD]

    def tok_words(i, m, g=0, n=16):
        k = _B_SLOT[m]
        return x_blk(i, k)[8 * g:8 * (g + n), :] if k < 4 else _get(r_v[k - 4], i, g, n)

    def put_phi(blk, p, t, zero, pos, neg):
        _put(phi_v[blk].at[2 * p + t], 0, 0, jnp.concatenate([pos, neg], axis=0))
        return _get(phi_v[blk], 16 + zero, 0, 1, [0])

    def get_phi(blk, p, t, zero, zeros=()):
        return _bf(_paced(_get(phi_v[blk], 2 * p + t + zero, 0, 8, [0]), zeros))

    def phase1(i, zero, program):
        pk, pv, part = {}, {}, {}

        def kprod(m, t, zeros):
            pk[m - 1, t] = _dg(_bf(_paced(_get(lk_v, m - 1, 0, 32), zeros)),
                               _bf(tok_words(i, m - 1, 8 * t, 8)), 1, 1)

        def vprod(m, s, zeros):
            n = _ORDER[s]
            part[m, n] = _dg(_bf(_paced(_get(r2_v[m - 1], 7 * i + n, 0, 8, range(2)), zeros)),
                             _bf(_get(lv_v[m - 1], n, 0, 16, range(2))), 1, 0)
            if s == 6:
                for o in range(2):
                    val = jnp.concatenate([_mix(2 * o + t, lambda n: part[m, n]) for t in range(2)], axis=0)
                    pv[m - 1, 2 * o], pv[m - 1, 2 * o + 1] = val[:, :128], val[:, 128:]

        def kv(blk, c, zeros):
            vt = _mix(blk, lambda m: pv[m, c]).astype(_BF).T
            for h in range(2):
                p = 2 * c + h
                phi = jnp.concatenate([get_phi(blk, p, 0, zero, zeros[h::2]), get_phi(blk, p, 1, zero)], axis=1)
                kv_v[8 * (blk // 2) + p] += _dg(vt[64 * h:64 * h + 64], phi, 1, 1)

        def wait(j, t, zeros):
            for cp in (cp_v(2 * j), cp_v(2 * j + 1)) if j < 2 else (cp_w(1),):
                cp.wait()
            if j == 0:
                cp_w(1).start()
            elif j == 1:
                cp_phi.wait()
                cp_x(1).start()
                for k in range(4):
                    cp_wo(k).start()
            else:
                for k in range(2, _NT):
                    cp_x(k).start()
                cp_w(0).start()
                for k in range(_NT):
                    for cp in cp_ffn(k):
                        cp.start()
                fold(1, lk_v)

        def token_piece(m, g):
            def run():
                def block(k, j):
                    r = 64 * (j % 2) + 8 * g
                    return _bf(x_blk(i, k)[r:r + 8, 256 * (j // 2):256 * (j // 2) + 256]).astype(_F32)
                sub = _put_operands(_RIGHT, m, block, r2_v[m], 7 * (i + zero), g)
                if _B_SLOT[m] > 3:
                    for j in range(4):
                        _put(r_v[_B_SLOT[m] - 4].at[i + zero], 8 * (j % 2) + g, 2 * (j // 2), sub[j])
                return _get(r2_v[m], 7 * _NT, 0, 1, [0])
            return run

        def value_piece(m, g):
            def run():
                def block(k, j):
                    r = 128 * (j % 2) + 8 * g
                    return _bf(wv_v[k, r:r + 8, 256 * (j // 2):256 * (j // 2) + 256]).astype(_F32)
                _put_operands(_LEFT, m, block, lv_v[m], 0, g)
                return _get(lv_v[m], 7 + zero, 0, 1, [0])
            return run

        def feat_piece(blk, t, p):
            def run():
                ep, en, sp, sn = _dual_exp(_mix(blk, lambda m: pk[m, t][64 * p:64 * p + 64]))
                ep, en = ep * _rep8(_recip(sp)), en * _rep8(_recip(sn))
                z_v[8 * (blk // 2) + p] += jnp.concatenate([ep, en], axis=0)
                return put_phi(blk, p, t, zero, ep, en)
            return run

        def score_piece(c):
            def run():
                xh = _bf(x_v[i, 16 * c:16 * c + 16, :]).astype(_F32)
                wr = wr_v[...].astype(_F32).reshape(1, _D)
                gw = gw_v[...].astype(_F32).reshape(1, _D)
                g = jax.nn.sigmoid(jnp.sum(xh * gw, axis=1, keepdims=True))
                g_v[4 * i + c // 4, 32 * (c % 4):32 * (c % 4) + 32, :] = jnp.broadcast_to(g, (32, 128))
                sc = jnp.sum(xh * wr, axis=1, keepdims=True).astype(_BF).astype(_F32)
                best, bidx = top_v[...], arg_v[0]
                for j in range(4):
                    rj = sc[8 * j:8 * j + 8]
                    upd = rj > best
                    best = jnp.where(upd, rj, best)
                    bidx = jnp.where(upd, i * _T + 32 * c + 8 * j, bidx)
                top_v[...] = best
                arg_v[0] = bidx
                return arg_v[1 + zero] | pltpu.bitcast(g_v[_S // 128 + zero, 0:8, :], _I32)
            return run

        def pieces(name):
            if name[0] == "r":
                return [token_piece(int(name[1]) - 1, g) for g in range(8)]
            if name == "m":
                return [feature_matrix]
            if name == "s":
                return [score_piece(c) for c in range(16)]
            if name[0] == "a":
                return [value_piece(int(name[1]) - 1, g) for g in range(16)]
            if name == "o":
                start = jnp.minimum(11 * (i - 1), 32 - 11)
                return [out_piece(start + j // 2, 2 * (j % 2)) for j in range(22)]
            return [feat_piece(int(name[1]), t, p) for t in ([int(name[2])] if name[2:] else range(2))
                    for p in range(8)]

        _play(program, {"k": (kprod, 2), "v": (vprod, 7), "g": (kv, 4), "W": (wait, 1)}, pieces)

    def later_tile(i):
        cp_x(i).wait()
        phase1(i, i >> 8, _PHASE1)

    zero = arg_v[1, 0, 0]
    cp_wr.wait()
    cp_gw.wait()
    cp_x(0).wait()
    cp_v(2).start()
    cp_v(3).start()
    cp_phi.start()
    phase1(0, zero, _FIRST)
    for k in range(4):
        cp_wo(k).wait()
    pl.loop(1, _NT)(later_tile)

    cp_w(0).wait()
    best = top_v[...]
    bidx = arg_v[0] + jax.lax.broadcasted_iota(_I32, (8, 128), 0)
    rmax = jnp.max(best, axis=0, keepdims=True)
    idx = jnp.min(jnp.where(best == rmax, bidx, _S - 1))
    r_sel = jax.nn.sigmoid(rmax)
    tsel = idx // _T
    rsel = idx - tsel * _T
    grp = _bf(x_v[tsel, pl.ds(pl.multiple_of((rsel >> 4) << 3, 8), 8), :]).astype(_F32)
    hit = jax.lax.broadcasted_iota(_I32, (16, _D), 0) == (rsel & 15)
    x_sel = jnp.sum(jnp.where(hit, grp, 0.0), axis=0, keepdims=True)

    def state_piece(p):
        def run():
            rows = jax.lax.broadcasted_iota(_I32, (64, 128), 0)
            cols = jax.lax.broadcasted_iota(_I32, (64, 128), 1)
            _put(kvm_v.at[p], 0, 0, jnp.where((rows >> 5) == (cols & 1), kv_v[p], 0.0))
            z_v[p] = jnp.broadcast_to(jnp.sum(z_v[p], axis=1, keepdims=True), (128, 128))
            return pltpu.bitcast(z_v[_NP + zero, 0:8, :], _I32)
        return run

    def column_piece(c):
        def run():
            xc_v[128 * c:128 * c + 128, :] = _col_bcast(x_sel[:, 128 * c:128 * c + 128])
            return pltpu.bitcast(xc_v[pl.ds(pl.multiple_of(_D + zero, 8), 8), :], _I32)
        return run

    fold(0, lq_v, [state_piece(p) for p in range(_NP)] + [column_piece(c) for c in range(8)])

    def phase2(i):
        ti = (tsel + 1 + i) % _NT
        for cp in cp_ffn(i):
            cp.wait()
        zero = i >> 8
        pq, po, ot = {}, {}, {}

        def qprod(m, t, zeros):
            pq[m - 1, t] = _dg(_bf(_paced(_get(lq_v, m - 1, 0, 32), zeros)),
                               _bf(tok_words(ti, m - 1, 8 * t, 8)), 1, 1)

        def attn(blk, t, zeros):
            for p in range(8):
                a_v[blk][t][64 * p:64 * p + 64, :] = _dg(
                    _bf(_get(kvm_v, 8 * (blk // 2) + p, 0, 4, [0])), get_phi(blk, p, t, zero, zeros[p::8]), 1, 0)

        def oprod(m, c, zeros):
            if m not in ot:
                at = []
                for t in range(2):
                    rows = pl.ds(pl.multiple_of(zero, 8), _HD)
                    at.append(_operand(_LEFT[m - 1], lambda k: a_v[(0, 2, 1, 3)[k]][t][rows, :]).astype(_BF).T)
                ot[m] = jnp.concatenate(at, axis=0)
            k = _B_SLOT[m - 1]
            w = wo_v[k, :, 128 * c:128 * c + 128] if k < 4 else _get(lo_v, k - 4, 0, 32, [c])
            po[m - 1, c] = _dg(ot[m], _bf(jnp.concatenate([_paced(w[0:64], zeros), w[64:]], axis=0)), 1, 0)

        def feat_piece(blk, t, p):
            def run():
                ep, en, sp, sn = _dual_exp(_mix(blk, lambda m: pq[m, t][64 * p:64 * p + 64]))
                z = z_v[8 * (blk // 2) + p]
                dp, dn = _pair_reduce(ep * z[0:64], jnp.add), _pair_reduce(en * z[64:128], jnp.add)
                inv = _recip(dp * sn + sp * (dn + 1e-6 * sn))
                return put_phi(blk, p, t, zero, ep * _rep8(sn * inv), en * _rep8(sp * inv))
            return run

        def hidden_piece(c, half):
            def run():
                for k, w in enumerate((wg_v, wu_v)):
                    acc = f_v[2 * c + k + zero] if half else None
                    f_v[2 * c + k] = _matvec(w.at[i], xc_v, c, 32 * half, 32 * half + 32, acc)
                return pltpu.bitcast(f_v[22 + zero], _I32)
            return run

        def act_piece(c):
            def run():
                hg, hu = (jnp.sum(f_v[2 * c + k + zero], axis=0, keepdims=True) for k in range(2))
                hc_v[128 * c:128 * c + 128, :] = _col_bcast(hg * jax.nn.sigmoid(hg) * hu)
            return run

        def down_piece(c, half):
            def run():
                for cc in (c, c + 1):
                    f_v[14 + cc] = _matvec(wd_v.at[i], hc_v, cc, 28 * half, 28 * half + 28, f_v[14 + cc + zero])
                return pltpu.bitcast(f_v[22 + zero], _I32)
            return run

        def emit_piece(blk, u, c):
            def run():
                h, d = blk // 2, blk % 2
                g = g_v[4 * ti + 2 * h + u]
                tok = jax.lax.broadcasted_iota(_I32, (128, 128), 0) + (ti * _T + _HT * h + 128 * u)
                o = []
                for cc in (c, c + 1):
                    y = jnp.sum(f_v[14 + 4 * d + cc + zero], axis=0, keepdims=True) * r_sel
                    b = _bf(x_blk(ti, 2 * d + h)[64 * u:64 * u + 64, 128 * cc:128 * cc + 128]).astype(_F32)
                    b = b + jnp.where(tok == idx, y, 0.0)
                    o.append(g * _mix(blk, lambda m: po[m, cc][128 * u:128 * u + 128]) + (1.0 - g) * b)
                out_v[blk][ti, 128 * u:128 * u + 128, 128 * c:128 * c + 256] = (
                    jnp.concatenate(o, axis=1).astype(_BF))
                if (u, c) == (1, 2):
                    cp_o(ti, blk).start()
                    out_v[blk][_NT, 16:32, 0:128] = jnp.zeros((16, 128), _BF)
                return pltpu.bitcast(out_v[blk][_NT + zero, 0:16, 0:128], _I32)
            return run

        def pieces(name):
            if name[0] == "h":
                return [hidden_piece(c, int(name[1])) for c in range(_FC // 128)]
            if name == "a":
                return [act_piece(c) for c in range(_FC // 128)]
            if name == "d":
                return [down_piece(c, half) for c in (4, 6, 0, 2) for half in range(2)]
            if name[0] == "e":
                return [emit_piece(int(name[1]), u, c) for c in (0, 2) for u in range(2)]
            return [feat_piece(int(name[1]), t, p) for t in ([int(name[2])] if name[2:] else range(2))
                    for p in range(8)]

        _play(_PHASE2, {"q": (qprod, 2), "o": (oprod, 4), "g": (attn, 2)}, pieces)

    pl.loop(0, _NT)(phase2)
    for t in range(_NT):
        for blk in range(4):
            cp_o(t, blk).wait()


@jax.jit
def pallas_gated_mix__linear_kernel_hedgehog__moe_arch_mod__prompt_kernel(
    A_x: jax.Array,
    A_wqkv: jax.Array,
    A_w_phi: jax.Array,
    A_wo: jax.Array,
    B_x: jax.Array,
    B_w_r: jax.Array,
    B_w_gate: jax.Array,
    B_w_up: jax.Array,
    B_w_down: jax.Array,
    gate_w: jax.Array,
):
    del B_x
    hbm = pl.BlockSpec(memory_space=pl.ANY)
    dma = pltpu.SemaphoreType.DMA
    out = pl.pallas_call(
        _kernel,
        out_shape=jax.ShapeDtypeStruct((_S, _D), _BF),
        in_specs=[hbm] * 9,
        out_specs=hbm,
        scratch_shapes=[
            pltpu.VMEM((_NT, _HT, _D), _I32),
            pltpu.VMEM((2, _HD, _D), _I32),
            pltpu.VMEM((_NT, _HD, _FC), _I32),
            pltpu.VMEM((_NT, _HD, _FC), _I32),
            pltpu.VMEM((_NT, _FC // 2, _D), _I32),
            pltpu.VMEM((_H, _DH, _DH), _BF),
            pltpu.VMEM((_D,), _BF),
            pltpu.VMEM((_D,), _BF),
            pltpu.VMEM((4, 256, _HD), _I32),
            pltpu.VMEM((4, 256, _HD), _I32),
            pltpu.VMEM((2, 8, 8, 16, 128), _BF),
            pltpu.VMEM((7, 32, 4, 16, 128), _BF),
            pltpu.VMEM((7, 32, 4, 16, 128), _BF),
            [pltpu.VMEM((8, 16, 2, 16, 128), _BF)] * 7,
            pltpu.VMEM((6, 32, 4, 16, 128), _BF),
            [pltpu.VMEM((_NT, 16, 4, 16, 128), _BF)] * 5,
            [pltpu.VMEM((7 * _NT + 1, 8, 2, 16, 128), _BF)] * 7,
            [pltpu.VMEM((17, 8, 1, 16, 128), _BF)] * 4,
            [[pltpu.VMEM((_HD, 128), _F32)] * 2] * 4,
            pltpu.VMEM((_NP, 64, 128), _F32),
            pltpu.VMEM((_NP + 1, 128, 128), _F32),
            pltpu.VMEM((_NP, 4, 1, 16, 128), _BF),
            pltpu.VMEM((_S // 128 + 1, 128, 128), _F32),
            pltpu.VMEM((8, 128), _F32),
            pltpu.VMEM((2, 8, 128), _I32),
            pltpu.VMEM((23, 8, 128), _F32),
            pltpu.VMEM((_D + 8, 128), _F32),
            pltpu.VMEM((_FC, 128), _F32),
            [pltpu.VMEM((_NT + 1, _HT, _HD), _BF)] * 4,
            dma((_NT,)), dma((2,)), dma((4,)), dma((4,)), dma((3,)),
            dma((_NT,)), dma((_NT,)), dma((_NT,)), dma((4 * _NT,)),
        ],
        compiler_params=pltpu.CompilerParams(vmem_limit_bytes=100 * 1024 * 1024, disable_semaphore_checks=True),
    )(A_x.reshape(_S, _D), A_wqkv, A_w_phi, A_wo, B_w_r, B_w_gate, B_w_up, B_w_down, gate_w)
    return out.reshape(1, _S, _D)
```

```python
import jax
import jax.numpy as jnp
import jax.experimental.pallas as pl
import jax.experimental.pallas.tpu as pltpu

_BF = jnp.bfloat16
_F32 = jnp.float32
_I32 = jnp.int32
_LOG2E = 1.4426950408889634

_S, _D, _H, _DH, _F = 2048, 1024, 32, 32, 3584
_T = 512
_HT = _T // 2
_HD = _D // 2
_NT = _S // _T
_FC = _F // _NT
_NP = _H // 2

_LEFT = ((0, 1, 3), (2, 1, 3), (0,), (3,), (0, 1, 1), (2, -1, 0), (1, -1, 3))
_RIGHT = ((0, 1, 3), (0,), (1, -1, 3), (2, -1, 0), (3,), (0, 1, 1), (2, 1, 3))
_A_SLOT = (4, 5, 0, 3, 6, 7, 8)
_B_SLOT = (4, 0, 5, 6, 3, 7, 8)
_ORDER = (1, 4, 3, 2, 0, 6, 5)

_FIRST = ("+r2 +r3 +r4 +r5 +r1 +r6 +r7 ! W0 +a3 +a5 ! v3 v5 W1 +m +a4 ! +a2 +a1 v4:3,5,2,2,2,3,2 +a7 "
          "v2:4,4,3,3,3,3,3 v1:3,3,2,2,2,2,2 +a6 v7:5,5,4,4,4,3,4 W2 k4 k5:1,1 k2 +f2 k3:5,4 +s +f1 k1:6,6 "
          "k7:6,9 +f0 k6:7,6 v6:2,1,0,1,0,2,1 +f3 g0:2,2,2,2 g1.2 g2:5,5,5,6 g1.0 g1.3 g1.1 g3:0,0,1,0")
_PHASE1 = ("+r2 +r3 +r4 +r6 +r5 +r7 +r1 +o k5.1:6 k2.1:9 k2.0:8 +f2 v2:2,2,2,2,2,1,1 +f1 k5.0:9 "
           "v5:5,5,5,5,5,5,4 k4 k3:8,6 +s v4:2,2,2,2,2,4,2 v3:3,3,3,3,3,3,3 k7:2,2 k1:5,2 +f0 g2 g1.0:1 "
           "g1.1 v1:1,0,1,1,0,1,0 g1.3 v7:3,4,3,3,3,3,5 g1.2 k6:12,14 +f3 v6:2,0,2,2,2,2,2 g0:1,1,3,2 "
           "g3:1,0,2,3")
_PHASE2 = ("+h0 +h1 q4.1:2 q4.0:4 q7.1:1 q1:1,2 q7.0:3 q5.0 +f0 q5.1:2 q3:7,6 q2.0:9 g0 +f1 q2.1:9 +f2 "
           "q6:6,6 +f3 +a g1 o3:2,3,3,3 ! g2 o6:4,3,3,3 g3 +d o5:2,2,2,4 +e1 o1.0:2 o2:1,1,1,1 o4:2,2,2,2 "
           "+e2 o1.2:1 o1.1 o1.3:2 +e3 o7:0,1,3,1 +e0 !")


def _dg(a, b, ca, cb):
    return jax.lax.dot_general(a, b, (((ca,), (cb,)), ((), ())), preferred_element_type=_F32)


def _bf(w):
    return pltpu.bitcast(w, _BF)


def _put(ref, g, c, v):
    for j in range(v.shape[1] // 128):
        ref[pl.ds(g, v.shape[0] // 16), c + j] = v[:, 128 * j:128 * j + 128].reshape(-1, 16, 128).astype(_BF)


def _get(ref, k, g, n, tiles=range(4)):
    words = ref.bitcast(_I32)
    return jnp.concatenate([words[k, pl.ds(g, n), c].reshape(8 * n, 128) for c in tiles], axis=1)


def _a_sums(a11, a12, a21, a22):
    return (a11 + a22, a21 + a22, a11 + a12, a21 - a11, a12 - a22)


def _b_sums(b11, b12, b21, b22):
    return (b11 + b22, b12 - b22, b21 - b11, b11 + b12, b21 + b22)


def _operand(rule, block):
    if len(rule) == 1:
        return block(rule[0])
    return block(rule[0]) + block(rule[2]) if rule[1] > 0 else block(rule[0]) - block(rule[2])


def _put_operands(side, m, block, ref, base, g):
    sub = [_operand(side[m], lambda k: block(k, j)) for j in range(4)]
    for n in range(7):
        _put(ref.at[base + n], g, 0, _operand(side[n], lambda j: sub[j]))
    return sub


def _mix(c, m):
    if c == 0:
        return m(0) + m(3) - m(4) + m(6)
    if c == 1:
        return m(2) + m(4)
    if c == 2:
        return m(1) + m(3)
    return m(0) - m(1) + m(2) + m(5)


def _paced(w, zeros):
    if not zeros:
        return w
    groups = w.shape[0] // 8
    first = [w[8 * g:8 * g + 8, 0:128] for g in range(groups)]
    for j, z in enumerate(zeros):
        g = max((j + 1) * groups // len(zeros) - 1, 0)
        first[g] = first[g] | z
    first = jnp.concatenate(first, axis=0)
    return first if w.shape[1] == 128 else jnp.concatenate([first, w[:, 128:]], axis=1)


def _play(program, steps, pieces):
    queue = []
    for word in program.split():
        if word == "!":
            while queue:
                queue.pop(0)()
        elif word[0] == "+":
            queue.extend(pieces(word[1:]))
        else:
            name, _, counts = word.partition(":")
            name, _, tile = name.partition(".")
            step, tiles = steps[name[0]]
            tiles = [int(tile)] if tile else range(tiles)
            counts = [int(n) for n in counts.split(",")] if counts else [0] * len(tiles)
            for t, n in zip(tiles, counts):
                step(int(name[1:]), t, [queue.pop(0)() for _ in range(min(n, len(queue)))])
    assert not queue


def _recip(v):
    r = pl.reciprocal(v, approx=True)
    return r * (2.0 - v * r)


def _pair_reduce(v, op):
    r = v[0:8]
    for j in range(1, 8):
        r = op(r, v[8 * j:8 * j + 8])
    r = op(r, pltpu.roll(r, 2, 0))
    return op(r, pltpu.roll(r, 4, 0))


def _rep8(v):
    return jnp.concatenate([v] * 8, axis=0)


def _dual_exp(p):
    ep = jnp.exp2(p - _rep8(_pair_reduce(p, jnp.maximum)))
    en = jnp.exp2(_rep8(_pair_reduce(p, jnp.minimum)) - p)
    return ep, en, _pair_reduce(ep, jnp.add), _pair_reduce(en, jnp.add)


def _col_bcast(row):
    return jnp.broadcast_to(row, (128, row.shape[1])).T


def _matvec(w_ref, col_ref, c, j0, j1, acc=None):
    for j in range(j0, j1):
        t = _bf(w_ref[8 * j:8 * j + 8, 128 * c:128 * c + 128]).astype(_F32) * col_ref[16 * j:16 * j + 16, :]
        acc = t[0:8] if acc is None else acc + t[0:8]
        acc = acc + t[8:16]
    return acc


def _kernel(x_hbm, wqkv_hbm, wphi_hbm, wo_hbm, wr_hbm, wg_hbm, wu_hbm, wd_hbm, gw_hbm,
            out_hbm,
            x_v, w_v, wg_v, wu_v, wd_v, wphi_v, wr_v, gw_v,
            wv_v, wo_v, lm_v, ls_v, lk_v, lq_v, lv_v, lo_v, r_v, r2_v, phi_v, a_v,
            kv_v, z_v, kvm_v, g_v, top_v, arg_v, f_v, xc_v, hc_v, out_v,
            sem_x, sem_w, sem_v, sem_wo, sem_s, sem_g, sem_u, sem_d, sem_o):
    x_hbm, wqkv_hbm, wo_hbm, wg_hbm, wu_hbm, wd_hbm = (
        r.bitcast(_I32) for r in (x_hbm, wqkv_hbm, wo_hbm, wg_hbm, wu_hbm, wd_hbm))

    def cp_x(i):
        return pltpu.make_async_copy(x_hbm.at[pl.ds(i * _HT, _HT)], x_v.at[i], sem_x.at[i])

    def cp_w(j):
        return pltpu.make_async_copy(wqkv_hbm.at[:, pl.ds(j * _D, _D)], w_v.at[j], sem_w.at[j])

    def cp_v(k):
        return pltpu.make_async_copy(wqkv_hbm.at[pl.ds(256 * (k % 2), 256), pl.ds(2 * _D + _HD * (k // 2), _HD)],
                                     wv_v.at[k], sem_v.at[k])

    def cp_wo(k):
        return pltpu.make_async_copy(wo_hbm.at[pl.ds(256 * (k // 2), 256), pl.ds(_HD * (k % 2), _HD)],
                                     wo_v.at[k], sem_wo.at[k])

    cp_phi, cp_wr, cp_gw = (pltpu.make_async_copy(src, dst, sem_s.at[j]) for j, (src, dst) in enumerate(
        ((wphi_hbm, wphi_v), (wr_hbm, wr_v), (gw_hbm, gw_v))))

    def cp_ffn(i):
        cols = pl.ds(i * _FC, _FC)
        return (pltpu.make_async_copy(wg_hbm.at[:, cols], wg_v.at[i], sem_g.at[i]),
                pltpu.make_async_copy(wu_hbm.at[:, cols], wu_v.at[i], sem_u.at[i]),
                pltpu.make_async_copy(wd_hbm.at[pl.ds(i * (_FC // 2), _FC // 2)], wd_v.at[i], sem_d.at[i]))

    def cp_o(t, blk):
        return pltpu.make_async_copy(
            out_v[blk].at[t], out_hbm.at[pl.ds(t * _T + _HT * (blk // 2), _HT), pl.ds(_HD * (blk % 2), _HD)],
            sem_o.at[4 * t + blk])

    cp_wr.start()
    cp_gw.start()
    cp_x(0).start()
    cp_v(0).start()
    cp_v(1).start()

    kv_v[...] = jnp.zeros_like(kv_v)
    z_v[...] = jnp.zeros_like(z_v)
    f_v[...] = jnp.zeros_like(f_v)
    xc_v[_D:, :] = jnp.zeros((8, 128), _F32)
    top_v[...] = jnp.full((8, 128), -jnp.inf, _F32)
    arg_v[...] = jnp.zeros_like(arg_v)
    g_v[_S // 128, 0:8, :] = jnp.zeros((8, 128), _F32)
    for ref in (*r2_v, *lv_v, lo_v, lm_v, *phi_v):
        ref[ref.shape[0] - 1, 0, 0] = jnp.zeros((16, 128), _BF)
    for ref in out_v:
        ref[_NT, 0:16, 0:128] = jnp.zeros((16, 128), _BF)

    def feature_matrix():
        rows = jax.lax.broadcasted_iota(_I32, (64, _DH), 0)
        cols = jax.lax.broadcasted_iota(_I32, (64, _DH), 1)
        sel = jnp.where(rows >> 1 == cols, 1.0, 0.0).astype(_BF)
        half = _dg(sel, wphi_v[...].reshape(_H * _DH, _DH), 1, 1)
        rows = jax.lax.broadcasted_iota(_I32, (128, _D), 0)
        cols = jax.lax.broadcasted_iota(_I32, (128, _D), 1)
        keep = ((cols >> 5) & 3) == 2 * (rows >> 6) + (rows & 1)
        _put(lm_v.at[0], 0, 0, jnp.where(keep, jnp.concatenate([half, half], axis=0), 0.0))
        return _get(lm_v, 1 + zero, 0, 1, [0])

    def fold(j, l_v, queue=()):
        for g in range(4):
            for d in range(2):
                blk = []
                for gg in (g, g + 4):
                    c = slice(128 * gg, 128 * gg + 128)
                    for dd in (d, d + 2):
                        w = _paced(w_v[j, 128 * dd:128 * dd + 128, c], [queue.pop(0)() for _ in queue[:1]])
                        blk.append(_dg(_bf(_get(lm_v, 0, 0, 8, [gg])), _bf(w), 1, 1) * _LOG2E)
                blk += _a_sums(*blk)
                for m in range(7):
                    _put(l_v.at[m], 8 * g, 2 * d, blk[_A_SLOT[m]])

    def out_piece(g, c):
        def run():
            r = pl.ds(pl.multiple_of(8 * g, 8), 8)
            sums = _b_sums(*[_bf(wo_v.at[k][r, 128 * c:128 * c + 256]).astype(_F32) for k in range(4)])
            for k in range(5):
                _put(lo_v.at[k], g, c, sums[k])
            return _get(lo_v, 5, 0, 1, [0])
        return run

    def x_blk(i, k):
        return x_v.at[i, 128 * (k % 2):128 * (k % 2) + 128, _HD * (k // 2):_HD * (k // 2) + _HD]

    def tok_words(i, m, g=0, n=16):
        k = _B_SLOT[m]
        return x_blk(i, k)[8 * g:8 * (g + n), :] if k < 4 else _get(r_v[k - 4], i, g, n)

    def put_phi(blk, p, t, zero, pos, neg):
        _put(phi_v[blk].at[2 * p + t], 0, 0, jnp.concatenate([pos, neg], axis=0))
        return _get(phi_v[blk], 16 + zero, 0, 1, [0])

    def get_phi(blk, p, t, zero, zeros=()):
        return _bf(_paced(_get(phi_v[blk], 2 * p + t + zero, 0, 8, [0]), zeros))

    def phase1(i, zero, program):
        pk, ps, pv, part = {}, {}, {}, {}

        def kprod(m, t, zeros):
            w = _paced(_get(lk_v, m - 1, 0, 32), zeros)
            if m in (2, 3, 4, 5):
                w = jnp.concatenate([_get(ls_v, 0, 0, 1), w], axis=0)
            out = _dg(_bf(w), _bf(tok_words(i, m - 1, 8 * t, 8)), 1, 1)
            ps[m - 1, t], pk[m - 1, t] = out[:8], out[-_HD:]

        def vprod(m, s, zeros):
            n = _ORDER[s]
            part[m, n] = _dg(_bf(_paced(_get(r2_v[m - 1], 7 * i + n, 0, 8, range(2)), zeros)),
                             _bf(_get(lv_v[m - 1], n, 0, 16, range(2))), 1, 0)
            if s == 6:
                for o in range(2):
                    val = jnp.concatenate([_mix(2 * o + t, lambda n: part[m, n]) for t in range(2)], axis=0)
                    pv[m - 1, 2 * o], pv[m - 1, 2 * o + 1] = val[:, :128], val[:, 128:]

        def kv(blk, c, zeros):
            vt = _mix(blk, lambda m: pv[m, c]).astype(_BF).T
            for h in range(2):
                p = 2 * c + h
                phi = jnp.concatenate([get_phi(blk, p, 0, zero, zeros[h::2]), get_phi(blk, p, 1, zero)], axis=1)
                kv_v[8 * (blk // 2) + p] += _dg(vt[64 * h:64 * h + 64], phi, 1, 1)

        def wait(j, t, zeros):
            for cp in (cp_v(2 * j), cp_v(2 * j + 1)) if j < 2 else (cp_w(1),):
                cp.wait()
            if j == 0:
                cp_w(1).start()
            elif j == 1:
                cp_phi.wait()
                cp_x(1).start()
                for k in range(4):
                    cp_wo(k).start()
            else:
                for k in range(2, _NT):
                    cp_x(k).start()
                cp_w(0).start()
                for k in range(_NT):
                    for cp in cp_ffn(k):
                        cp.start()
                fold(1, lk_v)

        def token_piece(m, g):
            def run():
                def block(k, j):
                    r = 64 * (j % 2) + 8 * g
                    return _bf(x_blk(i, k)[r:r + 8, 256 * (j // 2):256 * (j // 2) + 256]).astype(_F32)
                sub = _put_operands(_RIGHT, m, block, r2_v[m], 7 * (i + zero), g)
                if _B_SLOT[m] > 3:
                    for j in range(4):
                        _put(r_v[_B_SLOT[m] - 4].at[i + zero], 8 * (j % 2) + g, 2 * (j // 2), sub[j])
                return _get(r2_v[m], 7 * _NT, 0, 1, [0])
            return run

        def value_piece(m, g):
            def run():
                def block(k, j):
                    r = 128 * (j % 2) + 8 * g
                    return _bf(wv_v[k, r:r + 8, 256 * (j // 2):256 * (j // 2) + 256]).astype(_F32)
                _put_operands(_LEFT, m, block, lv_v[m], 0, g)
                return _get(lv_v[m], 7 + zero, 0, 1, [0])
            return run

        def feat_piece(blk, t, p):
            def run():
                ep, en, sp, sn = _dual_exp(_mix(blk, lambda m: pk[m, t][64 * p:64 * p + 64]))
                ep, en = ep * _rep8(_recip(sp)), en * _rep8(_recip(sn))
                z_v[8 * (blk // 2) + p] += jnp.concatenate([ep, en], axis=0)
                return put_phi(blk, p, t, zero, ep, en)
            return run

        def score_piece(c):
            def run():
                h, t = c // 2, c % 2
                both, one = (ps[1, t], ps[3, t]) if h == 0 else (ps[4, t], ps[2, t])
                sc, gl = (both[k:k + 1] + both[k + 1:k + 2] + one[k + 1 - h:k + 2 - h] for k in (0, 2))
                g_v[4 * i + c] = _col_bcast(jax.nn.sigmoid(gl))
                sc = jnp.broadcast_to(sc, (8, 128)).astype(_BF).astype(_F32)
                best = top_v[...]
                upd = sc > best
                top_v[...] = jnp.where(upd, sc, best)
                arg_v[0] = jnp.where(upd, i * _T + 128 * c, arg_v[0])
                return arg_v[1 + zero] | pltpu.bitcast(g_v[_S // 128 + zero, 0:8, :], _I32)
            return run

        def pieces(name):
            if name[0] == "r":
                return [token_piece(int(name[1]) - 1, g) for g in range(8)]
            if name == "m":
                return [feature_matrix]
            if name == "s":
                return [score_piece(c) for c in range(4)]
            if name[0] == "a":
                return [value_piece(int(name[1]) - 1, g) for g in range(16)]
            if name == "o":
                start = jnp.minimum(11 * (i - 1), 32 - 11)
                return [out_piece(start + j // 2, 2 * (j % 2)) for j in range(22)]
            return [feat_piece(int(name[1]), t, p) for t in ([int(name[2])] if name[2:] else range(2))
                    for p in range(8)]

        _play(program, {"k": (kprod, 2), "v": (vprod, 7), "g": (kv, 4), "W": (wait, 1)}, pieces)

    def later_tile(i):
        cp_x(i).wait()
        phase1(i, i >> 8, _PHASE1)

    zero = arg_v[1, 0, 0]
    cp_wr.wait()
    cp_gw.wait()
    rows = jax.lax.broadcasted_iota(_I32, (16, _HD), 0)
    extra = jnp.zeros((16, _HD), _F32)
    for k, ref in enumerate((wr_v, gw_v)):
        w = ref[...].astype(_F32).reshape(1, _D)
        for d in range(2):
            extra = jnp.where(rows == 2 * k + d, w[:, _HD * d:_HD * d + _HD], extra)
    _put(ls_v.at[0], 0, 0, extra)
    cp_x(0).wait()
    cp_v(2).start()
    cp_v(3).start()
    cp_phi.start()
    phase1(0, zero, _FIRST)
    for k in range(4):
        cp_wo(k).wait()
    pl.loop(1, _NT)(later_tile)

    cp_w(0).wait()
    best = top_v[...]
    bidx = arg_v[0] + jax.lax.broadcasted_iota(_I32, (8, 128), 1)
    rmax = jnp.broadcast_to(jnp.max(best[0:1], axis=1, keepdims=True), (1, 128))
    idx = jnp.min(jnp.where(best == rmax, bidx, _S - 1))
    r_sel = jax.nn.sigmoid(rmax)
    tsel = idx // _T
    rsel = idx - tsel * _T
    grp = _bf(x_v[tsel, pl.ds(pl.multiple_of((rsel >> 4) << 3, 8), 8), :]).astype(_F32)
    hit = jax.lax.broadcasted_iota(_I32, (16, _D), 0) == (rsel & 15)
    x_sel = jnp.sum(jnp.where(hit, grp, 0.0), axis=0, keepdims=True)

    def state_piece(p):
        def run():
            rows = jax.lax.broadcasted_iota(_I32, (64, 128), 0)
            cols = jax.lax.broadcasted_iota(_I32, (64, 128), 1)
            _put(kvm_v.at[p], 0, 0, jnp.where((rows >> 5) == (cols & 1), kv_v[p], 0.0))
            z_v[p] = jnp.broadcast_to(jnp.sum(z_v[p], axis=1, keepdims=True), (128, 128))
            return pltpu.bitcast(z_v[_NP + zero, 0:8, :], _I32)
        return run

    def column_piece(c):
        def run():
            xc_v[128 * c:128 * c + 128, :] = _col_bcast(x_sel[:, 128 * c:128 * c + 128])
            return pltpu.bitcast(xc_v[pl.ds(pl.multiple_of(_D + zero, 8), 8), :], _I32)
        return run

    fold(0, lq_v, [state_piece(p) for p in range(_NP)] + [column_piece(c) for c in range(8)])

    def phase2(i):
        ti = (tsel + 1 + i) % _NT
        for cp in cp_ffn(i):
            cp.wait()
        zero = i >> 8
        pq, po, ot = {}, {}, {}

        def qprod(m, t, zeros):
            pq[m - 1, t] = _dg(_bf(_paced(_get(lq_v, m - 1, 0, 32), zeros)),
                               _bf(tok_words(ti, m - 1, 8 * t, 8)), 1, 1)

        def attn(blk, t, zeros):
            for p in range(8):
                a_v[blk][t][64 * p:64 * p + 64, :] = _dg(
                    _bf(_get(kvm_v, 8 * (blk // 2) + p, 0, 4, [0])), get_phi(blk, p, t, zero, zeros[p::8]), 1, 0)

        def oprod(m, c, zeros):
            if m not in ot:
                at = []
                for t in range(2):
                    rows = pl.ds(pl.multiple_of(zero, 8), _HD)
                    at.append(_operand(_LEFT[m - 1], lambda k: a_v[(0, 2, 1, 3)[k]][t][rows, :]).astype(_BF).T)
                ot[m] = jnp.concatenate(at, axis=0)
            k = _B_SLOT[m - 1]
            w = wo_v[k, :, 128 * c:128 * c + 128] if k < 4 else _get(lo_v, k - 4, 0, 32, [c])
            po[m - 1, c] = _dg(ot[m], _bf(jnp.concatenate([_paced(w[0:64], zeros), w[64:]], axis=0)), 1, 0)

        def feat_piece(blk, t, p):
            def run():
                ep, en, sp, sn = _dual_exp(_mix(blk, lambda m: pq[m, t][64 * p:64 * p + 64]))
                z = z_v[8 * (blk // 2) + p]
                dp, dn = _pair_reduce(ep * z[0:64], jnp.add), _pair_reduce(en * z[64:128], jnp.add)
                inv = _recip(dp * sn + sp * (dn + 1e-6 * sn))
                return put_phi(blk, p, t, zero, ep * _rep8(sn * inv), en * _rep8(sp * inv))
            return run

        def hidden_piece(c, half):
            def run():
                for k, w in enumerate((wg_v, wu_v)):
                    acc = f_v[2 * c + k + zero] if half else None
                    f_v[2 * c + k] = _matvec(w.at[i], xc_v, c, 32 * half, 32 * half + 32, acc)
                return pltpu.bitcast(f_v[22 + zero], _I32)
            return run

        def act_piece(c):
            def run():
                hg, hu = (jnp.sum(f_v[2 * c + k + zero], axis=0, keepdims=True) for k in range(2))
                hc_v[128 * c:128 * c + 128, :] = _col_bcast(hg * jax.nn.sigmoid(hg) * hu)
            return run

        def down_piece(c, half):
            def run():
                for cc in (c, c + 1):
                    f_v[14 + cc] = _matvec(wd_v.at[i], hc_v, cc, 28 * half, 28 * half + 28, f_v[14 + cc + zero])
                return pltpu.bitcast(f_v[22 + zero], _I32)
            return run

        def emit_piece(blk, u, c):
            def run():
                h, d = blk // 2, blk % 2
                g = g_v[4 * ti + 2 * h + u]
                tok = jax.lax.broadcasted_iota(_I32, (128, 128), 0) + (ti * _T + _HT * h + 128 * u)
                o = []
                for cc in (c, c + 1):
                    y = jnp.sum(f_v[14 + 4 * d + cc + zero], axis=0, keepdims=True) * r_sel
                    b = _bf(x_blk(ti, 2 * d + h)[64 * u:64 * u + 64, 128 * cc:128 * cc + 128]).astype(_F32)
                    b = b + jnp.where(tok == idx, y, 0.0)
                    o.append(g * _mix(blk, lambda m: po[m, cc][128 * u:128 * u + 128]) + (1.0 - g) * b)
                out_v[blk][ti, 128 * u:128 * u + 128, 128 * c:128 * c + 256] = (
                    jnp.concatenate(o, axis=1).astype(_BF))
                if (u, c) == (1, 2):
                    cp_o(ti, blk).start()
                    out_v[blk][_NT, 16:32, 0:128] = jnp.zeros((16, 128), _BF)
                return pltpu.bitcast(out_v[blk][_NT + zero, 0:16, 0:128], _I32)
            return run

        def pieces(name):
            if name[0] == "h":
                return [hidden_piece(c, int(name[1])) for c in range(_FC // 128)]
            if name == "a":
                return [act_piece(c) for c in range(_FC // 128)]
            if name == "d":
                return [down_piece(c, half) for c in (4, 6, 0, 2) for half in range(2)]
            if name[0] == "e":
                return [emit_piece(int(name[1]), u, c) for c in (0, 2) for u in range(2)]
            return [feat_piece(int(name[1]), t, p) for t in ([int(name[2])] if name[2:] else range(2))
                    for p in range(8)]

        _play(_PHASE2, {"q": (qprod, 2), "o": (oprod, 4), "g": (attn, 2)}, pieces)

    pl.loop(0, _NT)(phase2)
    for t in range(_NT):
        for blk in range(4):
            cp_o(t, blk).wait()


@jax.jit
def pallas_gated_mix__linear_kernel_hedgehog__moe_arch_mod__prompt_kernel(
    A_x: jax.Array,
    A_wqkv: jax.Array,
    A_w_phi: jax.Array,
    A_wo: jax.Array,
    B_x: jax.Array,
    B_w_r: jax.Array,
    B_w_gate: jax.Array,
    B_w_up: jax.Array,
    B_w_down: jax.Array,
    gate_w: jax.Array,
):
    del B_x
    hbm = pl.BlockSpec(memory_space=pl.ANY)
    dma = pltpu.SemaphoreType.DMA
    out = pl.pallas_call(
        _kernel,
        out_shape=jax.ShapeDtypeStruct((_S, _D), _BF),
        in_specs=[hbm] * 9,
        out_specs=hbm,
        scratch_shapes=[
            pltpu.VMEM((_NT, _HT, _D), _I32),
            pltpu.VMEM((2, _HD, _D), _I32),
            pltpu.VMEM((_NT, _HD, _FC), _I32),
            pltpu.VMEM((_NT, _HD, _FC), _I32),
            pltpu.VMEM((_NT, _FC // 2, _D), _I32),
            pltpu.VMEM((_H, _DH, _DH), _BF),
            pltpu.VMEM((_D,), _BF),
            pltpu.VMEM((_D,), _BF),
            pltpu.VMEM((4, 256, _HD), _I32),
            pltpu.VMEM((4, 256, _HD), _I32),
            pltpu.VMEM((2, 8, 8, 16, 128), _BF),
            pltpu.VMEM((1, 1, 4, 16, 128), _BF),
            pltpu.VMEM((7, 32, 4, 16, 128), _BF),
            pltpu.VMEM((7, 32, 4, 16, 128), _BF),
            [pltpu.VMEM((8, 16, 2, 16, 128), _BF)] * 7,
            pltpu.VMEM((6, 32, 4, 16, 128), _BF),
            [pltpu.VMEM((_NT, 16, 4, 16, 128), _BF)] * 5,
            [pltpu.VMEM((7 * _NT + 1, 8, 2, 16, 128), _BF)] * 7,
            [pltpu.VMEM((17, 8, 1, 16, 128), _BF)] * 4,
            [[pltpu.VMEM((_HD, 128), _F32)] * 2] * 4,
            pltpu.VMEM((_NP, 64, 128), _F32),
            pltpu.VMEM((_NP + 1, 128, 128), _F32),
            pltpu.VMEM((_NP, 4, 1, 16, 128), _BF),
            pltpu.VMEM((_S // 128 + 1, 128, 128), _F32),
            pltpu.VMEM((8, 128), _F32),
            pltpu.VMEM((2, 8, 128), _I32),
            pltpu.VMEM((23, 8, 128), _F32),
            pltpu.VMEM((_D + 8, 128), _F32),
            pltpu.VMEM((_FC, 128), _F32),
            [pltpu.VMEM((_NT + 1, _HT, _HD), _BF)] * 4,
            dma((_NT,)), dma((2,)), dma((4,)), dma((4,)), dma((3,)),
            dma((_NT,)), dma((_NT,)), dma((_NT,)), dma((4 * _NT,)),
        ],
        compiler_params=pltpu.CompilerParams(vmem_limit_bytes=100 * 1024 * 1024, disable_semaphore_checks=True),
    )(A_x.reshape(_S, _D), A_wqkv, A_w_phi, A_wo, B_w_r, B_w_gate, B_w_up, B_w_down, gate_w)
    return out.reshape(1, _S, _D)
```
